```python
import jax
import jax.numpy as jnp

def _softmax(x, axis=-1):
    return jax.nn.softmax(x, axis=axis)
def _gelu(x):
    return jax.nn.gelu(x, approximate=True)
def _silu(x):
    return jax.nn.silu(x)
def _sigmoid(x):
    return jax.nn.sigmoid(x)
def _layernorm(x, axis=-1, eps=1e-5):
    m = jnp.mean(x, axis=axis, keepdims=True)
    v = jnp.var(x, axis=axis, keepdims=True)
    return (x - m) / jnp.sqrt(v + eps)
def _scatter_add(tgt, idx, src, axis=0):
    return tgt.at[idx].add(src)
def _segment_sum(src, seg, n):
    return jax.ops.segment_sum(src, seg, n)
class _Rng:
    def __init__(self, key):
        self._k = key
    def _next(self):
        self._k, sub = jax.random.split(self._k)
        return sub
    def normal(self, shape):
        return jax.random.normal(self._next(), shape, dtype=jnp.bfloat16)
    def randint(self, lo, hi, shape):
        return jax.random.randint(self._next(), shape, lo, hi, dtype=jnp.int32)
    def uniform(self, shape, lo=0.0, hi=1.0):
        return jax.random.uniform(self._next(), shape, jnp.bfloat16, lo, hi)
    def permutation(self, n):
        return jax.random.permutation(self._next(), n)


kernel_name = 'sequential_preLN__linear_attn_block__moe_arch_mod__prompt'

def setup_inputs():
    _rng = _Rng(jax.random.key(int.from_bytes(__import__("os").urandom(4), "little")))
    _w = (lambda a: (lambda t: t.astype(jnp.bfloat16) if jnp.issubdtype(t.dtype, jnp.floating) else t)(jnp.asarray(a)))
    def _A_setup():
        B, S, D = 1, 2048, 1024
        return {
            "x": _w((lambda *s: _rng.normal(s) * 0.05)(B, S, D)),
            "wqkv": _w((lambda *s: _rng.normal(s) * 0.05)(D, 3 * D)),
            "wo": _w((lambda *s: _rng.normal(s) * 0.05)(D, D)),
        }
    _A_in = _A_setup()

    def _B_setup():
        B, S, D, F, C = 1, 2048, 1024, 3584, 2
        return {
            "x": _w((lambda *s: _rng.normal(s) * 0.05)(B, S, D)),
            "w_r": _w((lambda *s: _rng.normal(s) * 0.05)(D)),
            "w_gate": _w((lambda *s: _rng.normal(s) * 0.05)(D, F)),
            "w_up": _w((lambda *s: _rng.normal(s) * 0.05)(D, F)),
            "w_down": _w((lambda *s: _rng.normal(s) * 0.05)(F, D)),
        }
    _B_in = _B_setup()

    return {
        "A_x": _A_in["x"],
        "A_wqkv": _A_in["wqkv"],
        "A_wo": _A_in["wo"],
        "B_x": _B_in["x"],
        "B_w_r": _B_in["w_r"],
        "B_w_gate": _B_in["w_gate"],
        "B_w_up": _B_in["w_up"],
        "B_w_down": _B_in["w_down"],
    }

def reference(A_x, A_wqkv, A_wo, B_x, B_w_r, B_w_gate, B_w_up, B_w_down):
    def _A_ref(x, wqkv, wo):
        B, S, D = x.shape
        H = 32; Dh = D // H
        qkv = (lambda x, *d: x.transpose(*d))((x @ wqkv).reshape(B, S, 3, H, Dh), 2, 0, 3, 1, 4)
        q, k, v = qkv[0], qkv[1], qkv[2]
        phi = lambda t: jnp.where(t > 0, t + 1, jnp.exp(t)) + 1e-6
        pq, pk = phi(q), phi(k)
        kv = jnp.einsum("bhsd,bhse->bhde", pk, v)
        z = jnp.einsum("bhsd->bhd", pk)
        num = jnp.einsum("bhqd,bhde->bhqe", pq, kv)
        den = jnp.einsum("bhqd,bhd->bhq", pq, z)[..., None] + 1e-6
        o = num / den
        return (lambda x, *d: x.transpose(*d))(o, 0, 2, 1, 3).reshape(B, S, D) @ wo

    def _B_ref(x, w_r, w_gate, w_up, w_down):
        B, S, D = x.shape
        C = 2
        r = x @ w_r
        idx = jnp.argsort(-r, axis=-1)[:, :C]
        idx_e = jnp.repeat(idx.reshape(B, C, 1), D, axis=2)
        x_sel = jnp.take_along_axis(x, idx_e, axis=1)
        g = _silu(x_sel @ w_gate)
        u = x_sel @ w_up
        y = (g * u) @ w_down
        r_sel = _sigmoid(jnp.take_along_axis(r, idx, axis=1))
        y = y * r_sel.reshape(B, C, 1)
        b_off = (jnp.arange(B) * S).reshape(B, 1)
        flat_idx = (idx + b_off).reshape(B * C)
        zero = (x * 0.0).reshape(B * S, D)
        upd = _scatter_add(zero, flat_idx, y.reshape(B * C, D), axis=0)
        return x + upd.reshape(B, S, D)

    x = A_x
    h = x + _A_ref(_layernorm(x, axis=-1), A_wqkv, A_wo)
    h2 = h + _B_ref(_layernorm(h, axis=-1), B_w_r, B_w_gate, B_w_up, B_w_down)
    return h2
```

```python
import functools

import jax
import jax.numpy as jnp
from jax import lax
import jax.experimental.pallas as pl
import jax.experimental.pallas.tpu as pltpu

S = 2048
D = 1024
F = 3584
H = 32
DH = D // H
LN_EPS = 1e-5
PHI_EPS = 1e-6
TM = 512
NT = S // TM
G = 128
NG = D // G
RB = 16

f32 = jnp.float32
bf16 = jnp.bfloat16


def _ln(x):
    mu = jnp.mean(x, axis=-1, keepdims=True)
    xc = x - mu
    var = jnp.mean(xc * xc, axis=-1, keepdims=True)
    return xc * lax.rsqrt(var + LN_EPS)


def _phi(t):
    return jnp.where(t > 0, t + 1.0, jnp.exp(t)) + PHI_EPS


def _dot(a, b):
    return jnp.dot(a, b, preferred_element_type=f32)


def _dot_nt(a, b):
    return lax.dot_general(a, b, (((1,), (1,)), ((), ())), preferred_element_type=f32)


def _dot_tn(a, b):
    return lax.dot_general(a, b, (((0,), (0,)), ((), ())), preferred_element_type=f32)


def _kernel(x_hbm, wqkv_hbm, wo_hbm, wr_ref, wg_hbm, wu_hbm, wd_hbm, out_hbm,
            x_v, xn_v, hn_v, out_v, wq_v, wk_v, wv_v, wo_v, wqt_v, p_v, m_v,
            wg_v, wu_v, wd_v, fix_v,
            sem_x, sem_w, sem_o, sem_f):
    def x_copy(t):
        return pltpu.make_async_copy(x_hbm.at[pl.ds(t * TM, TM)], x_v.at[pl.ds(t * TM, TM)], sem_x.at[t])

    def out_copy(t):
        return pltpu.make_async_copy(out_v.at[pl.ds(t * TM, TM)], out_hbm.at[pl.ds(t * TM, TM)], sem_o.at[t])

    wk_copy = pltpu.make_async_copy(wqkv_hbm.at[:, pl.ds(D, D)], wk_v, sem_w.at[0])
    wq_copy = pltpu.make_async_copy(wqkv_hbm.at[:, pl.ds(0, D)], wq_v, sem_w.at[1])
    wv_copy = pltpu.make_async_copy(wqkv_hbm.at[:, pl.ds(2 * D, D)], wv_v, sem_w.at[2])
    wo_copy = pltpu.make_async_copy(wo_hbm, wo_v, sem_w.at[3])
    wg_copy = pltpu.make_async_copy(wg_hbm, wg_v, sem_w.at[4])
    wu_copy = pltpu.make_async_copy(wu_hbm, wu_v, sem_w.at[5])
    wd_copy = pltpu.make_async_copy(wd_hbm, wd_v, sem_w.at[6])

    x_copy(0).start()
    wk_copy.start()
    for t in range(1, NT):
        x_copy(t).start()
    wq_copy.start()
    wv_copy.start()
    wo_copy.start()
    wg_copy.start()
    wu_copy.start()
    wd_copy.start()

    zacc = jnp.zeros((8, D), f32)
    for t in range(NT):
        rows = pl.ds(t * TM, TM)
        x_copy(t).wait()
        xn = _ln(x_v[rows, :].astype(f32)).astype(bf16)
        xn_v[rows, :] = xn
        if t == 0:
            wk_copy.wait()
        pk = _phi(_dot(xn, wk_v[...]))
        zacc = zacc + jnp.sum(pk.reshape(TM // 8, 8, D), axis=0)
        pp = _dot_tn(pk.astype(bf16), xn)
        if t == 0:
            p_v[...] = pp
        else:
            p_v[...] += pp
        if t == 1:
            wq_copy.wait()
            for c in range(NG):
                wqt_v[pl.ds(c * G, G), :] = wq_v[:, pl.ds(c * G, G)].T

    wv_copy.wait()
    wo_copy.wait()
    ri = lax.broadcasted_iota(jnp.int32, (G, G), 0) // DH
    ci = lax.broadcasted_iota(jnp.int32, (G, G), 1) // DH
    same_head = ri == ci
    for g in range(NG):
        sl = pl.ds(g * G, G)
        kv = _dot(p_v[sl, :].astype(bf16), wv_v[:, sl])
        kv = jnp.where(same_head, kv, 0.0).astype(bf16)
        m_v[sl, :] = _dot(kv, wo_v[sl, :]).astype(bf16)
    z = jnp.sum(zacc, axis=0, keepdims=True)
    zb = jnp.broadcast_to(z, (G, D)).T

    wr = wr_ref[...].astype(f32)
    imin = jnp.iinfo(jnp.int32).min
    k1 = jnp.full((1, 1), imin, jnp.int32)
    k2 = jnp.full((1, 1), imin, jnp.int32)
    for t in range(NT):
        rows = pl.ds(t * TM, TM)
        pqt = _phi(_dot_nt(wqt_v[...], xn_v[rows, :]))
        zt = jnp.concatenate([zb] * (TM // G), axis=1)
        den = jnp.sum((pqt * zt).reshape(H, DH, TM), axis=1, keepdims=True) + PHI_EPS
        pqn = (pqt.reshape(H, DH, TM) * (1.0 / den)).reshape(D, TM).astype(bf16)
        attn = _dot_tn(pqn, m_v[...])
        h = x_v[rows, :].astype(f32) + attn
        hn = _ln(h)
        hn_v[rows, :] = hn.astype(bf16)
        out_v[rows, :] = (h + hn).astype(bf16)
        out_copy(t).start()
        r = jnp.sum(hn * wr, axis=-1, keepdims=True)
        u = lax.bitcast_convert_type(r, jnp.int32)
        u = u ^ ((u >> 31) & 0x7FFFFFFF)
        idx = lax.broadcasted_iota(jnp.int32, (TM, 1), 0) + t * TM
        key = (u & ~(S - 1)) | (S - 1 - idx)
        t1 = jnp.max(key, axis=0, keepdims=True)
        t2 = jnp.max(jnp.where(key == t1, imin, key), axis=0, keepdims=True)
        k2 = jnp.maximum(jnp.minimum(k1, t1), jnp.maximum(k2, t2))
        k1 = jnp.maximum(k1, t1)

    def unkey(k):
        i = (S - 1) - (k & (S - 1))
        u = k & ~(S - 1)
        u = u ^ ((u >> 31) & 0x7FFFFFFF)
        return i, lax.bitcast_convert_type(u, f32)

    i1v, r1 = unkey(k1)
    i2v, r2 = unkey(k2)
    i1 = i1v[0, 0]
    i2 = i2v[0, 0]
    b1 = pl.multiple_of((i1 // RB) * RB, RB)
    b2 = pl.multiple_of((i2 // RB) * RB, RB)
    rid = lax.broadcasted_iota(jnp.int32, (RB, 1), 0)
    row1 = jnp.sum(jnp.where(rid + b1 == i1, hn_v[pl.ds(b1, RB), :].astype(f32), 0.0), axis=0, keepdims=True)
    row2 = jnp.sum(jnp.where(rid + b2 == i2, hn_v[pl.ds(b2, RB), :].astype(f32), 0.0), axis=0, keepdims=True)
    xsel = jnp.where(rid == 0, row1, jnp.where(rid == 1, row2, 0.0)).astype(bf16)
    wg_copy.wait()
    wu_copy.wait()
    wd_copy.wait()
    gt = _dot(xsel, wg_v[...])
    ut = _dot(xsel, wu_v[...])
    a = (gt * jax.nn.sigmoid(gt) * ut).astype(bf16)
    y = _dot(a, wd_v[...])
    y1 = y[0:1, :] * jax.nn.sigmoid(r1)
    y2 = y[1:2, :] * jax.nn.sigmoid(r2)

    def fixed(b):
        gid = rid + b
        upd = jnp.where(gid == i1, y1, 0.0) + jnp.where(gid == i2, y2, 0.0)
        return (out_v[pl.ds(b, RB), :].astype(f32) + upd).astype(bf16)

    fix_v[0] = fixed(b1)
    fix_v[1] = fixed(b2)
    for t in range(NT):
        out_copy(t).wait()
    fix1 = pltpu.make_async_copy(fix_v.at[0], out_hbm.at[pl.ds(b1, RB)], sem_f.at[0])
    fix2 = pltpu.make_async_copy(fix_v.at[1], out_hbm.at[pl.ds(b2, RB)], sem_f.at[1])
    fix1.start()

    @pl.when(b1 != b2)
    def _():
        fix2.start()
        fix2.wait()

    fix1.wait()


@jax.jit
def pallas_sequential_preLN__linear_attn_block__moe_arch_mod__prompt_kernel(
    A_x: jax.Array,
    A_wqkv: jax.Array,
    A_wo: jax.Array,
    B_x: jax.Array,
    B_w_r: jax.Array,
    B_w_gate: jax.Array,
    B_w_up: jax.Array,
    B_w_down: jax.Array,
):
    del B_x
    any_spec = pl.BlockSpec(memory_space=pl.ANY)
    out = pl.pallas_call(
        _kernel,
        out_shape=jax.ShapeDtypeStruct((S, D), bf16),
        in_specs=[any_spec, any_spec, any_spec,
                  pl.BlockSpec(memory_space=pltpu.VMEM),
                  any_spec, any_spec, any_spec],
        out_specs=any_spec,
        scratch_shapes=[
            pltpu.VMEM((S, D), bf16),
            pltpu.VMEM((S, D), bf16),
            pltpu.VMEM((S, D), bf16),
            pltpu.VMEM((S, D), bf16),
            pltpu.VMEM((D, D), bf16),
            pltpu.VMEM((D, D), bf16),
            pltpu.VMEM((D, D), bf16),
            pltpu.VMEM((D, D), bf16),
            pltpu.VMEM((D, D), bf16),
            pltpu.VMEM((D, D), f32),
            pltpu.VMEM((D, D), bf16),
            pltpu.VMEM((D, F), bf16),
            pltpu.VMEM((D, F), bf16),
            pltpu.VMEM((F, D), bf16),
            pltpu.VMEM((2, RB, D), bf16),
            pltpu.SemaphoreType.DMA((NT,)),
            pltpu.SemaphoreType.DMA((7,)),
            pltpu.SemaphoreType.DMA((NT,)),
            pltpu.SemaphoreType.DMA((2,)),
        ],
        compiler_params=pltpu.CompilerParams(vmem_limit_bytes=100 * 1024 * 1024),
    )(A_x.reshape(S, D), A_wqkv, A_wo, B_w_r.reshape(1, D), B_w_gate, B_w_up, B_w_down)
    return out.reshape(1, S, D)
```

```python
import jax
import jax.numpy as jnp
from jax import lax
import jax.experimental.pallas as pl
import jax.experimental.pallas.tpu as pltpu

S = 2048
D = 1024
F = 3584
H = 32
DH = D // H
LN_EPS = 1e-5
PHI_EPS = 1e-6
G = 128
NG = D // G
RB = 16
FC = 256
NF = F // FC
T = 512
NT = S // T
HT = T // 2
PAD = HT

f32 = jnp.float32
bf16 = jnp.bfloat16
u32 = jnp.uint32
i32 = jnp.int32
IMIN = jnp.iinfo(jnp.int32).min

X_PIECES = ((0, 256), (256, 256), (512, 512), (1024, 1024))

SCOPES = False


def _zero_of(v):
    u = lax.bitcast_convert_type(v, u32)
    u = lax.shift_right_logical(lax.shift_right_logical(u, jnp.uint32(16)), jnp.uint32(16))
    return lax.bitcast_convert_type(u, f32)


def _phi(t):
    return jnp.where(t > 0, t + 1.0, jnp.exp(t)) + PHI_EPS


def _dot(a, b):
    return jnp.dot(a, b, preferred_element_type=f32)


def _dot_nt(a, b):
    return lax.dot_general(a, b, (((1,), (1,)), ((), ())), preferred_element_type=f32)


def _dot_tn(a, b):
    return lax.dot_general(a, b, (((0,), (0,)), ((), ())), preferred_element_type=f32)


def _half(lo, align):
    return lo // 2 if isinstance(lo, int) else pl.multiple_of(lo // 2, align // 2)


def _put(ref, lo, val, align=16):
    ref[pl.ds(_half(lo, align), val.shape[0] // 2), :] = pltpu.bitcast(val, u32)


def _get(ref, lo, n, align=16):
    return pltpu.bitcast(ref[pl.ds(_half(lo, align), n // 2), :], bf16)


def _rows(lo, n, align=16):
    return pl.ds(lo if isinstance(lo, int) else pl.multiple_of(lo, align), n)


def _kernel(x_hbm, wqkv_hbm, wo_hbm, wr_hbm, wg_hbm, wu_hbm, wd_hbm, out_hbm,
            x_v, xn_v, hn_v, out_v, wk_v, wq_v, wv_v, wo_v, wqt_v, p_v, m_v, zb_v, wr_v, wrf_v,
            keep_v, attn_v, za_v, wg_v, wu_v, wd_v, fix_v,
            sem_x, sem_k, sem_w, sem_o, sem_f):
    scope = [None]

    def mark(name):
        if not SCOPES:
            return
        if scope[0] is not None:
            scope[0].__exit__(None, None, None)
        scope[0] = None
        if name:
            scope[0] = jax.named_scope(name)
            scope[0].__enter__()

    def x_copy(i):
        lo, n = X_PIECES[i]
        return pltpu.make_async_copy(x_hbm.at[pl.ds(lo, n)], x_v.at[pl.ds(PAD + lo, n)], sem_x.at[i])

    def wk_copy(i):
        lo = i * 256 if isinstance(i, int) else pl.multiple_of(i * 256, 256)
        n = 512 if isinstance(i, int) and i == 2 else 256
        return pltpu.make_async_copy(wqkv_hbm.at[:, pl.ds(D + lo, n)], wk_v.at[:, pl.ds(lo, n)], sem_k.at[i])

    def wv_copy(i):
        return pltpu.make_async_copy(wqkv_hbm.at[:, pl.ds(2 * D + i * 512, 512)], wv_v.at[i], sem_w.at[i])

    def out_copy(lo, n, s):
        return pltpu.make_async_copy(out_v.at[_rows(lo + PAD, n)], out_hbm.at[_rows(lo, n)], sem_o.at[s])

    wo_copy = pltpu.make_async_copy(wo_hbm, wo_v, sem_w.at[2])
    wg_copy = pltpu.make_async_copy(wg_hbm, wg_v, sem_w.at[3])
    wu_copy = pltpu.make_async_copy(wu_hbm, wu_v, sem_w.at[4])
    wd_copy = pltpu.make_async_copy(wd_hbm, wd_v, sem_w.at[5])
    wr_copy = pltpu.make_async_copy(wr_hbm, wr_v, sem_w.at[6])
    wq_copy = pltpu.make_async_copy(wqkv_hbm.at[:, pl.ds(0, D)], wq_v, sem_w.at[7])

    x_copy(0).start()

    def start_wk(i, c):
        wk_copy(i).start()
        return c

    lax.fori_loop(0, 2, start_wk, 0)
    x_copy(1).start()

    def zero_pad(i, c):
        rows = pl.ds(pl.multiple_of(i * 32, 32), 32)
        x_v[rows, :] = jnp.zeros((32, D), bf16)
        attn_v[rows, :] = jnp.zeros((32, D), f32)
        return c

    lax.fori_loop(0, PAD // 32, zero_pad, 0)

    def ln_rows(lo, n, sub):
        link = None
        outs = []
        for q in range(0, n, sub):
            x = x_v[_rows(lo + (PAD + q), sub), :].astype(f32)
            mu = jnp.sum(x, axis=-1, keepdims=True) * (1.0 / D)
            if link is not None:
                mu = mu + link
            xc = x - mu
            var = jnp.sum(xc * xc, axis=-1, keepdims=True) * (1.0 / D)
            y = xc * lax.rsqrt(var + LN_EPS)
            link = _zero_of(y[:, D - G:])[:, 0:1]
            yb = y.astype(bf16)
            _put(xn_v, lo + q, yb)
            outs.append(yb)
        return jnp.concatenate(outs, axis=0) if len(outs) > 1 else outs[0]

    def kproj(xn, c0, c1):
        pk = _phi(_dot(xn, wk_v[:, pl.ds(c0, c1 - c0)]))
        zs = jnp.sum(pk.reshape(xn.shape[0] // 8, 8, c1 - c0), axis=0)
        return pk.astype(bf16), zs

    wk_copy(2).start()
    mark('W0')
    x_copy(0).wait()
    mark('R0')
    x_copy(2).start()
    ln_rows(0, 256, 256)
    mark('R12')

    def ka_body(i, c):
        wk_copy(i).wait()
        col = pl.multiple_of(i * 256, 256)
        pk = _phi(_dot(_get(xn_v, 0, 256), wk_v[:, pl.ds(col, 256)]))
        za_v[i] = jnp.sum(pk.reshape(32, 8, 256), axis=0)
        keep_v[i, pl.ds(0, 128), :] = pltpu.bitcast(pk.astype(bf16), u32)
        return c

    lax.fori_loop(0, 2, ka_body, 0)
    x_copy(3).start()
    wq_copy.start()
    mark('W3')
    x_copy(1).wait()
    mark('R3')
    wv_copy(0).start()
    wv_copy(1).start()
    wo_copy.start()
    wr_copy.start()
    pk_a = jnp.concatenate([pltpu.bitcast(keep_v[i, pl.ds(0, 128), :], bf16) for i in range(2)], axis=1)
    p_v[pl.ds(0, 512), :] = _dot_tn(pk_a, _get(xn_v, 0, 256))
    xb = ln_rows(256, 256, 64)
    pk_b, z_b = kproj(xb, 0, 512)
    p_v[pl.ds(0, 512), :] += _dot_tn(pk_b, xb)
    mark('W4')
    wk_copy(2).wait()
    x_copy(2).wait()
    mark('R4')
    wg_copy.start()
    wu_copy.start()
    wd_copy.start()
    x0 = _get(xn_v, 0, T)
    pk_c, z_c = kproj(x0, 512, D)
    p_v[pl.ds(512, 512), :] = _dot_tn(pk_c, x0)
    ln_rows(T, T, 64)
    zacc = jnp.concatenate([jnp.concatenate([za_v[0], za_v[1]], axis=1) + z_b, z_c], axis=1)
    mark('W5')
    x_copy(3).wait()
    wq_copy.wait()
    mark('L1')

    def l1_body(i, z):
        lo = (i + 1) * T
        xn = _get(xn_v, lo, T, T)
        pk, zs = kproj(xn, 0, D)
        p_v[...] += _dot_tn(pk, xn)
        nxt = jnp.minimum(i + 2, NT - 1) * T
        ln_rows(nxt, T, 32)
        c0 = jnp.minimum(i * 3, NG - 3) * G
        for c in range(3):
            col = pl.multiple_of(c0 + c * G, G)
            _put(wqt_v, col, wq_v[:, pl.ds(col, G)].T, G)
        return z + zs

    zacc = lax.fori_loop(0, NT - 1, l1_body, zacc)

    mark('W6')
    wv_copy(0).wait()
    wv_copy(1).wait()
    wo_copy.wait()
    wr_copy.wait()
    mark('M')

    def qproj(lo, n, zb):
        pqt = _phi(_dot_nt(_get(wqt_v, 0, D), _get(xn_v, lo, n, G)))
        zt = jnp.concatenate([zb] * (n // G), axis=1)
        den = jnp.sum((pqt * zt).reshape(H, DH, n), axis=1, keepdims=True) + PHI_EPS
        inv = pl.reciprocal(den, approx=True)
        inv = inv * (2.0 - den * inv)
        return (pqt.reshape(H, DH, n) * inv).reshape(D, n).astype(bf16)

    def ml_body(i, c):
        z = jnp.sum(zacc, axis=0, keepdims=True)
        zb = jnp.broadcast_to(z, (G, D)).T
        zb_v[...] = zb
        wrf_v[...] = jnp.broadcast_to(wr_v[...].reshape(1, D).astype(f32), (8, D))
        ri = lax.broadcasted_iota(i32, (G, G), 0) // DH
        ci = lax.broadcasted_iota(i32, (G, G), 1) // DH
        same_head = ri == ci
        base = i * (D // 2)
        kvs = {}

        def kv(g):
            t = _dot(p_v[_rows(base + g * G, G, G), :].astype(bf16), wv_v[i, :, pl.ds(g * G, G)])
            kvs[g] = jnp.where(same_head, t, 0.0).astype(bf16)

        def mrow(g):
            _put(m_v, base + g * G, _dot(kvs.pop(g), wo_v[_rows(base + g * G, G, G), :]).astype(bf16), G)

        kv(0)
        kv(1)
        mrow(0)
        keep_v[i] = pltpu.bitcast(qproj(i * HT, HT, zb), u32)
        kv(2)
        mrow(1)
        kv(3)
        mrow(2)
        mrow(3)
        return c

    lax.fori_loop(0, 2, ml_body, 0)

    sub_id = lax.broadcasted_iota(i32, (8, G), 0)

    def keys(r, lo, n):
        rb = lax.bitcast_convert_type(jnp.broadcast_to(r, (n, G)), i32)
        u = rb ^ ((rb >> 31) & 0x7FFFFFFF)
        code0 = (S - 1 - lo) - sub_id
        return rb, [(u[s8:s8 + 8] & ~(S - 1)) | (code0 - s8) for s8 in range(0, n, 8)]

    def merge(a1, a2, b1, b2):
        gt = a1 > b1
        lo = jnp.where(gt, b1, a1)
        other = jnp.where(gt, a2, b2)
        return jnp.where(gt, a1, b1), jnp.where(lo > other, lo, other)

    def post(lo, attn, n, sub, state, link):
        k1, k2 = state
        wr = wrf_v[0:1, :]
        for q in range(0, n, sub):
            rows = _rows(lo + (PAD + q), sub)
            h = x_v[rows, :].astype(f32) + attn[q:q + sub]
            mu = jnp.broadcast_to(jnp.sum(h, axis=-1, keepdims=True) * (1.0 / D), (sub, G))
            if link is not None:
                mu = mu + link
            xc = h - jnp.concatenate([mu] * NG, axis=1)
            var = jnp.sum(xc * xc, axis=-1, keepdims=True) * (1.0 / D)
            hn = xc * lax.rsqrt(var + LN_EPS)
            hn_v[rows, :] = hn
            out_v[rows, :] = (h + hn).astype(bf16)
            rb, ks = keys(jnp.sum(hn * wr, axis=-1, keepdims=True), lo + q, sub)
            link = _zero_of(rb | jnp.concatenate([k2] * (sub // 8), axis=0))
            for key in ks:
                gt = key > k1
                lo2 = jnp.where(gt, k1, key)
                k2 = jnp.where(lo2 > k2, lo2, k2)
                k1 = jnp.where(gt, key, k1)
        return (k1, k2), link

    def post_last(lo, attn, n, state):
        rows = pl.ds(lo + PAD, n)
        h = x_v[rows, :].astype(f32) + attn
        xc = h - jnp.sum(h, axis=-1, keepdims=True) * (1.0 / D)
        var = jnp.sum(xc * xc, axis=-1, keepdims=True) * (1.0 / D)
        t = jnp.sum(xc * wrf_v[0:1, :], axis=-1, keepdims=True)
        rstd = lax.rsqrt(var + LN_EPS)
        hn = xc * rstd
        hn_v[rows, :] = hn
        out_v[rows, :] = (h + hn).astype(bf16)
        _, ks = keys(t * rstd, lo, n)
        pairs = []
        for a, b in zip(ks[0::2], ks[1::2]):
            gt = a > b
            pairs.append((jnp.where(gt, a, b), jnp.where(gt, b, a)))
        pairs.append(state)
        while len(pairs) > 1:
            nxt = [merge(*pairs[j], *pairs[j + 1]) for j in range(0, len(pairs) - 1, 2)]
            pairs = nxt + pairs[len(nxt) * 2:]
        return pairs[0]

    def keep_load():
        return jnp.concatenate([pltpu.bitcast(keep_v[0], bf16), pltpu.bitcast(keep_v[1], bf16)], axis=1)

    def l2_body(i, state):
        lo = i * T
        lhs = keep_load()
        pqn = pltpu.bitcast(qproj(lo + T, T, zb_v[...]), u32)
        keep_v[0] = pqn[:, :HT]
        keep_v[1] = pqn[:, HT:]
        (k1, k2), _ = post(lo - HT, attn_v[...], HT, 16, state, None)
        state = jnp.where(i > 0, k1, IMIN), jnp.where(i > 0, k2, IMIN)

        @pl.when(i > 0)
        def _():
            out_copy(lo - HT, HT, 2 * i - 1).start()

        m = _get(m_v, 0, D)
        at = _dot_tn(lhs[:, :HT], m)
        attn_v[...] = _dot_tn(lhs[:, HT:], m)
        state, _ = post(lo, at, HT, 32, state, None)
        out_copy(lo, HT, 2 * i).start()
        return state

    mark('L2')
    init = jnp.full((8, G), IMIN, i32)
    state = lax.fori_loop(0, NT - 1, l2_body, (init, init))

    mark('W7')
    wg_copy.wait()
    wu_copy.wait()
    wd_copy.wait()
    mark('T')
    lhs = keep_load()
    m = _get(m_v, 0, D)
    lo = S - T
    at_a = _dot_tn(lhs[:, :256], m)
    at_b = _dot_tn(lhs[:, 256:384], m)
    at_c = _dot_tn(lhs[:, 384:], m)
    state, link = post(lo - HT, attn_v[...], HT, 32, state, None)
    state, link = post(lo, at_a, 256, 32, state, link)
    out_copy(lo - HT, T, 2 * NT - 3).start()
    state, link = post(lo + 256, at_b, 128, 32, state, link)
    k1, k2 = post_last(lo + 384, at_c, 128, state)
    out_copy(lo + HT, HT, 2 * NT - 2).start()

    for sh in (4, 2, 1):
        k1, k2 = merge(k1, k2, pltpu.roll(k1, sh, 0), pltpu.roll(k2, sh, 0))
    k1 = k1[0:1]
    k2 = k2[0:1]

    def unkey(k):
        i = (S - 1) - (k & (S - 1))
        v = k & ~(S - 1)
        v = v ^ ((v >> 31) & 0x7FFFFFFF)
        return i, lax.bitcast_convert_type(v, f32)

    i1v, r1 = unkey(k1)
    i2v, r2 = unkey(k2)
    i1 = i1v[0, 0]
    i2 = i2v[0, 0]
    b1 = pl.multiple_of((i1 // RB) * RB, RB)
    b2 = pl.multiple_of((i2 // RB) * RB, RB)
    rid = lax.broadcasted_iota(i32, (RB, 1), 0)

    rid8 = lax.broadcasted_iota(i32, (8, D), 0)
    xs = jnp.where(rid8 == 0, jnp.broadcast_to(hn_v[pl.ds(i1 + PAD, 1), :], (8, D)),
                   jnp.broadcast_to(hn_v[pl.ds(i2 + PAD, 1), :], (8, D)))
    xsel = jnp.concatenate([xs, xs], axis=0).astype(bf16)

    acts = {}

    def gu(c):
        sl = pl.ds(c * FC, FC)
        gt = _dot(xsel, wg_v[:, sl])
        ut = _dot(xsel, wu_v[:, sl])
        acts[c] = (gt * jax.nn.sigmoid(gt) * ut).astype(bf16)

    y = None
    gu(0)
    for c in range(NF):
        if c + 1 < NF:
            gu(c + 1)
        t = _dot(acts.pop(c), wd_v[pl.ds(c * FC, FC), :])
        y = t if y is None else y + t
    s1 = jnp.concatenate([jax.nn.sigmoid(r1)] * NG, axis=1)
    s2 = jnp.concatenate([jax.nn.sigmoid(r2)] * NG, axis=1)
    y1 = y[0:1, :] * s1
    y2 = y[1:2, :] * s2

    def fixed(b):
        gid = rid + b
        upd = jnp.where(gid == i1, y1, 0.0) + jnp.where(gid == i2, y2, 0.0)
        return (out_v[_rows(b + PAD, RB), :].astype(f32) + upd).astype(bf16)

    fix_v[0] = fixed(b1)
    fix_v[1] = fixed(b2)
    mark('W8')
    for i in range(2 * NT - 3):
        out_copy(i * HT, HT, i).wait()
    out_copy(lo - HT, T, 2 * NT - 3).wait()
    out_copy(lo + HT, HT, 2 * NT - 2).wait()
    mark('E')
    fix1 = pltpu.make_async_copy(fix_v.at[0], out_hbm.at[pl.ds(b1, RB)], sem_f.at[0])
    fix2 = pltpu.make_async_copy(fix_v.at[1], out_hbm.at[pl.ds(b2, RB)], sem_f.at[1])
    fix1.start()

    @pl.when(b1 != b2)
    def _():
        fix2.start()
        fix2.wait()

    fix1.wait()
    mark(None)


@jax.jit
def pallas_sequential_preLN__linear_attn_block__moe_arch_mod__prompt_kernel(
    A_x: jax.Array,
    A_wqkv: jax.Array,
    A_wo: jax.Array,
    B_x: jax.Array,
    B_w_r: jax.Array,
    B_w_gate: jax.Array,
    B_w_up: jax.Array,
    B_w_down: jax.Array,
):
    del B_x
    any_spec = pl.BlockSpec(memory_space=pl.ANY)
    out = pl.pallas_call(
        _kernel,
        out_shape=jax.ShapeDtypeStruct((S, D), bf16),
        in_specs=[any_spec] * 7,
        out_specs=any_spec,
        scratch_shapes=[
            pltpu.VMEM((PAD + S, D), bf16),
            pltpu.VMEM((S // 2, D), u32),
            pltpu.VMEM((PAD + S, D), f32),
            pltpu.VMEM((PAD + S, D), bf16),
            pltpu.VMEM((D, D), bf16),
            pltpu.VMEM((D, D), bf16),
            pltpu.VMEM((2, D, D // 2), bf16),
            pltpu.VMEM((D, D), bf16),
            pltpu.VMEM((D // 2, D), u32),
            pltpu.VMEM((D, D), f32),
            pltpu.VMEM((D // 2, D), u32),
            pltpu.VMEM((D, G), f32),
            pltpu.VMEM((D,), bf16),
            pltpu.VMEM((8, D), f32),
            pltpu.VMEM((2, D // 2, HT), u32),
            pltpu.VMEM((HT, D), f32),
            pltpu.VMEM((2, 8, 256), f32),
            pltpu.VMEM((D, F), bf16),
            pltpu.VMEM((D, F), bf16),
            pltpu.VMEM((F, D), bf16),
            pltpu.VMEM((2, RB, D), bf16),
            pltpu.SemaphoreType.DMA((len(X_PIECES),)),
            pltpu.SemaphoreType.DMA((3,)),
            pltpu.SemaphoreType.DMA((8,)),
            pltpu.SemaphoreType.DMA((2 * NT - 1,)),
            pltpu.SemaphoreType.DMA((2,)),
        ],
        compiler_params=pltpu.CompilerParams(vmem_limit_bytes=100 * 1024 * 1024, disable_bounds_checks=True, disable_semaphore_checks=True),
    )(A_x.reshape(S, D), A_wqkv, A_wo, B_w_r, B_w_gate, B_w_up, B_w_down)
    return out.reshape(1, S, D)
```

```python
import jax
import jax.numpy as jnp
from jax import lax
import jax.experimental.pallas as pl
import jax.experimental.pallas.tpu as pltpu

S = 2048
D = 1024
F = 3584
H = 32
DH = D // H
LN_EPS = 1e-5
PHI_EPS = 1e-6
G = 128
NG = D // G
RB = 16
FC = 256
NF = F // FC
T = 512
NT = S // T
HT = T // 2
PAD = HT

f32 = jnp.float32
bf16 = jnp.bfloat16
u32 = jnp.uint32
i32 = jnp.int32
IMIN = jnp.iinfo(jnp.int32).min

X_PIECES = ((0, 256), (256, 256), (512, 512), (1024, 1024))

SCOPES = False


def _zero_of(v):
    u = lax.bitcast_convert_type(v, u32)
    u = lax.shift_right_logical(lax.shift_right_logical(u, jnp.uint32(16)), jnp.uint32(16))
    return lax.bitcast_convert_type(u, f32)


def _phi(t):
    return jnp.where(t > 0, t + 1.0, jnp.exp(t)) + PHI_EPS


def _dot(a, b):
    return jnp.dot(a, b, preferred_element_type=f32)


def _dot_nt(a, b):
    return lax.dot_general(a, b, (((1,), (1,)), ((), ())), preferred_element_type=f32)


def _dot_tn(a, b):
    return lax.dot_general(a, b, (((0,), (0,)), ((), ())), preferred_element_type=f32)


def _half(lo, align):
    return lo // 2 if isinstance(lo, int) else pl.multiple_of(lo // 2, align // 2)


def _put(ref, lo, val, align=16):
    ref[pl.ds(_half(lo, align), val.shape[0] // 2), :] = pltpu.bitcast(val, u32)


def _get(ref, lo, n, align=16):
    return pltpu.bitcast(ref[pl.ds(_half(lo, align), n // 2), :], bf16)


def _rows(lo, n, align=16):
    return pl.ds(lo if isinstance(lo, int) else pl.multiple_of(lo, align), n)


def _kernel(x_hbm, wqkv_hbm, wo_hbm, wr_hbm, wg_hbm, wu_hbm, wd_hbm, out_hbm,
            x_v, xn_v, hn_v, out_v, wk_v, wq_v, wv_v, wo_v, wqt_v, p_v, m_v, zb_v, wr_v, wrf_v,
            keep_v, attn_v, za_v, pka_v, wg_v, wu_v, wd_v, fix_v,
            sem_x, sem_k, sem_w, sem_o, sem_f):
    scope = [None]

    def mark(name):
        if not SCOPES:
            return
        if scope[0] is not None:
            scope[0].__exit__(None, None, None)
        scope[0] = None
        if name:
            scope[0] = jax.named_scope(name)
            scope[0].__enter__()

    def x_copy(i):
        lo, n = X_PIECES[i]
        return pltpu.make_async_copy(x_hbm.at[pl.ds(lo, n)], x_v.at[pl.ds(PAD + lo, n)], sem_x.at[i])

    def wk_copy(i):
        lo = i * G if isinstance(i, int) else pl.multiple_of(i * G, G)
        n = 512 if isinstance(i, int) and i == 4 else G
        return pltpu.make_async_copy(wqkv_hbm.at[:, pl.ds(D + lo, n)], wk_v.at[:, pl.ds(lo, n)], sem_k.at[i])

    def wv_copy(i):
        return pltpu.make_async_copy(wqkv_hbm.at[:, pl.ds(2 * D + i * 512, 512)], wv_v.at[i], sem_w.at[i])

    def out_copy(lo, n, s):
        return pltpu.make_async_copy(out_v.at[_rows(lo + PAD, n)], out_hbm.at[_rows(lo, n)], sem_o.at[s])

    wo_copy = pltpu.make_async_copy(wo_hbm, wo_v, sem_w.at[2])
    wg_copy = pltpu.make_async_copy(wg_hbm, wg_v, sem_w.at[3])
    wu_copy = pltpu.make_async_copy(wu_hbm, wu_v, sem_w.at[4])
    wd_copy = pltpu.make_async_copy(wd_hbm, wd_v, sem_w.at[5])
    wr_copy = pltpu.make_async_copy(wr_hbm, wr_v, sem_w.at[6])
    wq_copy = pltpu.make_async_copy(wqkv_hbm.at[:, pl.ds(0, D)], wq_v, sem_w.at[7])

    x_copy(0).start()

    def start_wk(i, c):
        wk_copy(i).start()
        return c

    lax.fori_loop(0, 4, start_wk, 0)
    x_copy(1).start()

    def zero_pad(i, c):
        rows = pl.ds(pl.multiple_of(i * 32, 32), 32)
        x_v[rows, :] = jnp.zeros((32, D), bf16)
        attn_v[rows, :] = jnp.zeros((32, D), f32)
        return c

    lax.fori_loop(0, PAD // 32, zero_pad, 0)

    def ln_rows(lo, n, sub):
        link = None
        outs = []
        for q in range(0, n, sub):
            x = x_v[_rows(lo + (PAD + q), sub), :].astype(f32)
            mu = jnp.sum(x, axis=-1, keepdims=True) * (1.0 / D)
            if link is not None:
                mu = mu + link
            xc = x - mu
            var = jnp.sum(xc * xc, axis=-1, keepdims=True) * (1.0 / D)
            y = xc * lax.rsqrt(var + LN_EPS)
            link = _zero_of(y[:, D - G:])[:, 0:1]
            yb = y.astype(bf16)
            _put(xn_v, lo + q, yb)
            outs.append(yb)
        return jnp.concatenate(outs, axis=0) if len(outs) > 1 else outs[0]

    def kproj(xn, c0, c1):
        pk = _phi(_dot(xn, wk_v[:, pl.ds(c0, c1 - c0)]))
        zs = jnp.sum(pk.reshape(xn.shape[0] // 8, 8, c1 - c0), axis=0)
        return pk.astype(bf16), zs

    wk_copy(4).start()
    mark('W0')
    x_copy(0).wait()
    mark('R0')
    x_copy(2).start()
    ln_rows(0, 256, 256)
    mark('R12')

    def ka_body(i, c):
        wk_copy(i).wait()
        col = pl.multiple_of(i * G, G)
        pk = _phi(_dot(_get(xn_v, 0, 256), wk_v[:, pl.ds(col, G)]))
        za_v[i] = jnp.sum(pk.reshape(32, 8, G), axis=0)
        pka_v[i] = pltpu.bitcast(pk.astype(bf16), u32)
        return c

    lax.fori_loop(0, 4, ka_body, 0)
    x_copy(3).start()
    wq_copy.start()
    mark('W3')
    x_copy(1).wait()
    mark('R3')
    wv_copy(0).start()
    wv_copy(1).start()
    wo_copy.start()
    wr_copy.start()
    pk_a = jnp.concatenate([pltpu.bitcast(pka_v[i], bf16) for i in range(4)], axis=1)
    p_v[pl.ds(0, 512), :] = _dot_tn(pk_a, _get(xn_v, 0, 256))
    xb = ln_rows(256, 256, 64)
    pk_b, z_b = kproj(xb, 0, 512)
    p_v[pl.ds(0, 512), :] += _dot_tn(pk_b, xb)
    mark('W4')
    wk_copy(4).wait()
    x_copy(2).wait()
    mark('R4')
    wg_copy.start()
    wu_copy.start()
    wd_copy.start()
    x0 = _get(xn_v, 0, T)
    pk_c, z_c = kproj(x0, 512, D)
    p_v[pl.ds(512, 512), :] = _dot_tn(pk_c, x0)
    ln_rows(T, T, 64)
    zacc = jnp.concatenate([jnp.concatenate([za_v[i] for i in range(4)], axis=1) + z_b, z_c], axis=1)
    mark('W5')
    x_copy(3).wait()
    wq_copy.wait()
    mark('L1')

    def l1_body(i, z):
        lo = (i + 1) * T
        xn = _get(xn_v, lo, T, T)
        pk, zs = kproj(xn, 0, D)
        p_v[...] += _dot_tn(pk, xn)
        nxt = jnp.minimum(i + 2, NT - 1) * T
        ln_rows(nxt, T, 32)
        c0 = jnp.minimum(i * 3, NG - 3) * G
        for c in range(3):
            col = pl.multiple_of(c0 + c * G, G)
            _put(wqt_v, col, wq_v[:, pl.ds(col, G)].T, G)
        return z + zs

    zacc = lax.fori_loop(0, NT - 1, l1_body, zacc)

    mark('W6')
    wv_copy(0).wait()
    wv_copy(1).wait()
    wo_copy.wait()
    wr_copy.wait()
    mark('M')

    def qproj(lo, n, zb):
        pqt = _phi(_dot_nt(_get(wqt_v, 0, D), _get(xn_v, lo, n, G)))
        zt = jnp.concatenate([zb] * (n // G), axis=1)
        den = jnp.sum((pqt * zt).reshape(H, DH, n), axis=1, keepdims=True) + PHI_EPS
        inv = pl.reciprocal(den, approx=True)
        inv = inv * (2.0 - den * inv)
        return (pqt.reshape(H, DH, n) * inv).reshape(D, n).astype(bf16)

    def ml_body(i, c):
        z = jnp.sum(zacc, axis=0, keepdims=True)
        zb = jnp.broadcast_to(z, (G, D)).T
        zb_v[...] = zb
        wrf_v[...] = jnp.broadcast_to(wr_v[...].reshape(1, D).astype(f32), (8, D))
        ri = lax.broadcasted_iota(i32, (G, G), 0) // DH
        ci = lax.broadcasted_iota(i32, (G, G), 1) // DH
        same_head = ri == ci
        base = i * (D // 2)
        kvs = {}

        def kv(g):
            t = _dot(p_v[_rows(base + g * G, G, G), :].astype(bf16), wv_v[i, :, pl.ds(g * G, G)])
            kvs[g] = jnp.where(same_head, t, 0.0).astype(bf16)

        def mrow(g):
            _put(m_v, base + g * G, _dot(kvs.pop(g), wo_v[_rows(base + g * G, G, G), :]).astype(bf16), G)

        kv(0)
        kv(1)
        mrow(0)
        keep_v[i] = pltpu.bitcast(qproj(i * HT, HT, zb), u32)
        kv(2)
        mrow(1)
        kv(3)
        mrow(2)
        mrow(3)
        return c

    lax.fori_loop(0, 2, ml_body, 0)

    sub_id = lax.broadcasted_iota(i32, (8, G), 0)

    def keys(r, lo, n):
        rb = lax.bitcast_convert_type(jnp.broadcast_to(r, (n, G)), i32)
        u = rb ^ ((rb >> 31) & 0x7FFFFFFF)
        code0 = (S - 1 - lo) - sub_id
        return rb, [(u[s8:s8 + 8] & ~(S - 1)) | (code0 - s8) for s8 in range(0, n, 8)]

    def merge(a1, a2, b1, b2):
        gt = a1 > b1
        lo = jnp.where(gt, b1, a1)
        other = jnp.where(gt, a2, b2)
        return jnp.where(gt, a1, b1), jnp.where(lo > other, lo, other)

    def post(lo, attn, n, sub, state, link):
        k1, k2 = state
        wr = wrf_v[0:1, :]
        for q in range(0, n, sub):
            rows = _rows(lo + (PAD + q), sub)
            h = x_v[rows, :].astype(f32) + attn[q:q + sub]
            mu = jnp.broadcast_to(jnp.sum(h, axis=-1, keepdims=True) * (1.0 / D), (sub, G))
            if link is not None:
                mu = mu + link
            xc = h - jnp.concatenate([mu] * NG, axis=1)
            var = jnp.sum(xc * xc, axis=-1, keepdims=True) * (1.0 / D)
            hn = xc * lax.rsqrt(var + LN_EPS)
            hn_v[rows, :] = hn
            out_v[rows, :] = (h + hn).astype(bf16)
            rb, ks = keys(jnp.sum(hn * wr, axis=-1, keepdims=True), lo + q, sub)
            link = _zero_of(rb | jnp.concatenate([k2] * (sub // 8), axis=0))
            for key in ks:
                gt = key > k1
                lo2 = jnp.where(gt, k1, key)
                k2 = jnp.where(lo2 > k2, lo2, k2)
                k1 = jnp.where(gt, key, k1)
        return (k1, k2), link

    def post_last(lo, attn, n, state):
        rows = pl.ds(lo + PAD, n)
        h = x_v[rows, :].astype(f32) + attn
        xc = h - jnp.sum(h, axis=-1, keepdims=True) * (1.0 / D)
        var = jnp.sum(xc * xc, axis=-1, keepdims=True) * (1.0 / D)
        t = jnp.sum(xc * wrf_v[0:1, :], axis=-1, keepdims=True)
        rstd = lax.rsqrt(var + LN_EPS)
        hn = xc * rstd
        hn_v[rows, :] = hn
        out_v[rows, :] = (h + hn).astype(bf16)
        _, ks = keys(t * rstd, lo, n)
        pairs = []
        for a, b in zip(ks[0::2], ks[1::2]):
            gt = a > b
            pairs.append((jnp.where(gt, a, b), jnp.where(gt, b, a)))
        pairs.append(state)
        while len(pairs) > 1:
            nxt = [merge(*pairs[j], *pairs[j + 1]) for j in range(0, len(pairs) - 1, 2)]
            pairs = nxt + pairs[len(nxt) * 2:]
        return pairs[0]

    def keep_load():
        return jnp.concatenate([pltpu.bitcast(keep_v[0], bf16), pltpu.bitcast(keep_v[1], bf16)], axis=1)

    def l2_body(i, state):
        lo = i * T
        lhs = keep_load()
        pqn = pltpu.bitcast(qproj(lo + T, T, zb_v[...]), u32)
        keep_v[0] = pqn[:, :HT]
        keep_v[1] = pqn[:, HT:]
        (k1, k2), _ = post(lo - HT, attn_v[...], HT, 16, state, None)
        state = jnp.where(i > 0, k1, IMIN), jnp.where(i > 0, k2, IMIN)

        @pl.when(i > 0)
        def _():
            out_copy(lo - HT, HT, 2 * i - 1).start()

        m = _get(m_v, 0, D)
        at = _dot_tn(lhs[:, :HT], m)
        attn_v[...] = _dot_tn(lhs[:, HT:], m)
        state, _ = post(lo, at, HT, 32, state, None)
        out_copy(lo, HT, 2 * i).start()
        return state

    mark('L2')
    init = jnp.full((8, G), IMIN, i32)
    state = lax.fori_loop(0, NT - 1, l2_body, (init, init))

    mark('W7')
    wg_copy.wait()
    wu_copy.wait()
    wd_copy.wait()
    mark('T')
    lhs = keep_load()
    m = _get(m_v, 0, D)
    lo = S - T
    at_a = _dot_tn(lhs[:, :256], m)
    at_b = _dot_tn(lhs[:, 256:384], m)
    at_c = _dot_tn(lhs[:, 384:], m)
    state, link = post(lo - HT, attn_v[...], HT, 32, state, None)
    state, link = post(lo, at_a, 256, 32, state, link)
    out_copy(lo - HT, T, 2 * NT - 3).start()
    state, link = post(lo + 256, at_b, 128, 32, state, link)
    k1, k2 = post_last(lo + 384, at_c, 128, state)
    out_copy(lo + HT, HT, 2 * NT - 2).start()

    for sh in (4, 2, 1):
        k1, k2 = merge(k1, k2, pltpu.roll(k1, sh, 0), pltpu.roll(k2, sh, 0))
    k1 = k1[0:1]
    k2 = k2[0:1]

    def unkey(k):
        i = (S - 1) - (k & (S - 1))
        v = k & ~(S - 1)
        v = v ^ ((v >> 31) & 0x7FFFFFFF)
        return i, lax.bitcast_convert_type(v, f32)

    i1v, r1 = unkey(k1)
    i2v, r2 = unkey(k2)
    i1 = i1v[0, 0]
    i2 = i2v[0, 0]
    b1 = pl.multiple_of((i1 // RB) * RB, RB)
    b2 = pl.multiple_of((i2 // RB) * RB, RB)
    rid = lax.broadcasted_iota(i32, (RB, 1), 0)

    rid8 = lax.broadcasted_iota(i32, (8, D), 0)
    xs = jnp.where(rid8 == 0, jnp.broadcast_to(hn_v[pl.ds(i1 + PAD, 1), :], (8, D)),
                   jnp.broadcast_to(hn_v[pl.ds(i2 + PAD, 1), :], (8, D)))
    xsel = jnp.concatenate([xs, xs], axis=0).astype(bf16)

    acts = {}

    def gu(c):
        sl = pl.ds(c * FC, FC)
        gt = _dot(xsel, wg_v[:, sl])
        ut = _dot(xsel, wu_v[:, sl])
        acts[c] = (gt * jax.nn.sigmoid(gt) * ut).astype(bf16)

    y = None
    gu(0)
    for c in range(NF):
        if c + 1 < NF:
            gu(c + 1)
        t = _dot(acts.pop(c), wd_v[pl.ds(c * FC, FC), :])
        y = t if y is None else y + t
    s1 = jnp.concatenate([jax.nn.sigmoid(r1)] * NG, axis=1)
    s2 = jnp.concatenate([jax.nn.sigmoid(r2)] * NG, axis=1)
    y1 = y[0:1, :] * s1
    y2 = y[1:2, :] * s2

    def fixed(b):
        gid = rid + b
        upd = jnp.where(gid == i1, y1, 0.0) + jnp.where(gid == i2, y2, 0.0)
        return (out_v[_rows(b + PAD, RB), :].astype(f32) + upd).astype(bf16)

    fix_v[0] = fixed(b1)
    fix_v[1] = fixed(b2)
    mark('W8')
    for i in range(2 * NT - 3):
        out_copy(i * HT, HT, i).wait()
    out_copy(lo - HT, T, 2 * NT - 3).wait()
    out_copy(lo + HT, HT, 2 * NT - 2).wait()
    mark('E')
    fix1 = pltpu.make_async_copy(fix_v.at[0], out_hbm.at[pl.ds(b1, RB)], sem_f.at[0])
    fix2 = pltpu.make_async_copy(fix_v.at[1], out_hbm.at[pl.ds(b2, RB)], sem_f.at[1])
    fix1.start()

    @pl.when(b1 != b2)
    def _():
        fix2.start()
        fix2.wait()

    fix1.wait()
    mark(None)


@jax.jit
def pallas_sequential_preLN__linear_attn_block__moe_arch_mod__prompt_kernel(
    A_x: jax.Array,
    A_wqkv: jax.Array,
    A_wo: jax.Array,
    B_x: jax.Array,
    B_w_r: jax.Array,
    B_w_gate: jax.Array,
    B_w_up: jax.Array,
    B_w_down: jax.Array,
):
    del B_x
    any_spec = pl.BlockSpec(memory_space=pl.ANY)
    out = pl.pallas_call(
        _kernel,
        out_shape=jax.ShapeDtypeStruct((S, D), bf16),
        in_specs=[any_spec] * 7,
        out_specs=any_spec,
        scratch_shapes=[
            pltpu.VMEM((PAD + S, D), bf16),
            pltpu.VMEM((S // 2, D), u32),
            pltpu.VMEM((PAD + S, D), f32),
            pltpu.VMEM((PAD + S, D), bf16),
            pltpu.VMEM((D, D), bf16),
            pltpu.VMEM((D, D), bf16),
            pltpu.VMEM((2, D, D // 2), bf16),
            pltpu.VMEM((D, D), bf16),
            pltpu.VMEM((D // 2, D), u32),
            pltpu.VMEM((D, D), f32),
            pltpu.VMEM((D // 2, D), u32),
            pltpu.VMEM((D, G), f32),
            pltpu.VMEM((D,), bf16),
            pltpu.VMEM((8, D), f32),
            pltpu.VMEM((2, D // 2, HT), u32),
            pltpu.VMEM((HT, D), f32),
            pltpu.VMEM((4, 8, G), f32),
            pltpu.VMEM((4, 128, G), u32),
            pltpu.VMEM((D, F), bf16),
            pltpu.VMEM((D, F), bf16),
            pltpu.VMEM((F, D), bf16),
            pltpu.VMEM((2, RB, D), bf16),
            pltpu.SemaphoreType.DMA((len(X_PIECES),)),
            pltpu.SemaphoreType.DMA((5,)),
            pltpu.SemaphoreType.DMA((8,)),
            pltpu.SemaphoreType.DMA((2 * NT - 1,)),
            pltpu.SemaphoreType.DMA((2,)),
        ],
        compiler_params=pltpu.CompilerParams(vmem_limit_bytes=100 * 1024 * 1024, disable_bounds_checks=True, disable_semaphore_checks=True),
    )(A_x.reshape(S, D), A_wqkv, A_wo, B_w_r, B_w_gate, B_w_up, B_w_down)
    return out.reshape(1, S, D)
```

```python
import jax
import jax.numpy as jnp
from jax import lax
import jax.experimental.pallas as pl
import jax.experimental.pallas.tpu as pltpu

S = 2048
D = 1024
F = 3584
H = 32
DH = D // H
LN_EPS = 1e-5
PHI_EPS = 1e-6
G = 128
NG = D // G
RB = 16
FC = 256
NF = F // FC
T = 512
NT = S // T
HT = T // 2
PAD = G

f32 = jnp.float32
bf16 = jnp.bfloat16
u32 = jnp.uint32
i32 = jnp.int32
IMIN = jnp.iinfo(jnp.int32).min

X_PIECES = ((0, 256), (256, 256), (512, 512), (1024, 1024))

SCOPES = False


def _zero_of(v):
    u = lax.bitcast_convert_type(v, u32)
    u = lax.shift_right_logical(lax.shift_right_logical(u, jnp.uint32(16)), jnp.uint32(16))
    return lax.bitcast_convert_type(u, f32)


def _phi(t):
    return jnp.where(t > 0, t + 1.0, jnp.exp(t)) + PHI_EPS


def _dot(a, b):
    return jnp.dot(a, b, preferred_element_type=f32)


def _dot_nt(a, b):
    return lax.dot_general(a, b, (((1,), (1,)), ((), ())), preferred_element_type=f32)


def _dot_tn(a, b):
    return lax.dot_general(a, b, (((0,), (0,)), ((), ())), preferred_element_type=f32)


def _half(lo, align):
    return lo // 2 if isinstance(lo, int) else pl.multiple_of(lo // 2, align // 2)


def _put(ref, lo, val, align=16):
    ref[pl.ds(_half(lo, align), val.shape[0] // 2), :] = pltpu.bitcast(val, u32)


def _get(ref, lo, n, align=16):
    return pltpu.bitcast(ref[pl.ds(_half(lo, align), n // 2), :], bf16)


def _rows(lo, n, align=16):
    return pl.ds(lo if isinstance(lo, int) else pl.multiple_of(lo, align), n)


def _kernel(x_hbm, wqkv_hbm, wo_hbm, wr_hbm, wg_hbm, wu_hbm, wd_hbm, out_hbm,
            x_v, xn_v, hn_v, out_v, wk_v, wq_v, wv_v, wo_v, wqt_v, p_v, m_v, zb_v, wr_v, wrf_v,
            keep_v, attn_v, za_v, pka_v, wg_v, wu_v, wd_v, fix_v,
            sem_x, sem_k, sem_w, sem_o, sem_f):
    scope = [None]

    def mark(name):
        if not SCOPES:
            return
        if scope[0] is not None:
            scope[0].__exit__(None, None, None)
        scope[0] = None
        if name:
            scope[0] = jax.named_scope(name)
            scope[0].__enter__()

    def x_copy(i):
        lo, n = X_PIECES[i]
        return pltpu.make_async_copy(x_hbm.at[pl.ds(lo, n)], x_v.at[pl.ds(PAD + lo, n)], sem_x.at[i])

    def wk_copy(i):
        lo = i * G if isinstance(i, int) else pl.multiple_of(i * G, G)
        n = 512 if isinstance(i, int) and i == 4 else G
        return pltpu.make_async_copy(wqkv_hbm.at[:, pl.ds(D + lo, n)], wk_v.at[:, pl.ds(lo, n)], sem_k.at[i])

    def wv_copy(i):
        return pltpu.make_async_copy(wqkv_hbm.at[:, pl.ds(2 * D + i * 512, 512)], wv_v.at[i], sem_w.at[i])

    def out_copy(lo, n, s):
        return pltpu.make_async_copy(out_v.at[_rows(lo + PAD, n)], out_hbm.at[_rows(lo, n)], sem_o.at[s])

    wo_copy = pltpu.make_async_copy(wo_hbm, wo_v, sem_w.at[2])
    wg_copy = pltpu.make_async_copy(wg_hbm, wg_v, sem_w.at[3])
    wu_copy = pltpu.make_async_copy(wu_hbm, wu_v, sem_w.at[4])
    wd_copy = pltpu.make_async_copy(wd_hbm, wd_v, sem_w.at[5])
    wr_copy = pltpu.make_async_copy(wr_hbm, wr_v, sem_w.at[6])
    wq_copy = pltpu.make_async_copy(wqkv_hbm.at[:, pl.ds(0, D)], wq_v, sem_w.at[7])

    x_copy(0).start()

    def start_wk(i, c):
        wk_copy(i).start()
        return c

    lax.fori_loop(0, 4, start_wk, 0)
    x_copy(1).start()

    def zero_pad(i, c):
        rows = pl.ds(pl.multiple_of(i * 32, 32), 32)
        x_v[rows, :] = jnp.zeros((32, D), bf16)
        attn_v[rows, :] = jnp.zeros((32, D), f32)
        return c

    lax.fori_loop(0, PAD // 32, zero_pad, 0)

    def ln_rows(lo, n, sub):
        link = None
        outs = []
        for q in range(0, n, sub):
            x = x_v[_rows(lo + (PAD + q), sub), :].astype(f32)
            mu = jnp.sum(x, axis=-1, keepdims=True) * (1.0 / D)
            if link is not None:
                mu = mu + link
            xc = x - mu
            var = jnp.sum(xc * xc, axis=-1, keepdims=True) * (1.0 / D)
            y = xc * lax.rsqrt(var + LN_EPS)
            link = _zero_of(y[:, D - G:])[:, 0:1]
            yb = y.astype(bf16)
            _put(xn_v, lo + q, yb)
            outs.append(yb)
        return jnp.concatenate(outs, axis=0) if len(outs) > 1 else outs[0]

    def kproj(xn, c0, c1):
        pk = _phi(_dot(xn, wk_v[:, pl.ds(c0, c1 - c0)]))
        zs = jnp.sum(pk.reshape(xn.shape[0] // 8, 8, c1 - c0), axis=0)
        return pk.astype(bf16), zs

    wk_copy(4).start()
    mark('W0')
    x_copy(0).wait()
    mark('R0')
    x_copy(2).start()
    ln_rows(0, 256, 256)
    mark('R12')

    def ka_body(i, c):
        wk_copy(i).wait()
        col = pl.multiple_of(i * G, G)
        pk = _phi(_dot(_get(xn_v, 0, 256), wk_v[:, pl.ds(col, G)]))
        za_v[i] = jnp.sum(pk.reshape(32, 8, G), axis=0)
        pka_v[i] = pltpu.bitcast(pk.astype(bf16), u32)
        return c

    lax.fori_loop(0, 4, ka_body, 0)
    x_copy(3).start()
    wq_copy.start()
    mark('W3')
    x_copy(1).wait()
    mark('R3')
    wv_copy(0).start()
    wv_copy(1).start()
    wo_copy.start()
    wr_copy.start()
    pk_a = jnp.concatenate([pltpu.bitcast(pka_v[i], bf16) for i in range(4)], axis=1)
    p_v[pl.ds(0, 512), :] = _dot_tn(pk_a, _get(xn_v, 0, 256))
    xb = ln_rows(256, 256, 64)
    pk_b, z_b = kproj(xb, 0, 512)
    p_v[pl.ds(0, 512), :] += _dot_tn(pk_b, xb)
    mark('W4')
    wk_copy(4).wait()
    x_copy(2).wait()
    mark('R4')
    wg_copy.start()
    wu_copy.start()
    wd_copy.start()
    x0 = _get(xn_v, 0, T)
    pk_c, z_c = kproj(x0, 512, D)
    p_v[pl.ds(512, 512), :] = _dot_tn(pk_c, x0)
    ln_rows(T, T, 64)
    zacc = jnp.concatenate([jnp.concatenate([za_v[i] for i in range(4)], axis=1) + z_b, z_c], axis=1)
    mark('W5')
    x_copy(3).wait()
    wq_copy.wait()
    mark('L1')

    def l1_body(i, z):
        lo = (i + 1) * T
        xn = _get(xn_v, lo, T, T)
        pk, zs = kproj(xn, 0, D)
        p_v[...] += _dot_tn(pk, xn)
        nxt = jnp.minimum(i + 2, NT - 1) * T
        ln_rows(nxt, T, 32)
        c0 = jnp.minimum(i * 3, NG - 3) * G
        for c in range(3):
            col = pl.multiple_of(c0 + c * G, G)
            _put(wqt_v, col, wq_v[:, pl.ds(col, G)].T, G)
        return z + zs

    zacc = lax.fori_loop(0, NT - 1, l1_body, zacc)

    mark('W6')
    wv_copy(0).wait()
    wv_copy(1).wait()
    wo_copy.wait()
    wr_copy.wait()
    mark('M')

    def qproj(lo, n, zb):
        pqt = _phi(_dot_nt(_get(wqt_v, 0, D), _get(xn_v, lo, n, G)))
        zt = jnp.concatenate([zb] * (n // G), axis=1)
        den = jnp.sum((pqt * zt).reshape(H, DH, n), axis=1, keepdims=True) + PHI_EPS
        return (pqt.reshape(H, DH, n) * (1.0 / den)).reshape(D, n).astype(bf16)

    def ml_body(i, c):
        z = jnp.sum(zacc, axis=0, keepdims=True)
        zb = jnp.broadcast_to(z, (G, D)).T
        zb_v[...] = zb
        wrf_v[...] = jnp.broadcast_to(wr_v[...].reshape(1, D).astype(f32), (8, D))
        ri = lax.broadcasted_iota(i32, (G, G), 0) // DH
        ci = lax.broadcasted_iota(i32, (G, G), 1) // DH
        same_head = ri == ci
        base = i * (D // 2)
        kvs = {}

        def kv(g):
            t = _dot(p_v[_rows(base + g * G, G, G), :].astype(bf16), wv_v[i, :, pl.ds(g * G, G)])
            kvs[g] = jnp.where(same_head, t, 0.0).astype(bf16)

        def mrow(g):
            _put(m_v, base + g * G, _dot(kvs.pop(g), wo_v[_rows(base + g * G, G, G), :]).astype(bf16), G)

        kv(0)
        kv(1)
        mrow(0)
        keep_v[i] = pltpu.bitcast(qproj(i * HT, HT, zb), u32)
        kv(2)
        mrow(1)
        kv(3)
        mrow(2)
        mrow(3)
        return c

    lax.fori_loop(0, 2, ml_body, 0)

    sub_id = lax.broadcasted_iota(i32, (8, G), 0)

    def keys(r, lo, n):
        rb = lax.bitcast_convert_type(jnp.broadcast_to(r, (n, G)), i32)
        u = rb ^ ((rb >> 31) & 0x7FFFFFFF)
        code0 = (S - 1 - lo) - sub_id
        return rb, [(u[s8:s8 + 8] & ~(S - 1)) | (code0 - s8) for s8 in range(0, n, 8)]

    def merge(a1, a2, b1, b2):
        gt = a1 > b1
        lo = jnp.where(gt, b1, a1)
        other = jnp.where(gt, a2, b2)
        return jnp.where(gt, a1, b1), jnp.where(lo > other, lo, other)

    def post(lo, attn, n, sub, state, link):
        k1, k2 = state
        wr = wrf_v[0:1, :]
        for q in range(0, n, sub):
            rows = _rows(lo + (PAD + q), sub)
            h = x_v[rows, :].astype(f32) + attn[q:q + sub]
            mu = jnp.broadcast_to(jnp.sum(h, axis=-1, keepdims=True) * (1.0 / D), (sub, G))
            if link is not None:
                mu = mu + link
            xc = h - jnp.concatenate([mu] * NG, axis=1)
            var = jnp.sum(xc * xc, axis=-1, keepdims=True) * (1.0 / D)
            hn = xc * lax.rsqrt(var + LN_EPS)
            hn_v[rows, :] = hn
            out_v[rows, :] = (h + hn).astype(bf16)
            rb, ks = keys(jnp.sum(hn * wr, axis=-1, keepdims=True), lo + q, sub)
            link = _zero_of(rb | jnp.concatenate([k2] * (sub // 8), axis=0))
            for key in ks:
                gt = key > k1
                lo2 = jnp.where(gt, k1, key)
                k2 = jnp.where(lo2 > k2, lo2, k2)
                k1 = jnp.where(gt, key, k1)
        return (k1, k2), link

    def post_last(lo, attn, n, state):
        rows = pl.ds(lo + PAD, n)
        h = x_v[rows, :].astype(f32) + attn
        xc = h - jnp.sum(h, axis=-1, keepdims=True) * (1.0 / D)
        var = jnp.sum(xc * xc, axis=-1, keepdims=True) * (1.0 / D)
        t = jnp.sum(xc * wrf_v[0:1, :], axis=-1, keepdims=True)
        rstd = lax.rsqrt(var + LN_EPS)
        hn = xc * rstd
        hn_v[rows, :] = hn
        out_v[rows, :] = (h + hn).astype(bf16)
        _, ks = keys(t * rstd, lo, n)
        pairs = []
        for a, b in zip(ks[0::2], ks[1::2]):
            gt = a > b
            pairs.append((jnp.where(gt, a, b), jnp.where(gt, b, a)))
        pairs.append(state)
        while len(pairs) > 1:
            nxt = [merge(*pairs[j], *pairs[j + 1]) for j in range(0, len(pairs) - 1, 2)]
            pairs = nxt + pairs[len(nxt) * 2:]
        return pairs[0]

    def keep_load():
        return jnp.concatenate([pltpu.bitcast(keep_v[0], bf16), pltpu.bitcast(keep_v[1], bf16)], axis=1)

    def l2_body(i, state):
        lo = i * T
        lhs = keep_load()
        pqn = pltpu.bitcast(qproj(lo + T, T, zb_v[...]), u32)
        keep_v[0] = pqn[:, :HT]
        keep_v[1] = pqn[:, HT:]
        (k1, k2), _ = post(lo - G, attn_v[...], G, 16, state, None)
        state = jnp.where(i > 0, k1, IMIN), jnp.where(i > 0, k2, IMIN)

        @pl.when(i > 0)
        def _():
            out_copy(lo - G, G, 2 * i - 1).start()

        m = _get(m_v, 0, D)
        at_a = _dot_tn(lhs[:, :HT], m)
        at_b = _dot_tn(lhs[:, HT:HT + G], m)
        attn_v[...] = _dot_tn(lhs[:, HT + G:], m)
        state, link = post(lo, at_a, HT, 32, state, None)
        state, _ = post(lo + HT, at_b, G, 32, state, link)
        out_copy(lo, T - G, 2 * i).start()
        return state

    mark('L2')
    init = jnp.full((8, G), IMIN, i32)
    state = lax.fori_loop(0, NT - 1, l2_body, (init, init))

    mark('W7')
    wg_copy.wait()
    wu_copy.wait()
    wd_copy.wait()
    mark('T')
    lhs = keep_load()
    m = _get(m_v, 0, D)
    lo = S - T
    ats = [_dot_tn(lhs[:, c:c + G], m) for c in range(0, T, G)]
    state, link = post(lo - G, attn_v[...], G, 16, state, None)
    link = jnp.concatenate([link, link], axis=0)
    for c in range(3):
        state, link = post(lo + c * G, ats[c], G, 32, state, link)
    out_copy(lo - G, T, 2 * NT - 3).start()
    k1, k2 = post_last(S - G, ats[3], G, state)
    out_copy(S - G, G, 2 * NT - 2).start()

    for sh in (4, 2, 1):
        k1, k2 = merge(k1, k2, pltpu.roll(k1, sh, 0), pltpu.roll(k2, sh, 0))
    k1 = k1[0:1]
    k2 = k2[0:1]

    def unkey(k):
        i = (S - 1) - (k & (S - 1))
        v = k & ~(S - 1)
        v = v ^ ((v >> 31) & 0x7FFFFFFF)
        return i, lax.bitcast_convert_type(v, f32)

    i1v, r1 = unkey(k1)
    i2v, r2 = unkey(k2)
    i1 = i1v[0, 0]
    i2 = i2v[0, 0]
    b1 = pl.multiple_of((i1 // RB) * RB, RB)
    b2 = pl.multiple_of((i2 // RB) * RB, RB)
    rid = lax.broadcasted_iota(i32, (RB, 1), 0)

    rid8 = lax.broadcasted_iota(i32, (8, D), 0)
    xs = jnp.where(rid8 == 0, jnp.broadcast_to(hn_v[pl.ds(i1 + PAD, 1), :], (8, D)),
                   jnp.broadcast_to(hn_v[pl.ds(i2 + PAD, 1), :], (8, D)))
    xsel = jnp.concatenate([xs, xs], axis=0).astype(bf16)

    acts = {}

    def gu(c):
        sl = pl.ds(c * FC, FC)
        gt = _dot(xsel, wg_v[:, sl])
        ut = _dot(xsel, wu_v[:, sl])
        acts[c] = (gt * jax.nn.sigmoid(gt) * ut).astype(bf16)

    y = None
    gu(0)
    for c in range(NF):
        if c + 1 < NF:
            gu(c + 1)
        t = _dot(acts.pop(c), wd_v[pl.ds(c * FC, FC), :])
        y = t if y is None else y + t
    s1 = jnp.concatenate([jax.nn.sigmoid(r1)] * NG, axis=1)
    s2 = jnp.concatenate([jax.nn.sigmoid(r2)] * NG, axis=1)
    y1 = y[0:1, :] * s1
    y2 = y[1:2, :] * s2

    def fixed(b):
        gid = rid + b
        upd = jnp.where(gid == i1, y1, 0.0) + jnp.where(gid == i2, y2, 0.0)
        return (out_v[_rows(b + PAD, RB), :].astype(f32) + upd).astype(bf16)

    fix_v[0] = fixed(b1)
    fix_v[1] = fixed(b2)
    mark('W8')
    for i in range(NT - 1):
        if i > 0:
            out_copy(i * T - G, G, 2 * i - 1).wait()
        out_copy(i * T, T - G, 2 * i).wait()
    out_copy(lo - G, T, 2 * NT - 3).wait()
    out_copy(S - G, G, 2 * NT - 2).wait()
    mark('E')
    fix1 = pltpu.make_async_copy(fix_v.at[0], out_hbm.at[pl.ds(b1, RB)], sem_f.at[0])
    fix2 = pltpu.make_async_copy(fix_v.at[1], out_hbm.at[pl.ds(b2, RB)], sem_f.at[1])
    fix1.start()

    @pl.when(b1 != b2)
    def _():
        fix2.start()
        fix2.wait()

    fix1.wait()
    mark(None)


@jax.jit
def pallas_sequential_preLN__linear_attn_block__moe_arch_mod__prompt_kernel(
    A_x: jax.Array,
    A_wqkv: jax.Array,
    A_wo: jax.Array,
    B_x: jax.Array,
    B_w_r: jax.Array,
    B_w_gate: jax.Array,
    B_w_up: jax.Array,
    B_w_down: jax.Array,
):
    del B_x
    any_spec = pl.BlockSpec(memory_space=pl.ANY)
    out = pl.pallas_call(
        _kernel,
        out_shape=jax.ShapeDtypeStruct((S, D), bf16),
        in_specs=[any_spec] * 7,
        out_specs=any_spec,
        scratch_shapes=[
            pltpu.VMEM((PAD + S, D), bf16),
            pltpu.VMEM((S // 2, D), u32),
            pltpu.VMEM((PAD + S, D), f32),
            pltpu.VMEM((PAD + S, D), bf16),
            pltpu.VMEM((D, D), bf16),
            pltpu.VMEM((D, D), bf16),
            pltpu.VMEM((2, D, D // 2), bf16),
            pltpu.VMEM((D, D), bf16),
            pltpu.VMEM((D // 2, D), u32),
            pltpu.VMEM((D, D), f32),
            pltpu.VMEM((D // 2, D), u32),
            pltpu.VMEM((D, G), f32),
            pltpu.VMEM((D,), bf16),
            pltpu.VMEM((8, D), f32),
            pltpu.VMEM((2, D // 2, HT), u32),
            pltpu.VMEM((G, D), f32),
            pltpu.VMEM((4, 8, G), f32),
            pltpu.VMEM((4, 128, G), u32),
            pltpu.VMEM((D, F), bf16),
            pltpu.VMEM((D, F), bf16),
            pltpu.VMEM((F, D), bf16),
            pltpu.VMEM((2, RB, D), bf16),
            pltpu.SemaphoreType.DMA((len(X_PIECES),)),
            pltpu.SemaphoreType.DMA((5,)),
            pltpu.SemaphoreType.DMA((8,)),
            pltpu.SemaphoreType.DMA((2 * NT - 1,)),
            pltpu.SemaphoreType.DMA((2,)),
        ],
        compiler_params=pltpu.CompilerParams(vmem_limit_bytes=100 * 1024 * 1024, disable_bounds_checks=True, disable_semaphore_checks=True),
    )(A_x.reshape(S, D), A_wqkv, A_wo, B_w_r, B_w_gate, B_w_up, B_w_down)
    return out.reshape(1, S, D)
```

```python
import jax
import jax.numpy as jnp
from jax import lax
import jax.experimental.pallas as pl
import jax.experimental.pallas.tpu as pltpu

S = 2048
D = 1024
F = 3584
H = 32
DH = D // H
LN_EPS = 1e-5
PHI_EPS = 1e-6
G = 128
NG = D // G
RB = 16
FC = 256
NF = F // FC
T = 512
NT = S // T
HT = T // 2
PAD = G

f32 = jnp.float32
bf16 = jnp.bfloat16
u32 = jnp.uint32
i32 = jnp.int32
IMIN = jnp.iinfo(jnp.int32).min

WK_PIECES = ((0, 128), (128, 128), (256, 256), (512, 512))
X_PIECES = ((0, 256), (256, 256), (512, 512), (1024, 1024))

SCOPES = False


def _zero_of(v):
    u = lax.bitcast_convert_type(v, u32)
    u = lax.shift_right_logical(lax.shift_right_logical(u, jnp.uint32(16)), jnp.uint32(16))
    return lax.bitcast_convert_type(u, f32)


def _phi(t):
    return jnp.where(t > 0, t + 1.0, jnp.exp(t)) + PHI_EPS


def _dot(a, b):
    return jnp.dot(a, b, preferred_element_type=f32)


def _dot_nt(a, b):
    return lax.dot_general(a, b, (((1,), (1,)), ((), ())), preferred_element_type=f32)


def _dot_tn(a, b):
    return lax.dot_general(a, b, (((0,), (0,)), ((), ())), preferred_element_type=f32)


def _half(lo, align):
    return lo // 2 if isinstance(lo, int) else pl.multiple_of(lo // 2, align // 2)


def _put(ref, lo, val, align=16):
    ref[pl.ds(_half(lo, align), val.shape[0] // 2), :] = pltpu.bitcast(val, u32)


def _get(ref, lo, n, align=16):
    return pltpu.bitcast(ref[pl.ds(_half(lo, align), n // 2), :], bf16)


def _rows(lo, n, align=16):
    return pl.ds(lo if isinstance(lo, int) else pl.multiple_of(lo, align), n)


def _kernel(x_hbm, wqkv_hbm, wo_hbm, wr_hbm, wg_hbm, wu_hbm, wd_hbm, out_hbm,
            x_v, xn_v, hn_v, out_v, wk_v, wq_v, wv_v, wo_v, wqt_v, p_v, m_v, zb_v, wr_v, wrf_v,
            keep_v, attn_v, wg_v, wu_v, wd_v, fix_v,
            sem_x, sem_k, sem_w, sem_o, sem_f):
    scope = [None]

    def mark(name):
        if not SCOPES:
            return
        if scope[0] is not None:
            scope[0].__exit__(None, None, None)
        scope[0] = None
        if name:
            scope[0] = jax.named_scope(name)
            scope[0].__enter__()

    def x_copy(i):
        lo, n = X_PIECES[i]
        return pltpu.make_async_copy(x_hbm.at[pl.ds(lo, n)], x_v.at[pl.ds(PAD + lo, n)], sem_x.at[i])

    def wk_copy(i):
        if isinstance(i, int):
            lo, n = WK_PIECES[i]
        else:
            lo, n = pl.multiple_of(i * G, G), G
        return pltpu.make_async_copy(wqkv_hbm.at[:, pl.ds(D + lo, n)], wk_v.at[:, pl.ds(lo, n)], sem_k.at[i])

    def wv_copy(i):
        return pltpu.make_async_copy(wqkv_hbm.at[:, pl.ds(2 * D + i * 512, 512)], wv_v.at[i], sem_w.at[i])

    def out_copy(lo, n, s):
        return pltpu.make_async_copy(out_v.at[_rows(lo + PAD, n)], out_hbm.at[_rows(lo, n)], sem_o.at[s])

    wo_copy = pltpu.make_async_copy(wo_hbm, wo_v, sem_w.at[2])
    wg_copy = pltpu.make_async_copy(wg_hbm, wg_v, sem_w.at[3])
    wu_copy = pltpu.make_async_copy(wu_hbm, wu_v, sem_w.at[4])
    wd_copy = pltpu.make_async_copy(wd_hbm, wd_v, sem_w.at[5])
    wr_copy = pltpu.make_async_copy(wr_hbm, wr_v, sem_w.at[6])
    wq_copy = pltpu.make_async_copy(wqkv_hbm.at[:, pl.ds(0, D)], wq_v, sem_w.at[7])

    x_copy(0).start()

    def start_wk(i, c):
        wk_copy(i).start()
        return c

    lax.fori_loop(0, 2, start_wk, 0)
    wk_copy(2).start()

    def zero_pad(i, c):
        rows = pl.ds(pl.multiple_of(i * 32, 32), 32)
        x_v[rows, :] = jnp.zeros((32, D), bf16)
        attn_v[rows, :] = jnp.zeros((32, D), f32)
        return c

    lax.fori_loop(0, PAD // 32, zero_pad, 0)

    def ln_rows(lo, n, sub):
        link = None
        outs = []
        for q in range(0, n, sub):
            x = x_v[_rows(lo + (PAD + q), sub), :].astype(f32)
            mu = jnp.sum(x, axis=-1, keepdims=True) * (1.0 / D)
            if link is not None:
                mu = mu + link
            xc = x - mu
            var = jnp.sum(xc * xc, axis=-1, keepdims=True) * (1.0 / D)
            y = xc * lax.rsqrt(var + LN_EPS)
            link = _zero_of(y[:, D - G:])[:, 0:1]
            yb = y.astype(bf16)
            _put(xn_v, lo + q, yb)
            outs.append(yb)
        return jnp.concatenate(outs, axis=0) if len(outs) > 1 else outs[0]

    def kproj(xn, c0, c1):
        pk = _phi(_dot(xn, wk_v[:, pl.ds(c0, c1 - c0)]))
        zs = jnp.sum(pk.reshape(xn.shape[0] // 8, 8, c1 - c0), axis=0)
        return pk.astype(bf16), zs

    x_copy(1).start()
    mark('W0')
    x_copy(0).wait()
    mark('R0')
    wk_copy(3).start()
    ln_rows(0, 256, 256)
    mark('WA')
    wk_copy(0).wait()
    mark('A')
    x_copy(2).start()
    pk0, z0 = kproj(_get(xn_v, 0, 256), 0, 128)
    mark('WB')
    wk_copy(1).wait()
    mark('B')
    x_copy(3).start()
    wq_copy.start()
    pk1, z1 = kproj(_get(xn_v, 0, 256), 128, 256)
    p_v[pl.ds(0, 128), :] = _dot_tn(pk0, _get(xn_v, 0, 256))
    mark('WC')
    wk_copy(2).wait()
    mark('C')
    wv_copy(0).start()
    wv_copy(1).start()
    wo_copy.start()
    wr_copy.start()
    pk2, z2 = kproj(_get(xn_v, 0, 256), 256, 512)
    p_v[pl.ds(128, 128), :] = _dot_tn(pk1, _get(xn_v, 0, 256))
    mark('W3')
    x_copy(1).wait()
    mark('R3')
    p_v[pl.ds(256, 256), :] = _dot_tn(pk2, _get(xn_v, 0, 256))
    xb = ln_rows(256, 256, 128)
    pk_b, z_b = kproj(xb, 0, 512)
    p_v[pl.ds(0, 512), :] += _dot_tn(pk_b, xb)
    mark('W4')
    wk_copy(3).wait()
    x_copy(2).wait()
    mark('R4')
    wg_copy.start()
    wu_copy.start()
    wd_copy.start()
    x0 = _get(xn_v, 0, T)
    pk_c, z_c = kproj(x0, 512, D)
    p_v[pl.ds(512, 512), :] = _dot_tn(pk_c, x0)
    ln_rows(T, T, 64)
    zacc = jnp.concatenate([jnp.concatenate([z0, z1, z2], axis=1) + z_b, z_c], axis=1)
    mark('W5')
    x_copy(3).wait()
    wq_copy.wait()
    mark('L1')

    def l1_body(i, z):
        lo = (i + 1) * T
        xn = _get(xn_v, lo, T, T)
        pk, zs = kproj(xn, 0, D)
        p_v[...] += _dot_tn(pk, xn)
        nxt = jnp.minimum(i + 2, NT - 1) * T
        ln_rows(nxt, T, 32)
        c0 = jnp.minimum(i * 3, NG - 3) * G
        for c in range(3):
            col = pl.multiple_of(c0 + c * G, G)
            _put(wqt_v, col, wq_v[:, pl.ds(col, G)].T, G)
        return z + zs

    zacc = lax.fori_loop(0, NT - 1, l1_body, zacc)

    mark('W6')
    wv_copy(0).wait()
    wv_copy(1).wait()
    wo_copy.wait()
    wr_copy.wait()
    mark('M')

    def qproj(lo, n, zb):
        pqt = _phi(_dot_nt(_get(wqt_v, 0, D), _get(xn_v, lo, n, G)))
        zt = jnp.concatenate([zb] * (n // G), axis=1)
        den = jnp.sum((pqt * zt).reshape(H, DH, n), axis=1, keepdims=True) + PHI_EPS
        inv = pl.reciprocal(den, approx=True)
        inv = inv * (2.0 - den * inv)
        return (pqt.reshape(H, DH, n) * inv).reshape(D, n).astype(bf16)

    def ml_body(i, c):
        z = jnp.sum(zacc, axis=0, keepdims=True)
        zb = jnp.broadcast_to(z, (G, D)).T
        zb_v[...] = zb
        wrf_v[...] = jnp.broadcast_to(wr_v[...].reshape(1, D).astype(f32), (8, D))
        ri = lax.broadcasted_iota(i32, (G, G), 0) // DH
        ci = lax.broadcasted_iota(i32, (G, G), 1) // DH
        same_head = ri == ci
        base = i * (D // 2)
        kvs = {}

        def kv(g):
            t = _dot(p_v[_rows(base + g * G, G, G), :].astype(bf16), wv_v[i, :, pl.ds(g * G, G)])
            kvs[g] = jnp.where(same_head, t, 0.0).astype(bf16)

        def mrow(g):
            _put(m_v, base + g * G, _dot(kvs.pop(g), wo_v[_rows(base + g * G, G, G), :]).astype(bf16), G)

        kv(0)
        kv(1)
        mrow(0)
        keep_v[i] = pltpu.bitcast(qproj(i * HT, HT, zb), u32)
        kv(2)
        mrow(1)
        kv(3)
        mrow(2)
        mrow(3)
        return c

    lax.fori_loop(0, 2, ml_body, 0)

    sub_id = lax.broadcasted_iota(i32, (8, G), 0)

    def keys(r, lo, n):
        rb = lax.bitcast_convert_type(jnp.broadcast_to(r, (n, G)), i32)
        u = rb ^ ((rb >> 31) & 0x7FFFFFFF)
        code0 = (S - 1 - lo) - sub_id
        return rb, [(u[s8:s8 + 8] & ~(S - 1)) | (code0 - s8) for s8 in range(0, n, 8)]

    def merge(a1, a2, b1, b2):
        gt = a1 > b1
        lo = jnp.where(gt, b1, a1)
        other = jnp.where(gt, a2, b2)
        return jnp.where(gt, a1, b1), jnp.where(lo > other, lo, other)

    def post(lo, attn, n, sub, state, link):
        k1, k2 = state
        wr = wrf_v[0:1, :]
        for q in range(0, n, sub):
            rows = _rows(lo + (PAD + q), sub)
            h = x_v[rows, :].astype(f32) + attn[q:q + sub]
            mu = jnp.broadcast_to(jnp.sum(h, axis=-1, keepdims=True) * (1.0 / D), (sub, G))
            if link is not None:
                mu = mu + link
            xc = h - jnp.concatenate([mu] * NG, axis=1)
            var = jnp.sum(xc * xc, axis=-1, keepdims=True) * (1.0 / D)
            hn = xc * lax.rsqrt(var + LN_EPS)
            hn_v[rows, :] = hn
            out_v[rows, :] = (h + hn).astype(bf16)
            rb, ks = keys(jnp.sum(hn * wr, axis=-1, keepdims=True), lo + q, sub)
            link = _zero_of(rb | jnp.concatenate([k2] * (sub // 8), axis=0))
            for key in ks:
                gt = key > k1
                lo2 = jnp.where(gt, k1, key)
                k2 = jnp.where(lo2 > k2, lo2, k2)
                k1 = jnp.where(gt, key, k1)
        return (k1, k2), link

    def post_last(lo, attn, n, state):
        rows = pl.ds(lo + PAD, n)
        h = x_v[rows, :].astype(f32) + attn
        xc = h - jnp.sum(h, axis=-1, keepdims=True) * (1.0 / D)
        var = jnp.sum(xc * xc, axis=-1, keepdims=True) * (1.0 / D)
        t = jnp.sum(xc * wrf_v[0:1, :], axis=-1, keepdims=True)
        rstd = lax.rsqrt(var + LN_EPS)
        hn = xc * rstd
        hn_v[rows, :] = hn
        out_v[rows, :] = (h + hn).astype(bf16)
        _, ks = keys(t * rstd, lo, n)
        pairs = []
        for a, b in zip(ks[0::2], ks[1::2]):
            gt = a > b
            pairs.append((jnp.where(gt, a, b), jnp.where(gt, b, a)))
        pairs.append(state)
        while len(pairs) > 1:
            nxt = [merge(*pairs[j], *pairs[j + 1]) for j in range(0, len(pairs) - 1, 2)]
            pairs = nxt + pairs[len(nxt) * 2:]
        return pairs[0]

    def keep_load():
        return jnp.concatenate([pltpu.bitcast(keep_v[0], bf16), pltpu.bitcast(keep_v[1], bf16)], axis=1)

    def l2_body(i, state):
        lo = i * T
        lhs = keep_load()
        pqn = pltpu.bitcast(qproj(lo + T, T, zb_v[...]), u32)
        keep_v[0] = pqn[:, :HT]
        keep_v[1] = pqn[:, HT:]
        (k1, k2), _ = post(lo - G, attn_v[...], G, 16, state, None)
        state = jnp.where(i > 0, k1, IMIN), jnp.where(i > 0, k2, IMIN)

        @pl.when(i > 0)
        def _():
            out_copy(lo - G, G, 2 * i - 1).start()

        m = _get(m_v, 0, D)
        at_a = _dot_tn(lhs[:, :HT], m)
        at_b = _dot_tn(lhs[:, HT:HT + G], m)
        attn_v[...] = _dot_tn(lhs[:, HT + G:], m)
        state, link = post(lo, at_a, HT, 32, state, None)
        state, _ = post(lo + HT, at_b, G, 32, state, link)
        out_copy(lo, T - G, 2 * i).start()
        return state

    mark('L2')
    init = jnp.full((8, G), IMIN, i32)
    state = lax.fori_loop(0, NT - 1, l2_body, (init, init))

    mark('W7')
    wg_copy.wait()
    wu_copy.wait()
    wd_copy.wait()
    mark('T')
    lhs = keep_load()
    m = _get(m_v, 0, D)
    lo = S - T
    ats = [_dot_tn(lhs[:, c:c + G], m) for c in range(0, T, G)]
    state, link = post(lo - G, attn_v[...], G, 16, state, None)
    link = jnp.concatenate([link, link], axis=0)
    for c in range(3):
        state, link = post(lo + c * G, ats[c], G, 32, state, link)
    out_copy(lo - G, T, 2 * NT - 3).start()
    k1, k2 = post_last(S - G, ats[3], G, state)
    out_copy(S - G, G, 2 * NT - 2).start()

    for sh in (4, 2, 1):
        k1, k2 = merge(k1, k2, pltpu.roll(k1, sh, 0), pltpu.roll(k2, sh, 0))
    k1 = k1[0:1]
    k2 = k2[0:1]

    def unkey(k):
        i = (S - 1) - (k & (S - 1))
        v = k & ~(S - 1)
        v = v ^ ((v >> 31) & 0x7FFFFFFF)
        return i, lax.bitcast_convert_type(v, f32)

    i1v, r1 = unkey(k1)
    i2v, r2 = unkey(k2)
    i1 = i1v[0, 0]
    i2 = i2v[0, 0]
    b1 = pl.multiple_of((i1 // RB) * RB, RB)
    b2 = pl.multiple_of((i2 // RB) * RB, RB)
    rid = lax.broadcasted_iota(i32, (RB, 1), 0)

    rid8 = lax.broadcasted_iota(i32, (8, D), 0)
    xs = jnp.where(rid8 == 0, jnp.broadcast_to(hn_v[pl.ds(i1 + PAD, 1), :], (8, D)),
                   jnp.broadcast_to(hn_v[pl.ds(i2 + PAD, 1), :], (8, D)))
    xsel = jnp.concatenate([xs, xs], axis=0).astype(bf16)

    acts = {}

    def gu(c):
        sl = pl.ds(c * FC, FC)
        gt = _dot(xsel, wg_v[:, sl])
        ut = _dot(xsel, wu_v[:, sl])
        acts[c] = (gt * jax.nn.sigmoid(gt) * ut).astype(bf16)

    y = None
    gu(0)
    for c in range(NF):
        if c + 1 < NF:
            gu(c + 1)
        t = _dot(acts.pop(c), wd_v[pl.ds(c * FC, FC), :])
        y = t if y is None else y + t
    s1 = jnp.concatenate([jax.nn.sigmoid(r1)] * NG, axis=1)
    s2 = jnp.concatenate([jax.nn.sigmoid(r2)] * NG, axis=1)
    y1 = y[0:1, :] * s1
    y2 = y[1:2, :] * s2

    def fixed(b):
        gid = rid + b
        upd = jnp.where(gid == i1, y1, 0.0) + jnp.where(gid == i2, y2, 0.0)
        return (out_v[_rows(b + PAD, RB), :].astype(f32) + upd).astype(bf16)

    fix_v[0] = fixed(b1)
    fix_v[1] = fixed(b2)
    mark('W8')
    for i in range(NT - 1):
        if i > 0:
            out_copy(i * T - G, G, 2 * i - 1).wait()
        out_copy(i * T, T - G, 2 * i).wait()
    out_copy(lo - G, T, 2 * NT - 3).wait()
    out_copy(S - G, G, 2 * NT - 2).wait()
    mark('E')
    fix1 = pltpu.make_async_copy(fix_v.at[0], out_hbm.at[pl.ds(b1, RB)], sem_f.at[0])
    fix2 = pltpu.make_async_copy(fix_v.at[1], out_hbm.at[pl.ds(b2, RB)], sem_f.at[1])
    fix1.start()

    @pl.when(b1 != b2)
    def _():
        fix2.start()
        fix2.wait()

    fix1.wait()
    mark(None)


@jax.jit
def pallas_sequential_preLN__linear_attn_block__moe_arch_mod__prompt_kernel(
    A_x: jax.Array,
    A_wqkv: jax.Array,
    A_wo: jax.Array,
    B_x: jax.Array,
    B_w_r: jax.Array,
    B_w_gate: jax.Array,
    B_w_up: jax.Array,
    B_w_down: jax.Array,
):
    del B_x
    any_spec = pl.BlockSpec(memory_space=pl.ANY)
    out = pl.pallas_call(
        _kernel,
        out_shape=jax.ShapeDtypeStruct((S, D), bf16),
        in_specs=[any_spec] * 7,
        out_specs=any_spec,
        scratch_shapes=[
            pltpu.VMEM((PAD + S, D), bf16),
            pltpu.VMEM((S // 2, D), u32),
            pltpu.VMEM((PAD + S, D), f32),
            pltpu.VMEM((PAD + S, D), bf16),
            pltpu.VMEM((D, D), bf16),
            pltpu.VMEM((D, D), bf16),
            pltpu.VMEM((2, D, D // 2), bf16),
            pltpu.VMEM((D, D), bf16),
            pltpu.VMEM((D // 2, D), u32),
            pltpu.VMEM((D, D), f32),
            pltpu.VMEM((D // 2, D), u32),
            pltpu.VMEM((D, G), f32),
            pltpu.VMEM((D,), bf16),
            pltpu.VMEM((8, D), f32),
            pltpu.VMEM((2, D // 2, HT), u32),
            pltpu.VMEM((G, D), f32),
            pltpu.VMEM((D, F), bf16),
            pltpu.VMEM((D, F), bf16),
            pltpu.VMEM((F, D), bf16),
            pltpu.VMEM((2, RB, D), bf16),
            pltpu.SemaphoreType.DMA((len(X_PIECES),)),
            pltpu.SemaphoreType.DMA((4,)),
            pltpu.SemaphoreType.DMA((8,)),
            pltpu.SemaphoreType.DMA((2 * NT - 1,)),
            pltpu.SemaphoreType.DMA((2,)),
        ],
        compiler_params=pltpu.CompilerParams(vmem_limit_bytes=100 * 1024 * 1024, disable_bounds_checks=True, disable_semaphore_checks=True),
    )(A_x.reshape(S, D), A_wqkv, A_wo, B_w_r, B_w_gate, B_w_up, B_w_down)
    return out.reshape(1, S, D)
```

```python
import jax
import jax.numpy as jnp
from jax import lax
import jax.experimental.pallas as pl
import jax.experimental.pallas.tpu as pltpu

S = 2048
D = 1024
F = 3584
H = 32
DH = D // H
LN_EPS = 1e-5
PHI_EPS = 1e-6
G = 128
NG = D // G
RB = 16
FC = 256
NF = F // FC
T = 512
NT = S // T
HT = T // 2
PAD = G

f32 = jnp.float32
bf16 = jnp.bfloat16
u32 = jnp.uint32
i32 = jnp.int32
IMIN = jnp.iinfo(jnp.int32).min

WK_PIECES = ((0, 128), (128, 128), (256, 256), (512, 512))
X_PIECES = ((0, 256), (256, 256), (512, 512), (1024, 1024))


def _zero_of(v):
    u = lax.bitcast_convert_type(v, u32)
    u = lax.shift_right_logical(lax.shift_right_logical(u, jnp.uint32(16)), jnp.uint32(16))
    return lax.bitcast_convert_type(u, f32)


def _phi(t):
    return jnp.where(t > 0, t + 1.0, jnp.exp(t)) + PHI_EPS


def _dot(a, b):
    return jnp.dot(a, b, preferred_element_type=f32)


def _dot_nt(a, b):
    return lax.dot_general(a, b, (((1,), (1,)), ((), ())), preferred_element_type=f32)


def _dot_tn(a, b):
    return lax.dot_general(a, b, (((0,), (0,)), ((), ())), preferred_element_type=f32)


def _half(lo, align):
    return lo // 2 if isinstance(lo, int) else pl.multiple_of(lo // 2, align // 2)


def _put(ref, lo, val, align=16):
    ref[pl.ds(_half(lo, align), val.shape[0] // 2), :] = pltpu.bitcast(val, u32)


def _get(ref, lo, n, align=16):
    return pltpu.bitcast(ref[pl.ds(_half(lo, align), n // 2), :], bf16)


def _rows(lo, n, align=16):
    return pl.ds(lo if isinstance(lo, int) else pl.multiple_of(lo, align), n)


def _kernel(x_hbm, wqkv_hbm, wo_hbm, wr_hbm, wg_hbm, wu_hbm, wd_hbm, out_hbm,
            x_v, xn_v, hn_v, out_v, wk_v, wq_v, wv_v, wo_v, wqt_v, p_v, m_v, zb_v, wr_v, wrf_v,
            keep_v, attn_v, wg_v, wu_v, wd_v, fix_v,
            sem_x, sem_k, sem_w, sem_o, sem_f):
    def x_copy(i):
        lo, n = X_PIECES[i]
        return pltpu.make_async_copy(x_hbm.at[pl.ds(lo, n)], x_v.at[pl.ds(PAD + lo, n)], sem_x.at[i])

    def wk_copy(i):
        if isinstance(i, int):
            lo, n = WK_PIECES[i]
        else:
            lo, n = pl.multiple_of(i * G, G), G
        return pltpu.make_async_copy(wqkv_hbm.at[:, pl.ds(D + lo, n)], wk_v.at[:, pl.ds(lo, n)], sem_k.at[i])

    def wv_copy(i):
        return pltpu.make_async_copy(wqkv_hbm.at[:, pl.ds(2 * D + i * 512, 512)], wv_v.at[i], sem_w.at[i])

    def out_copy(lo, n, s):
        return pltpu.make_async_copy(out_v.at[_rows(lo + PAD, n)], out_hbm.at[_rows(lo, n)], sem_o.at[s])

    wo_copy = pltpu.make_async_copy(wo_hbm, wo_v, sem_w.at[2])
    wg_copy = pltpu.make_async_copy(wg_hbm, wg_v, sem_w.at[3])
    wu_copy = pltpu.make_async_copy(wu_hbm, wu_v, sem_w.at[4])
    wd_copy = pltpu.make_async_copy(wd_hbm, wd_v, sem_w.at[5])
    wr_copy = pltpu.make_async_copy(wr_hbm, wr_v, sem_w.at[6])
    wq_copy = pltpu.make_async_copy(wqkv_hbm.at[:, pl.ds(0, D)], wq_v, sem_w.at[7])

    x_copy(0).start()

    def start_wk(i, c):
        wk_copy(i).start()
        return c

    lax.fori_loop(0, 2, start_wk, 0)
    wk_copy(2).start()

    def zero_pad(i, c):
        rows = pl.ds(pl.multiple_of(i * 32, 32), 32)
        x_v[rows, :] = jnp.zeros((32, D), bf16)
        attn_v[rows, :] = jnp.zeros((32, D), f32)
        return c

    lax.fori_loop(0, PAD // 32, zero_pad, 0)

    def ln_rows(lo, n, sub):
        link = None
        outs = []
        for q in range(0, n, sub):
            x = x_v[_rows(lo + (PAD + q), sub), :].astype(f32)
            mu = jnp.sum(x, axis=-1, keepdims=True) * (1.0 / D)
            if link is not None:
                mu = mu + link
            xc = x - mu
            var = jnp.sum(xc * xc, axis=-1, keepdims=True) * (1.0 / D)
            y = xc * lax.rsqrt(var + LN_EPS)
            link = _zero_of(y[:, D - G:])[:, 0:1]
            yb = y.astype(bf16)
            _put(xn_v, lo + q, yb)
            outs.append(yb)
        return jnp.concatenate(outs, axis=0) if len(outs) > 1 else outs[0]

    def kproj(xn, c0, c1):
        pk = _phi(_dot(xn, wk_v[:, pl.ds(c0, c1 - c0)]))
        zs = jnp.sum(pk.reshape(xn.shape[0] // 8, 8, c1 - c0), axis=0)
        return pk.astype(bf16), zs

    x_copy(1).start()
    x_copy(0).wait()
    wk_copy(3).start()
    ln_rows(0, 256, 256)
    wk_copy(0).wait()
    x_copy(2).start()
    pk0, z0 = kproj(_get(xn_v, 0, 256), 0, 128)
    wk_copy(1).wait()
    x_copy(3).start()
    wq_copy.start()
    pk1, z1 = kproj(_get(xn_v, 0, 256), 128, 256)
    p_v[pl.ds(0, 128), :] = _dot_tn(pk0, _get(xn_v, 0, 256))
    wk_copy(2).wait()
    wv_copy(0).start()
    wv_copy(1).start()
    wo_copy.start()
    wr_copy.start()
    pk2, z2 = kproj(_get(xn_v, 0, 256), 256, 512)
    p_v[pl.ds(128, 128), :] = _dot_tn(pk1, _get(xn_v, 0, 256))
    x_copy(1).wait()
    p_v[pl.ds(256, 256), :] = _dot_tn(pk2, _get(xn_v, 0, 256))
    xb = ln_rows(256, 256, 128)
    pk_b, z_b = kproj(xb, 0, 512)
    p_v[pl.ds(0, 512), :] += _dot_tn(pk_b, xb)
    wk_copy(3).wait()
    x_copy(2).wait()
    wg_copy.start()
    wu_copy.start()
    wd_copy.start()
    x0 = _get(xn_v, 0, T)
    pk_c, z_c = kproj(x0, 512, D)
    p_v[pl.ds(512, 512), :] = _dot_tn(pk_c, x0)
    ln_rows(T, T, 64)
    zacc = jnp.concatenate([jnp.concatenate([z0, z1, z2], axis=1) + z_b, z_c], axis=1)
    x_copy(3).wait()
    wq_copy.wait()

    def l1_body(i, z):
        lo = (i + 1) * T
        xn = _get(xn_v, lo, T, T)
        pk, zs = kproj(xn, 0, D)
        p_v[...] += _dot_tn(pk, xn)
        nxt = jnp.minimum(i + 2, NT - 1) * T
        ln_rows(nxt, T, 32)
        c0 = jnp.minimum(i * 3, NG - 3) * G
        for c in range(3):
            col = pl.multiple_of(c0 + c * G, G)
            _put(wqt_v, col, wq_v[:, pl.ds(col, G)].T, G)
        return z + zs

    zacc = lax.fori_loop(0, NT - 1, l1_body, zacc)

    wv_copy(0).wait()
    wv_copy(1).wait()
    wo_copy.wait()
    wr_copy.wait()

    def qproj(lo, n, zb):
        pqt = _phi(_dot_nt(_get(wqt_v, 0, D), _get(xn_v, lo, n, G)))
        zt = jnp.concatenate([zb] * (n // G), axis=1)
        den = jnp.sum((pqt * zt).reshape(H, DH, n), axis=1, keepdims=True) + PHI_EPS
        inv = pl.reciprocal(den, approx=True)
        inv = inv * (2.0 - den * inv)
        return (pqt.reshape(H, DH, n) * inv).reshape(D, n).astype(bf16)

    def ml_body(i, c):
        z = jnp.sum(zacc, axis=0, keepdims=True)
        zb = jnp.broadcast_to(z, (G, D)).T
        zb_v[...] = zb
        wrf_v[...] = jnp.broadcast_to(wr_v[...].reshape(1, D).astype(f32), (8, D))
        ri = lax.broadcasted_iota(i32, (G, G), 0) // DH
        ci = lax.broadcasted_iota(i32, (G, G), 1) // DH
        same_head = ri == ci
        base = i * (D // 2)
        kvs = {}

        def kv(g):
            t = _dot(p_v[_rows(base + g * G, G, G), :].astype(bf16), wv_v[i, :, pl.ds(g * G, G)])
            kvs[g] = jnp.where(same_head, t, 0.0).astype(bf16)

        def mrow(g):
            _put(m_v, base + g * G, _dot(kvs.pop(g), wo_v[_rows(base + g * G, G, G), :]).astype(bf16), G)

        kv(0)
        kv(1)
        mrow(0)
        keep_v[i] = pltpu.bitcast(qproj(i * HT, HT, zb), u32)
        kv(2)
        mrow(1)
        kv(3)
        mrow(2)
        mrow(3)
        return c

    lax.fori_loop(0, 2, ml_body, 0)

    sub_id = lax.broadcasted_iota(i32, (8, G), 0)

    def keys(r, lo, n):
        rb = lax.bitcast_convert_type(jnp.broadcast_to(r, (n, G)), i32)
        u = rb ^ ((rb >> 31) & 0x7FFFFFFF)
        code0 = (S - 1 - lo) - sub_id
        return rb, [(u[s8:s8 + 8] & ~(S - 1)) | (code0 - s8) for s8 in range(0, n, 8)]

    def merge(a1, a2, b1, b2):
        gt = a1 > b1
        lo = jnp.where(gt, b1, a1)
        other = jnp.where(gt, a2, b2)
        return jnp.where(gt, a1, b1), jnp.where(lo > other, lo, other)

    def post(lo, attn, n, sub, state, link):
        k1, k2 = state
        wr = wrf_v[0:1, :]
        for q in range(0, n, sub):
            rows = _rows(lo + (PAD + q), sub)
            h = x_v[rows, :].astype(f32) + attn[q:q + sub]
            mu = jnp.broadcast_to(jnp.sum(h, axis=-1, keepdims=True) * (1.0 / D), (sub, G))
            if link is not None:
                mu = mu + link
            xc = h - jnp.concatenate([mu] * NG, axis=1)
            var = jnp.sum(xc * xc, axis=-1, keepdims=True) * (1.0 / D)
            hn = xc * lax.rsqrt(var + LN_EPS)
            hn_v[rows, :] = hn
            out_v[rows, :] = (h + hn).astype(bf16)
            rb, ks = keys(jnp.sum(hn * wr, axis=-1, keepdims=True), lo + q, sub)
            link = _zero_of(rb | jnp.concatenate([k2] * (sub // 8), axis=0))
            for key in ks:
                gt = key > k1
                lo2 = jnp.where(gt, k1, key)
                k2 = jnp.where(lo2 > k2, lo2, k2)
                k1 = jnp.where(gt, key, k1)
        return (k1, k2), link

    def post_last(lo, attn, n, state):
        rows = pl.ds(lo + PAD, n)
        h = x_v[rows, :].astype(f32) + attn
        xc = h - jnp.sum(h, axis=-1, keepdims=True) * (1.0 / D)
        var = jnp.sum(xc * xc, axis=-1, keepdims=True) * (1.0 / D)
        t = jnp.sum(xc * wrf_v[0:1, :], axis=-1, keepdims=True)
        rstd = lax.rsqrt(var + LN_EPS)
        hn = xc * rstd
        hn_v[rows, :] = hn
        out_v[rows, :] = (h + hn).astype(bf16)
        _, ks = keys(t * rstd, lo, n)
        pairs = []
        for a, b in zip(ks[0::2], ks[1::2]):
            gt = a > b
            pairs.append((jnp.where(gt, a, b), jnp.where(gt, b, a)))
        pairs.append(state)
        while len(pairs) > 1:
            nxt = [merge(*pairs[j], *pairs[j + 1]) for j in range(0, len(pairs) - 1, 2)]
            pairs = nxt + pairs[len(nxt) * 2:]
        return pairs[0]

    def keep_load():
        return jnp.concatenate([pltpu.bitcast(keep_v[0], bf16), pltpu.bitcast(keep_v[1], bf16)], axis=1)

    def l2_body(i, state):
        lo = i * T
        lhs = keep_load()
        pqn = pltpu.bitcast(qproj(lo + T, T, zb_v[...]), u32)
        keep_v[0] = pqn[:, :HT]
        keep_v[1] = pqn[:, HT:]
        (k1, k2), _ = post(lo - G, attn_v[...], G, 16, state, None)
        state = jnp.where(i > 0, k1, IMIN), jnp.where(i > 0, k2, IMIN)

        @pl.when(i > 0)
        def _():
            out_copy(lo - G, G, 2 * i - 1).start()

        m = _get(m_v, 0, D)
        at_a = _dot_tn(lhs[:, :HT], m)
        at_b = _dot_tn(lhs[:, HT:HT + G], m)
        attn_v[...] = _dot_tn(lhs[:, HT + G:], m)
        state, link = post(lo, at_a, HT, 32, state, None)
        state, _ = post(lo + HT, at_b, G, 32, state, link)
        out_copy(lo, T - G, 2 * i).start()
        return state

    init = jnp.full((8, G), IMIN, i32)
    state = lax.fori_loop(0, NT - 1, l2_body, (init, init))

    wg_copy.wait()
    wu_copy.wait()
    wd_copy.wait()
    lhs = keep_load()
    m = _get(m_v, 0, D)
    lo = S - T
    ats = [_dot_tn(lhs[:, c:c + G], m) for c in range(0, T, G)]
    state, link = post(lo - G, attn_v[...], G, 16, state, None)
    link = jnp.concatenate([link, link], axis=0)
    for c in range(3):
        state, link = post(lo + c * G, ats[c], G, 32, state, link)
    out_copy(lo - G, T, 2 * NT - 3).start()
    k1, k2 = post_last(S - G, ats[3], G, state)
    out_copy(S - G, G, 2 * NT - 2).start()

    for sh in (4, 2, 1):
        k1, k2 = merge(k1, k2, pltpu.roll(k1, sh, 0), pltpu.roll(k2, sh, 0))
    k1 = k1[0:1]
    k2 = k2[0:1]

    def unkey(k):
        i = (S - 1) - (k & (S - 1))
        v = k & ~(S - 1)
        v = v ^ ((v >> 31) & 0x7FFFFFFF)
        return i, lax.bitcast_convert_type(v, f32)

    i1v, r1 = unkey(k1)
    i2v, r2 = unkey(k2)
    i1 = i1v[0, 0]
    i2 = i2v[0, 0]
    b1 = pl.multiple_of((i1 // RB) * RB, RB)
    b2 = pl.multiple_of((i2 // RB) * RB, RB)
    rid = lax.broadcasted_iota(i32, (RB, 1), 0)

    rid8 = lax.broadcasted_iota(i32, (8, D), 0)
    xs = jnp.where(rid8 == 0, jnp.broadcast_to(hn_v[pl.ds(i1 + PAD, 1), :], (8, D)),
                   jnp.broadcast_to(hn_v[pl.ds(i2 + PAD, 1), :], (8, D)))
    xsel = jnp.concatenate([xs, xs], axis=0).astype(bf16)

    acts = {}

    def gu(c):
        sl = pl.ds(c * FC, FC)
        gt = _dot(xsel, wg_v[:, sl])
        ut = _dot(xsel, wu_v[:, sl])
        acts[c] = (gt * jax.nn.sigmoid(gt) * ut).astype(bf16)

    y = None
    gu(0)
    for c in range(NF):
        if c + 1 < NF:
            gu(c + 1)
        t = _dot(acts.pop(c), wd_v[pl.ds(c * FC, FC), :])
        y = t if y is None else y + t
    s1 = jnp.concatenate([jax.nn.sigmoid(r1)] * NG, axis=1)
    s2 = jnp.concatenate([jax.nn.sigmoid(r2)] * NG, axis=1)
    y1 = y[0:1, :] * s1
    y2 = y[1:2, :] * s2

    def fixed(b):
        gid = rid + b
        upd = jnp.where(gid == i1, y1, 0.0) + jnp.where(gid == i2, y2, 0.0)
        return (out_v[_rows(b + PAD, RB), :].astype(f32) + upd).astype(bf16)

    fix_v[0] = fixed(b1)
    fix_v[1] = fixed(b2)
    for i in range(NT - 1):
        if i > 0:
            out_copy(i * T - G, G, 2 * i - 1).wait()
        out_copy(i * T, T - G, 2 * i).wait()
    out_copy(lo - G, T, 2 * NT - 3).wait()
    out_copy(S - G, G, 2 * NT - 2).wait()
    fix1 = pltpu.make_async_copy(fix_v.at[0], out_hbm.at[pl.ds(b1, RB)], sem_f.at[0])
    fix2 = pltpu.make_async_copy(fix_v.at[1], out_hbm.at[pl.ds(b2, RB)], sem_f.at[1])
    fix1.start()

    @pl.when(b1 != b2)
    def _():
        fix2.start()
        fix2.wait()

    fix1.wait()


@jax.jit
def pallas_sequential_preLN__linear_attn_block__moe_arch_mod__prompt_kernel(
    A_x: jax.Array,
    A_wqkv: jax.Array,
    A_wo: jax.Array,
    B_x: jax.Array,
    B_w_r: jax.Array,
    B_w_gate: jax.Array,
    B_w_up: jax.Array,
    B_w_down: jax.Array,
):
    del B_x
    any_spec = pl.BlockSpec(memory_space=pl.ANY)
    out = pl.pallas_call(
        _kernel,
        out_shape=jax.ShapeDtypeStruct((S, D), bf16),
        in_specs=[any_spec] * 7,
        out_specs=any_spec,
        scratch_shapes=[
            pltpu.VMEM((PAD + S, D), bf16),
            pltpu.VMEM((S // 2, D), u32),
            pltpu.VMEM((PAD + S, D), f32),
            pltpu.VMEM((PAD + S, D), bf16),
            pltpu.VMEM((D, D), bf16),
            pltpu.VMEM((D, D), bf16),
            pltpu.VMEM((2, D, D // 2), bf16),
            pltpu.VMEM((D, D), bf16),
            pltpu.VMEM((D // 2, D), u32),
            pltpu.VMEM((D, D), f32),
            pltpu.VMEM((D // 2, D), u32),
            pltpu.VMEM((D, G), f32),
            pltpu.VMEM((D,), bf16),
            pltpu.VMEM((8, D), f32),
            pltpu.VMEM((2, D // 2, HT), u32),
            pltpu.VMEM((G, D), f32),
            pltpu.VMEM((D, F), bf16),
            pltpu.VMEM((D, F), bf16),
            pltpu.VMEM((F, D), bf16),
            pltpu.VMEM((2, RB, D), bf16),
            pltpu.SemaphoreType.DMA((len(X_PIECES),)),
            pltpu.SemaphoreType.DMA((4,)),
            pltpu.SemaphoreType.DMA((8,)),
            pltpu.SemaphoreType.DMA((2 * NT - 1,)),
            pltpu.SemaphoreType.DMA((2,)),
        ],
        compiler_params=pltpu.CompilerParams(vmem_limit_bytes=100 * 1024 * 1024, disable_bounds_checks=True, disable_semaphore_checks=True),
    )(A_x.reshape(S, D), A_wqkv, A_wo, B_w_r, B_w_gate, B_w_up, B_w_down)
    return out.reshape(1, S, D)
```

```python
import jax
import jax.numpy as jnp
from jax import lax
import jax.experimental.pallas as pl
import jax.experimental.pallas.tpu as pltpu

S = 2048
D = 1024
F = 3584
H = 32
DH = D // H
LN_EPS = 1e-5
PHI_EPS = 1e-6
G = 128
NG = D // G
RB = 16
FC = 256
NF = F // FC
T = 512
NT = S // T
HT = T // 2
PAD = G

f32 = jnp.float32
bf16 = jnp.bfloat16
u32 = jnp.uint32
i32 = jnp.int32
IMIN = jnp.iinfo(jnp.int32).min

WK_PIECES = ((0, 128), (128, 128), (256, 256), (512, 512))
X_PIECES = ((0, 256), (256, 256), (512, 512), (1024, 1024))


def _zero_of(v):
    u = lax.bitcast_convert_type(v, u32)
    u = lax.shift_right_logical(lax.shift_right_logical(u, jnp.uint32(16)), jnp.uint32(16))
    return lax.bitcast_convert_type(u, f32)


def _phi(t):
    return jnp.where(t > 0, t + 1.0, jnp.exp(t)) + PHI_EPS


def _dot(a, b):
    return jnp.dot(a, b, preferred_element_type=f32)


def _dot_nt(a, b):
    return lax.dot_general(a, b, (((1,), (1,)), ((), ())), preferred_element_type=f32)


def _dot_tn(a, b):
    return lax.dot_general(a, b, (((0,), (0,)), ((), ())), preferred_element_type=f32)


def _half(lo, align):
    return lo // 2 if isinstance(lo, int) else pl.multiple_of(lo // 2, align // 2)


def _put(ref, lo, val, align=16):
    ref[pl.ds(_half(lo, align), val.shape[0] // 2), :] = pltpu.bitcast(val, u32)


def _get(ref, lo, n, align=16):
    return pltpu.bitcast(ref[pl.ds(_half(lo, align), n // 2), :], bf16)


def _rows(lo, n, align=16):
    return pl.ds(lo if isinstance(lo, int) else pl.multiple_of(lo, align), n)


def _kernel(x_hbm, wqkv_hbm, wo_hbm, wr_hbm, wg_hbm, wu_hbm, wd_hbm, out_hbm,
            x_v, xn_v, hn_v, out_v, wk_v, wq_v, wv_v, wo_v, wqt_v, p_v, m_v, zb_v, wr_v, wrf_v,
            keep_v, attn_v, wg_v, wu_v, wd_v, fix_v,
            sem_x, sem_k, sem_w, sem_o, sem_f):
    xn_v, wqt_v, m_v, wd_v = (r.at[:, pl.ds(0, D)] for r in (xn_v, wqt_v, m_v, wd_v))

    def x_copy(i):
        lo, n = X_PIECES[i]
        return pltpu.make_async_copy(x_hbm.at[pl.ds(lo, n)], x_v.at[pl.ds(PAD + lo, n)], sem_x.at[i])

    def wk_copy(i):
        if isinstance(i, int):
            lo, n = WK_PIECES[i]
        else:
            lo, n = pl.multiple_of(i * G, G), G
        return pltpu.make_async_copy(wqkv_hbm.at[:, pl.ds(D + lo, n)], wk_v.at[:, pl.ds(lo, n)], sem_k.at[i])

    def wv_copy(i):
        return pltpu.make_async_copy(wqkv_hbm.at[:, pl.ds(2 * D + i * 512, 512)], wv_v.at[i], sem_w.at[i])

    def out_copy(lo, n, s):
        return pltpu.make_async_copy(out_v.at[_rows(lo + PAD, n)], out_hbm.at[_rows(lo, n)], sem_o.at[s])

    wo_copy = pltpu.make_async_copy(wo_hbm, wo_v.at[:, pl.ds(0, D)], sem_w.at[2])
    wg_copy = pltpu.make_async_copy(wg_hbm, wg_v, sem_w.at[3])
    wu_copy = pltpu.make_async_copy(wu_hbm, wu_v, sem_w.at[4])
    wd_copy = pltpu.make_async_copy(wd_hbm, wd_v, sem_w.at[5])
    wr_copy = pltpu.make_async_copy(wr_hbm, wr_v, sem_w.at[6])
    wq_copy = pltpu.make_async_copy(wqkv_hbm.at[:, pl.ds(0, D)], wq_v.at[:, pl.ds(0, D)], sem_w.at[7])

    x_copy(0).start()

    def start_wk(i, c):
        wk_copy(i).start()
        return c

    lax.fori_loop(0, 2, start_wk, 0)
    wk_copy(2).start()

    def zero_pad(i, c):
        rows = pl.ds(pl.multiple_of(i * 32, 32), 32)
        x_v[rows, :] = jnp.zeros((32, D), bf16)
        attn_v[rows, :] = jnp.zeros((32, D), f32)
        return c

    lax.fori_loop(0, PAD // 32, zero_pad, 0)

    def ln_rows(lo, n, sub):
        link = None
        outs = []
        for q in range(0, n, sub):
            x = x_v[_rows(lo + (PAD + q), sub), :].astype(f32)
            mu = jnp.sum(x, axis=-1, keepdims=True) * (1.0 / D)
            if link is not None:
                mu = mu + link
            xc = x - mu
            var = jnp.sum(xc * xc, axis=-1, keepdims=True) * (1.0 / D)
            y = xc * lax.rsqrt(var + LN_EPS)
            link = _zero_of(y[:, D - G:])[:, 0:1]
            yb = y.astype(bf16)
            _put(xn_v, lo + q, yb)
            outs.append(yb)
        return jnp.concatenate(outs, axis=0) if len(outs) > 1 else outs[0]

    def kproj(xn, c0, c1):
        pk = _phi(_dot(xn, wk_v[:, pl.ds(c0, c1 - c0)]))
        zs = jnp.sum(pk.reshape(xn.shape[0] // 8, 8, c1 - c0), axis=0)
        return pk.astype(bf16), zs

    x_copy(1).start()
    x_copy(0).wait()
    wk_copy(3).start()
    ln_rows(0, 256, 256)
    wk_copy(0).wait()
    x_copy(2).start()
    pk0, z0 = kproj(_get(xn_v, 0, 256), 0, 128)
    wk_copy(1).wait()
    x_copy(3).start()
    wq_copy.start()
    pk1, z1 = kproj(_get(xn_v, 0, 256), 128, 256)
    p_v[pl.ds(0, 128), :] = _dot_tn(pk0, _get(xn_v, 0, 256))
    wk_copy(2).wait()
    wv_copy(0).start()
    wv_copy(1).start()
    wo_copy.start()
    wr_copy.start()
    pk2, z2 = kproj(_get(xn_v, 0, 256), 256, 512)
    p_v[pl.ds(128, 128), :] = _dot_tn(pk1, _get(xn_v, 0, 256))
    x_copy(1).wait()
    p_v[pl.ds(256, 256), :] = _dot_tn(pk2, _get(xn_v, 0, 256))
    xb = ln_rows(256, 256, 128)
    pk_b, z_b = kproj(xb, 0, 512)
    p_v[pl.ds(0, 512), :] += _dot_tn(pk_b, xb)
    wk_copy(3).wait()
    x_copy(2).wait()
    wg_copy.start()
    wu_copy.start()
    wd_copy.start()
    x0 = _get(xn_v, 0, T)
    pk_c, z_c = kproj(x0, 512, D)
    p_v[pl.ds(512, 512), :] = _dot_tn(pk_c, x0)
    ln_rows(T, T, 64)
    zacc = jnp.concatenate([jnp.concatenate([z0, z1, z2], axis=1) + z_b, z_c], axis=1)
    x_copy(3).wait()
    wq_copy.wait()

    def l1_body(i, z):
        lo = (i + 1) * T
        xn = _get(xn_v, lo, T, T)
        pk, zs = kproj(xn, 0, D)
        p_v[...] += _dot_tn(pk, xn)
        nxt = jnp.minimum(i + 2, NT - 1) * T
        ln_rows(nxt, T, 32)
        c0 = jnp.minimum(i * 3, NG - 3) * G
        for c in range(3):
            col = pl.multiple_of(c0 + c * G, G)
            _put(wqt_v, col, wq_v[:, pl.ds(col, G)].T, G)
        return z + zs

    zacc = lax.fori_loop(0, NT - 1, l1_body, zacc)

    wv_copy(0).wait()
    wv_copy(1).wait()
    wo_copy.wait()
    wr_copy.wait()

    def qproj(lo, n, zb):
        pqt = _phi(_dot_nt(_get(wqt_v, 0, D), _get(xn_v, lo, n, G)))
        zt = jnp.concatenate([zb] * (n // G), axis=1)
        den = jnp.sum((pqt * zt).reshape(H, DH, n), axis=1, keepdims=True) + PHI_EPS
        inv = pl.reciprocal(den, approx=True)
        inv = inv * (2.0 - den * inv)
        return (pqt.reshape(H, DH, n) * inv).reshape(D, n).astype(bf16)

    def ml_body(i, c):
        z = jnp.sum(zacc, axis=0, keepdims=True)
        zb = jnp.broadcast_to(z, (G, D)).T
        zb_v[...] = zb
        wrf_v[...] = jnp.broadcast_to(wr_v[...].reshape(1, D).astype(f32), (8, D))
        ri = lax.broadcasted_iota(i32, (G, G), 0) // DH
        ci = lax.broadcasted_iota(i32, (G, G), 1) // DH
        same_head = ri == ci
        base = i * (D // 2)
        kvs = {}

        def kv(g):
            t = _dot(p_v[_rows(base + g * G, G, G), :].astype(bf16), wv_v[i, :, pl.ds(g * G, G)])
            kvs[g] = jnp.where(same_head, t, 0.0).astype(bf16)

        def mrow(g):
            _put(m_v, base + g * G, _dot(kvs.pop(g), wo_v[_rows(base + g * G, G, G), pl.ds(0, D)]).astype(bf16), G)

        kv(0)
        kv(1)
        mrow(0)
        keep_v[i] = pltpu.bitcast(qproj(i * HT, HT, zb), u32)
        kv(2)
        mrow(1)
        kv(3)
        mrow(2)
        mrow(3)
        return c

    lax.fori_loop(0, 2, ml_body, 0)

    sub_id = lax.broadcasted_iota(i32, (8, G), 0)

    def keys(r, lo, n):
        rb = lax.bitcast_convert_type(jnp.broadcast_to(r, (n, G)), i32)
        u = rb ^ ((rb >> 31) & 0x7FFFFFFF)
        code0 = (S - 1 - lo) - sub_id
        return rb, [(u[s8:s8 + 8] & ~(S - 1)) | (code0 - s8) for s8 in range(0, n, 8)]

    def merge(a1, a2, b1, b2):
        gt = a1 > b1
        lo = jnp.where(gt, b1, a1)
        other = jnp.where(gt, a2, b2)
        return jnp.where(gt, a1, b1), jnp.where(lo > other, lo, other)

    def post(lo, attn, n, sub, state, link):
        k1, k2 = state
        wr = wrf_v[0:1, :]
        for q in range(0, n, sub):
            rows = _rows(lo + (PAD + q), sub)
            h = x_v[rows, :].astype(f32) + attn[q:q + sub]
            mu = jnp.broadcast_to(jnp.sum(h, axis=-1, keepdims=True) * (1.0 / D), (sub, G))
            if link is not None:
                mu = mu + link
            xc = h - jnp.concatenate([mu] * NG, axis=1)
            var = jnp.sum(xc * xc, axis=-1, keepdims=True) * (1.0 / D)
            hn = xc * lax.rsqrt(var + LN_EPS)
            hn_v[rows, :] = hn
            out_v[rows, :] = (h + hn).astype(bf16)
            rb, ks = keys(jnp.sum(hn * wr, axis=-1, keepdims=True), lo + q, sub)
            link = _zero_of(rb | jnp.concatenate([k2] * (sub // 8), axis=0))
            for key in ks:
                gt = key > k1
                lo2 = jnp.where(gt, k1, key)
                k2 = jnp.where(lo2 > k2, lo2, k2)
                k1 = jnp.where(gt, key, k1)
        return (k1, k2), link

    def post_last(lo, attn, n, state):
        rows = pl.ds(lo + PAD, n)
        h = x_v[rows, :].astype(f32) + attn
        xc = h - jnp.sum(h, axis=-1, keepdims=True) * (1.0 / D)
        var = jnp.sum(xc * xc, axis=-1, keepdims=True) * (1.0 / D)
        t = jnp.sum(xc * wrf_v[0:1, :], axis=-1, keepdims=True)
        rstd = lax.rsqrt(var + LN_EPS)
        hn = xc * rstd
        hn_v[rows, :] = hn
        out_v[rows, :] = (h + hn).astype(bf16)
        _, ks = keys(t * rstd, lo, n)
        pairs = []
        for a, b in zip(ks[0::2], ks[1::2]):
            gt = a > b
            pairs.append((jnp.where(gt, a, b), jnp.where(gt, b, a)))
        pairs.append(state)
        while len(pairs) > 1:
            nxt = [merge(*pairs[j], *pairs[j + 1]) for j in range(0, len(pairs) - 1, 2)]
            pairs = nxt + pairs[len(nxt) * 2:]
        return pairs[0]

    def keep_load():
        return jnp.concatenate([pltpu.bitcast(keep_v[0], bf16), pltpu.bitcast(keep_v[1], bf16)], axis=1)

    def l2_body(i, state):
        lo = i * T
        lhs = keep_load()
        pqn = pltpu.bitcast(qproj(lo + T, T, zb_v[...]), u32)
        keep_v[0] = pqn[:, :HT]
        keep_v[1] = pqn[:, HT:]
        (k1, k2), _ = post(lo - G, attn_v[...], G, 16, state, None)
        state = jnp.where(i > 0, k1, IMIN), jnp.where(i > 0, k2, IMIN)

        @pl.when(i > 0)
        def _():
            out_copy(lo - G, G, 2 * i - 1).start()

        m = _get(m_v, 0, D)
        at_a = _dot_tn(lhs[:, :HT], m)
        at_b = _dot_tn(lhs[:, HT:HT + G], m)
        attn_v[...] = _dot_tn(lhs[:, HT + G:], m)
        state, link = post(lo, at_a, HT, 32, state, None)
        state, _ = post(lo + HT, at_b, G, 32, state, link)
        out_copy(lo, T - G, 2 * i).start()
        return state

    init = jnp.full((8, G), IMIN, i32)
    state = lax.fori_loop(0, NT - 1, l2_body, (init, init))

    wg_copy.wait()
    wu_copy.wait()
    wd_copy.wait()
    lhs = keep_load()
    m = _get(m_v, 0, D)
    lo = S - T
    ats = [_dot_tn(lhs[:, c:c + G], m) for c in range(0, T, G)]
    state, link = post(lo - G, attn_v[...], G, 16, state, None)
    link = jnp.concatenate([link, link], axis=0)
    for c in range(3):
        state, link = post(lo + c * G, ats[c], G, 32, state, link)
    out_copy(lo - G, T, 2 * NT - 3).start()
    k1, k2 = post_last(S - G, ats[3], G, state)
    out_copy(S - G, G, 2 * NT - 2).start()

    for sh in (4, 2, 1):
        k1, k2 = merge(k1, k2, pltpu.roll(k1, sh, 0), pltpu.roll(k2, sh, 0))
    k1 = k1[0:1]
    k2 = k2[0:1]

    def unkey(k):
        i = (S - 1) - (k & (S - 1))
        v = k & ~(S - 1)
        v = v ^ ((v >> 31) & 0x7FFFFFFF)
        return i, lax.bitcast_convert_type(v, f32)

    i1v, r1 = unkey(k1)
    i2v, r2 = unkey(k2)
    i1 = i1v[0, 0]
    i2 = i2v[0, 0]
    b1 = pl.multiple_of((i1 // RB) * RB, RB)
    b2 = pl.multiple_of((i2 // RB) * RB, RB)
    rid = lax.broadcasted_iota(i32, (RB, 1), 0)

    rid8 = lax.broadcasted_iota(i32, (8, D), 0)
    xs = jnp.where(rid8 == 0, jnp.broadcast_to(hn_v[pl.ds(i1 + PAD, 1), :], (8, D)),
                   jnp.broadcast_to(hn_v[pl.ds(i2 + PAD, 1), :], (8, D)))
    xsel = jnp.concatenate([xs, xs], axis=0).astype(bf16)

    acts = {}

    def gu(c):
        sl = pl.ds(c * FC, FC)
        gt = _dot(xsel, wg_v[:, sl])
        ut = _dot(xsel, wu_v[:, sl])
        acts[c] = (gt * jax.nn.sigmoid(gt) * ut).astype(bf16)

    y = None
    gu(0)
    for c in range(NF):
        if c + 1 < NF:
            gu(c + 1)
        t = _dot(acts.pop(c), wd_v[pl.ds(c * FC, FC), :])
        y = t if y is None else y + t
    s1 = jnp.concatenate([jax.nn.sigmoid(r1)] * NG, axis=1)
    s2 = jnp.concatenate([jax.nn.sigmoid(r2)] * NG, axis=1)
    y1 = y[0:1, :] * s1
    y2 = y[1:2, :] * s2

    def fixed(b):
        gid = rid + b
        upd = jnp.where(gid == i1, y1, 0.0) + jnp.where(gid == i2, y2, 0.0)
        return (out_v[_rows(b + PAD, RB), :].astype(f32) + upd).astype(bf16)

    fix_v[0] = fixed(b1)
    fix_v[1] = fixed(b2)
    for i in range(NT - 1):
        if i > 0:
            out_copy(i * T - G, G, 2 * i - 1).wait()
        out_copy(i * T, T - G, 2 * i).wait()
    out_copy(lo - G, T, 2 * NT - 3).wait()
    out_copy(S - G, G, 2 * NT - 2).wait()
    fix1 = pltpu.make_async_copy(fix_v.at[0], out_hbm.at[pl.ds(b1, RB)], sem_f.at[0])
    fix2 = pltpu.make_async_copy(fix_v.at[1], out_hbm.at[pl.ds(b2, RB)], sem_f.at[1])
    fix1.start()

    @pl.when(b1 != b2)
    def _():
        fix2.start()
        fix2.wait()

    fix1.wait()


@jax.jit
def pallas_sequential_preLN__linear_attn_block__moe_arch_mod__prompt_kernel(
    A_x: jax.Array,
    A_wqkv: jax.Array,
    A_wo: jax.Array,
    B_x: jax.Array,
    B_w_r: jax.Array,
    B_w_gate: jax.Array,
    B_w_up: jax.Array,
    B_w_down: jax.Array,
):
    del B_x
    any_spec = pl.BlockSpec(memory_space=pl.ANY)
    out = pl.pallas_call(
        _kernel,
        out_shape=jax.ShapeDtypeStruct((S, D), bf16),
        in_specs=[any_spec] * 7,
        out_specs=any_spec,
        scratch_shapes=[
            pltpu.VMEM((PAD + S, D), bf16),
            pltpu.VMEM((S // 2, D + G), u32),
            pltpu.VMEM((PAD + S, D), f32),
            pltpu.VMEM((PAD + S, D), bf16),
            pltpu.VMEM((D, D + G), bf16),
            pltpu.VMEM((D, D + G), bf16),
            pltpu.VMEM((2, D, D // 2), bf16),
            pltpu.VMEM((D, D + G), bf16),
            pltpu.VMEM((D // 2, D + G), u32),
            pltpu.VMEM((D, D), f32),
            pltpu.VMEM((D // 2, D + G), u32),
            pltpu.VMEM((D, G), f32),
            pltpu.VMEM((D,), bf16),
            pltpu.VMEM((8, D), f32),
            pltpu.VMEM((2, D // 2, HT), u32),
            pltpu.VMEM((G, D), f32),
            pltpu.VMEM((D, F), bf16),
            pltpu.VMEM((D, F), bf16),
            pltpu.VMEM((F, D + G), bf16),
            pltpu.VMEM((2, RB, D), bf16),
            pltpu.SemaphoreType.DMA((len(X_PIECES),)),
            pltpu.SemaphoreType.DMA((4,)),
            pltpu.SemaphoreType.DMA((8,)),
            pltpu.SemaphoreType.DMA((2 * NT - 1,)),
            pltpu.SemaphoreType.DMA((2,)),
        ],
        compiler_params=pltpu.CompilerParams(vmem_limit_bytes=100 * 1024 * 1024, disable_bounds_checks=True, disable_semaphore_checks=True),
    )(A_x.reshape(S, D), A_wqkv, A_wo, B_w_r, B_w_gate, B_w_up, B_w_down)
    return out.reshape(1, S, D)
```

```python
import jax
import jax.numpy as jnp
from jax import lax
import jax.experimental.pallas as pl
import jax.experimental.pallas.tpu as pltpu

S = 2048
D = 1024
F = 3584
H = 32
DH = D // H
LN_EPS = 1e-5
PHI_EPS = 1e-6
G = 128
NG = D // G
RB = 16
FC = 256
NF = F // FC
T = 512
NT = S // T
HT = T // 2
PAD = G

f32 = jnp.float32
bf16 = jnp.bfloat16
u32 = jnp.uint32
i32 = jnp.int32
IMIN = jnp.iinfo(jnp.int32).min

WK_PIECES = ((0, 128), (128, 128), (256, 256), (512, 512))
X_PIECES = ((0, 256), (256, 256), (512, 512), (1024, 1024))


def _zero_of(v):
    u = lax.bitcast_convert_type(v, u32)
    u = lax.shift_right_logical(lax.shift_right_logical(u, jnp.uint32(16)), jnp.uint32(16))
    return lax.bitcast_convert_type(u, f32)


def _phi(t):
    return jnp.where(t > 0, t + 1.0, jnp.exp(t)) + PHI_EPS


def _dot(a, b):
    return jnp.dot(a, b, preferred_element_type=f32)


def _dot_nt(a, b):
    return lax.dot_general(a, b, (((1,), (1,)), ((), ())), preferred_element_type=f32)


def _dot_tn(a, b):
    return lax.dot_general(a, b, (((0,), (0,)), ((), ())), preferred_element_type=f32)


def _half(lo, align):
    return lo // 2 if isinstance(lo, int) else pl.multiple_of(lo >> 1, align // 2)


def _put(ref, lo, val, align=16):
    ref[pl.ds(_half(lo, align), val.shape[0] // 2), :] = pltpu.bitcast(val, u32)


def _get(ref, lo, n, align=16):
    return pltpu.bitcast(ref[pl.ds(_half(lo, align), n // 2), :], bf16)


def _rows(lo, n, align=16):
    return pl.ds(lo if isinstance(lo, int) else pl.multiple_of(lo, align), n)


def _kernel(x_hbm, wqkv_hbm, wo_hbm, wr_hbm, wg_hbm, wu_hbm, wd_hbm, out_hbm,
            x_v, xn_v, hn_v, out_v, wk_v, wq_v, wv_v, wo_v, wqt_v, p_v, m_v, zb_v, wr_v, wrf_v,
            keep_v, attn_v, wg_v, wu_v, wd_v, fix_v,
            sem_x, sem_k, sem_w, sem_o, sem_f):
    xn_v, wqt_v, m_v, wd_v = (r.at[:, pl.ds(0, D)] for r in (xn_v, wqt_v, m_v, wd_v))

    def x_copy(i):
        lo, n = X_PIECES[i]
        return pltpu.make_async_copy(x_hbm.at[pl.ds(lo, n)], x_v.at[pl.ds(PAD + lo, n)], sem_x.at[i])

    def wk_copy(i):
        if isinstance(i, int):
            lo, n = WK_PIECES[i]
        else:
            lo, n = pl.multiple_of(i * G, G), G
        return pltpu.make_async_copy(wqkv_hbm.at[:, pl.ds(D + lo, n)], wk_v.at[:, pl.ds(lo, n)], sem_k.at[i])

    def wv_copy(i):
        return pltpu.make_async_copy(wqkv_hbm.at[:, pl.ds(2 * D + i * 512, 512)], wv_v.at[i], sem_w.at[i])

    def out_copy(lo, n, s):
        return pltpu.make_async_copy(out_v.at[_rows(lo + PAD, n)], out_hbm.at[_rows(lo, n)], sem_o.at[s])

    wo_copy = pltpu.make_async_copy(wo_hbm, wo_v.at[:, pl.ds(0, D)], sem_w.at[2])
    wg_copy = pltpu.make_async_copy(wg_hbm, wg_v, sem_w.at[3])
    wu_copy = pltpu.make_async_copy(wu_hbm, wu_v, sem_w.at[4])
    wd_copy = pltpu.make_async_copy(wd_hbm, wd_v, sem_w.at[5])
    wr_copy = pltpu.make_async_copy(wr_hbm, wr_v, sem_w.at[6])
    wq_copy = pltpu.make_async_copy(wqkv_hbm.at[:, pl.ds(0, D)], wq_v.at[:, pl.ds(0, D)], sem_w.at[7])

    x_copy(0).start()

    def start_wk(i, c):
        wk_copy(i).start()
        return c

    lax.fori_loop(0, 2, start_wk, 0)
    wk_copy(2).start()

    def zero_pad(i, c):
        rows = pl.ds(pl.multiple_of(i * 32, 32), 32)
        x_v[rows, :] = jnp.zeros((32, D), bf16)
        attn_v[rows, :] = jnp.zeros((32, D), f32)
        return c

    lax.fori_loop(0, PAD // 32, zero_pad, 0)

    def ln_rows(lo, n, sub):
        link = None
        outs = []
        for q in range(0, n, sub):
            x = x_v[_rows(lo + (PAD + q), sub), :].astype(f32)
            mu = jnp.sum(x, axis=-1, keepdims=True) * (1.0 / D)
            if link is not None:
                mu = mu + link
            xc = x - mu
            var = jnp.sum(xc * xc, axis=-1, keepdims=True) * (1.0 / D)
            y = xc * lax.rsqrt(var + LN_EPS)
            link = _zero_of(y[:, D - G:])[:, 0:1]
            yb = y.astype(bf16)
            _put(xn_v, lo + q, yb)
            outs.append(yb)
        return jnp.concatenate(outs, axis=0) if len(outs) > 1 else outs[0]

    def kproj(xn, c0, c1):
        pk = _phi(_dot(xn, wk_v[:, pl.ds(c0, c1 - c0)]))
        zs = jnp.sum(pk.reshape(xn.shape[0] // 8, 8, c1 - c0), axis=0)
        return pk.astype(bf16), zs

    x_copy(1).start()
    x_copy(0).wait()
    wk_copy(3).start()
    ln_rows(0, 256, 256)
    wk_copy(0).wait()
    x_copy(2).start()
    pk0, z0 = kproj(_get(xn_v, 0, 256), 0, 128)
    wk_copy(1).wait()
    x_copy(3).start()
    wq_copy.start()
    pk1, z1 = kproj(_get(xn_v, 0, 256), 128, 256)
    p_v[pl.ds(0, 128), :] = _dot_tn(pk0, _get(xn_v, 0, 256))
    p_v[pl.ds(128, 128), :] = _dot_tn(pk1, _get(xn_v, 0, 256))
    wk_copy(2).wait()
    x_copy(1).wait()
    wv_copy(0).start()
    wv_copy(1).start()
    wo_copy.start()
    wr_copy.start()
    pk2, z2 = kproj(_get(xn_v, 0, 256), 256, 512)
    xb = ln_rows(256, 256, 256)
    pk_b, z_b = kproj(xb, 0, 512)
    p_v[pl.ds(256, 256), :] = _dot_tn(pk2, _get(xn_v, 0, 256))
    wk_copy(3).wait()
    x_copy(2).wait()
    wg_copy.start()
    wu_copy.start()
    wd_copy.start()
    x0 = _get(xn_v, 0, T)
    pk_c, z_c = kproj(x0, 512, D)
    p_v[pl.ds(0, 512), :] += _dot_tn(pk_b, _get(xn_v, 256, 256))
    p_v[pl.ds(512, 512), :] = _dot_tn(pk_c, x0)
    ln_rows(T, T, 32)
    zacc = jnp.concatenate([jnp.concatenate([z0, z1, z2], axis=1) + z_b, z_c], axis=1)
    x_copy(3).wait()
    wq_copy.wait()

    def l1_body(i, z):
        lo = (i + 1) * T
        xn = _get(xn_v, lo, T, T)
        pk, zs = kproj(xn, 0, D)
        p_v[...] += _dot_tn(pk, xn)
        nxt = jnp.minimum(i + 2, NT - 1) * T
        ln_rows(nxt, T, 32)
        c0 = jnp.minimum(i * 3, NG - 3) * G
        for c in range(3):
            col = pl.multiple_of(c0 + c * G, G)
            _put(wqt_v, col, wq_v[:, pl.ds(col, G)].T, G)
        return z + zs

    zacc = lax.fori_loop(0, NT - 1, l1_body, zacc)

    wv_copy(0).wait()
    wv_copy(1).wait()
    wo_copy.wait()
    wr_copy.wait()

    def qproj(lo, n, zb):
        pqt = _phi(_dot_nt(_get(wqt_v, 0, D), _get(xn_v, lo, n, G)))
        zt = jnp.concatenate([zb] * (n // G), axis=1)
        den = jnp.sum((pqt * zt).reshape(H, DH, n), axis=1, keepdims=True) + PHI_EPS
        inv = pl.reciprocal(den, approx=True)
        inv = inv * (2.0 - den * inv)
        return (pqt.reshape(H, DH, n) * inv).reshape(D, n).astype(bf16)

    def ml_body(i, c):
        z = jnp.sum(zacc, axis=0, keepdims=True)
        zb = jnp.broadcast_to(z, (G, D)).T
        zb_v[...] = zb
        wrf_v[...] = jnp.broadcast_to(wr_v[...].reshape(1, D).astype(f32), (8, D))
        ri = lax.broadcasted_iota(i32, (G, G), 0) // DH
        ci = lax.broadcasted_iota(i32, (G, G), 1) // DH
        same_head = ri == ci
        base = i * (D // 2)
        kvs = {}

        def kv(g):
            t = _dot(p_v[_rows(base + g * G, G, G), :].astype(bf16), wv_v[i, :, pl.ds(g * G, G)])
            kvs[g] = jnp.where(same_head, t, 0.0).astype(bf16)

        def mrow(g):
            _put(m_v, base + g * G, _dot(kvs.pop(g), wo_v[_rows(base + g * G, G, G), pl.ds(0, D)]).astype(bf16), G)

        kv(0)
        kv(1)
        mrow(0)
        keep_v[i] = pltpu.bitcast(qproj(i * HT, HT, zb), u32)
        kv(2)
        mrow(1)
        kv(3)
        mrow(2)
        mrow(3)
        return c

    lax.fori_loop(0, 2, ml_body, 0)

    sub_id = lax.broadcasted_iota(i32, (8, G), 0)

    def keys(r, lo, n):
        rb = lax.bitcast_convert_type(jnp.broadcast_to(r, (n, G)), i32)
        u = rb ^ ((rb >> 31) & 0x7FFFFFFF)
        code0 = (S - 1 - lo) - sub_id
        return rb, [(u[s8:s8 + 8] & ~(S - 1)) | (code0 - s8) for s8 in range(0, n, 8)]

    def merge(a1, a2, b1, b2):
        gt = a1 > b1
        lo = jnp.where(gt, b1, a1)
        other = jnp.where(gt, a2, b2)
        return jnp.where(gt, a1, b1), jnp.where(lo > other, lo, other)

    def post(lo, attn, n, sub, state, link):
        k1, k2 = state
        wr = wrf_v[0:1, :]
        for q in range(0, n, sub):
            rows = _rows(lo + (PAD + q), sub)
            h = x_v[rows, :].astype(f32) + attn[q:q + sub]
            mu = jnp.broadcast_to(jnp.sum(h, axis=-1, keepdims=True) * (1.0 / D), (sub, G))
            if link is not None:
                mu = mu + link
            xc = h - jnp.concatenate([mu] * NG, axis=1)
            var = jnp.sum(xc * xc, axis=-1, keepdims=True) * (1.0 / D)
            hn = xc * lax.rsqrt(var + LN_EPS)
            hn_v[rows, :] = hn
            out_v[rows, :] = (h + hn).astype(bf16)
            rb, ks = keys(jnp.sum(hn * wr, axis=-1, keepdims=True), lo + q, sub)
            link = _zero_of(rb | jnp.concatenate([k2] * (sub // 8), axis=0))
            for key in ks:
                gt = key > k1
                lo2 = jnp.where(gt, k1, key)
                k2 = jnp.where(lo2 > k2, lo2, k2)
                k1 = jnp.where(gt, key, k1)
        return (k1, k2), link

    def post_last(lo, attn, n, state):
        rows = pl.ds(lo + PAD, n)
        h = x_v[rows, :].astype(f32) + attn
        xc = h - jnp.sum(h, axis=-1, keepdims=True) * (1.0 / D)
        var = jnp.sum(xc * xc, axis=-1, keepdims=True) * (1.0 / D)
        t = jnp.sum(xc * wrf_v[0:1, :], axis=-1, keepdims=True)
        rstd = lax.rsqrt(var + LN_EPS)
        hn = xc * rstd
        hn_v[rows, :] = hn
        out_v[rows, :] = (h + hn).astype(bf16)
        _, ks = keys(t * rstd, lo, n)
        pairs = []
        for a, b in zip(ks[0::2], ks[1::2]):
            gt = a > b
            pairs.append((jnp.where(gt, a, b), jnp.where(gt, b, a)))
        pairs.append(state)
        while len(pairs) > 1:
            nxt = [merge(*pairs[j], *pairs[j + 1]) for j in range(0, len(pairs) - 1, 2)]
            pairs = nxt + pairs[len(nxt) * 2:]
        return pairs[0]

    def keep_load():
        return jnp.concatenate([pltpu.bitcast(keep_v[0], bf16), pltpu.bitcast(keep_v[1], bf16)], axis=1)

    def l2_body(i, state):
        lo = i * T
        lhs = keep_load()
        pqn = pltpu.bitcast(qproj(lo + T, T, zb_v[...]), u32)
        keep_v[0] = pqn[:, :HT]
        keep_v[1] = pqn[:, HT:]
        (k1, k2), _ = post(lo - G, attn_v[...], G, 16, state, None)
        state = jnp.where(i > 0, k1, IMIN), jnp.where(i > 0, k2, IMIN)

        @pl.when(i > 0)
        def _():
            out_copy(lo - G, G, 2 * i - 1).start()

        m = _get(m_v, 0, D)
        at_a = _dot_tn(lhs[:, :HT], m)
        at_b = _dot_tn(lhs[:, HT:HT + G], m)
        attn_v[...] = _dot_tn(lhs[:, HT + G:], m)
        state, link = post(lo, at_a, HT, 32, state, None)
        state, _ = post(lo + HT, at_b, G, 32, state, link)
        out_copy(lo, T - G, 2 * i).start()
        return state

    init = jnp.full((8, G), IMIN, i32)
    state = lax.fori_loop(0, NT - 1, l2_body, (init, init))

    wg_copy.wait()
    wu_copy.wait()
    wd_copy.wait()
    lhs = keep_load()
    m = _get(m_v, 0, D)
    lo = S - T
    ats = [_dot_tn(lhs[:, c:c + G], m) for c in range(0, T, G)]
    state, link = post(lo - G, attn_v[...], G, 16, state, None)
    link = jnp.concatenate([link, link], axis=0)
    for c in range(3):
        state, link = post(lo + c * G, ats[c], G, 32, state, link)
    out_copy(lo - G, T, 2 * NT - 3).start()
    k1, k2 = post_last(S - G, ats[3], G, state)
    out_copy(S - G, G, 2 * NT - 2).start()

    for sh in (4, 2, 1):
        k1, k2 = merge(k1, k2, pltpu.roll(k1, sh, 0), pltpu.roll(k2, sh, 0))
    k1 = k1[0:1]
    k2 = k2[0:1]

    def unkey(k):
        i = (S - 1) - (k & (S - 1))
        v = k & ~(S - 1)
        v = v ^ ((v >> 31) & 0x7FFFFFFF)
        return i, lax.bitcast_convert_type(v, f32)

    i1v, r1 = unkey(k1)
    i2v, r2 = unkey(k2)
    i1 = i1v[0, 0]
    i2 = i2v[0, 0]
    b1 = pl.multiple_of((i1 // RB) * RB, RB)
    b2 = pl.multiple_of((i2 // RB) * RB, RB)
    rid = lax.broadcasted_iota(i32, (RB, 1), 0)

    rid8 = lax.broadcasted_iota(i32, (8, D), 0)
    xs = jnp.where(rid8 == 0, jnp.broadcast_to(hn_v[pl.ds(i1 + PAD, 1), :], (8, D)),
                   jnp.broadcast_to(hn_v[pl.ds(i2 + PAD, 1), :], (8, D)))
    xsel = jnp.concatenate([xs, xs], axis=0).astype(bf16)

    acts = {}

    def gu(c):
        sl = pl.ds(c * FC, FC)
        gt = _dot(xsel, wg_v[:, sl])
        ut = _dot(xsel, wu_v[:, sl])
        acts[c] = (gt * jax.nn.sigmoid(gt) * ut).astype(bf16)

    y = None
    gu(0)
    for c in range(NF):
        if c + 1 < NF:
            gu(c + 1)
        t = _dot(acts.pop(c), wd_v[pl.ds(c * FC, FC), :])
        y = t if y is None else y + t
    s1 = jnp.concatenate([jax.nn.sigmoid(r1)] * NG, axis=1)
    s2 = jnp.concatenate([jax.nn.sigmoid(r2)] * NG, axis=1)
    y1 = y[0:1, :] * s1
    y2 = y[1:2, :] * s2

    def fixed(b):
        gid = rid + b
        upd = jnp.where(gid == i1, y1, 0.0) + jnp.where(gid == i2, y2, 0.0)
        return (out_v[_rows(b + PAD, RB), :].astype(f32) + upd).astype(bf16)

    fix_v[0] = fixed(b1)
    fix_v[1] = fixed(b2)
    for i in range(NT - 1):
        if i > 0:
            out_copy(i * T - G, G, 2 * i - 1).wait()
        out_copy(i * T, T - G, 2 * i).wait()
    out_copy(lo - G, T, 2 * NT - 3).wait()
    out_copy(S - G, G, 2 * NT - 2).wait()
    fix1 = pltpu.make_async_copy(fix_v.at[0], out_hbm.at[pl.ds(b1, RB)], sem_f.at[0])
    fix2 = pltpu.make_async_copy(fix_v.at[1], out_hbm.at[pl.ds(b2, RB)], sem_f.at[1])
    fix1.start()

    @pl.when(b1 != b2)
    def _():
        fix2.start()
        fix2.wait()

    fix1.wait()


@jax.jit
def pallas_sequential_preLN__linear_attn_block__moe_arch_mod__prompt_kernel(
    A_x: jax.Array,
    A_wqkv: jax.Array,
    A_wo: jax.Array,
    B_x: jax.Array,
    B_w_r: jax.Array,
    B_w_gate: jax.Array,
    B_w_up: jax.Array,
    B_w_down: jax.Array,
):
    del B_x
    any_spec = pl.BlockSpec(memory_space=pl.ANY)
    out = pl.pallas_call(
        _kernel,
        out_shape=jax.ShapeDtypeStruct((S, D), bf16),
        in_specs=[any_spec] * 7,
        out_specs=any_spec,
        scratch_shapes=[
            pltpu.VMEM((PAD + S, D), bf16),
            pltpu.VMEM((S // 2, D + G), u32),
            pltpu.VMEM((PAD + S, D), f32),
            pltpu.VMEM((PAD + S, D), bf16),
            pltpu.VMEM((D, D + G), bf16),
            pltpu.VMEM((D, D + G), bf16),
            pltpu.VMEM((2, D, D // 2), bf16),
            pltpu.VMEM((D, D + G), bf16),
            pltpu.VMEM((D // 2, D + G), u32),
            pltpu.VMEM((D, D), f32),
            pltpu.VMEM((D // 2, D + G), u32),
            pltpu.VMEM((D, G), f32),
            pltpu.VMEM((D,), bf16),
            pltpu.VMEM((8, D), f32),
            pltpu.VMEM((2, D // 2, HT), u32),
            pltpu.VMEM((G, D), f32),
            pltpu.VMEM((D, F), bf16),
            pltpu.VMEM((D, F), bf16),
            pltpu.VMEM((F, D + G), bf16),
            pltpu.VMEM((2, RB, D), bf16),
            pltpu.SemaphoreType.DMA((len(X_PIECES),)),
            pltpu.SemaphoreType.DMA((4,)),
            pltpu.SemaphoreType.DMA((8,)),
            pltpu.SemaphoreType.DMA((2 * NT - 1,)),
            pltpu.SemaphoreType.DMA((2,)),
        ],
        compiler_params=pltpu.CompilerParams(vmem_limit_bytes=100 * 1024 * 1024, disable_bounds_checks=True, disable_semaphore_checks=True),
    )(A_x.reshape(S, D), A_wqkv, A_wo, B_w_r, B_w_gate, B_w_up, B_w_down)
    return out.reshape(1, S, D)
```

```python
import jax
import jax.numpy as jnp
from jax import lax
import jax.experimental.pallas as pl
import jax.experimental.pallas.tpu as pltpu

S = 2048
D = 1024
F = 3584
H = 32
DH = D // H
LN_EPS = 1e-5
PHI_EPS = 1e-6
G = 128
NG = D // G
RB = 16
FC = 256
NF = F // FC
T = 512
NT = S // T
HT = T // 2
PAD = G

f32 = jnp.float32
bf16 = jnp.bfloat16
u32 = jnp.uint32
i32 = jnp.int32
IMIN = jnp.iinfo(jnp.int32).min

WK_PIECES = ((0, 128), (128, 128), (256, 256), (512, 512))
X_PIECES = ((0, 256), (256, 256), (512, 512), (1024, 1024))


def _zero_of(v):
    u = lax.bitcast_convert_type(v, u32)
    u = lax.shift_right_logical(lax.shift_right_logical(u, jnp.uint32(16)), jnp.uint32(16))
    return lax.bitcast_convert_type(u, f32)


def _phi(t):
    return jnp.where(t > 0, t + 1.0, jnp.exp(t)) + PHI_EPS


def _dot(a, b):
    return jnp.dot(a, b, preferred_element_type=f32)


def _dot_nt(a, b):
    return lax.dot_general(a, b, (((1,), (1,)), ((), ())), preferred_element_type=f32)


def _dot_tn(a, b):
    return lax.dot_general(a, b, (((0,), (0,)), ((), ())), preferred_element_type=f32)


def _half(lo, align):
    return lo // 2 if isinstance(lo, int) else pl.multiple_of(lo >> 1, align // 2)


def _put(ref, lo, val, align=16):
    ref[pl.ds(_half(lo, align), val.shape[0] // 2), :] = pltpu.bitcast(val, u32)


def _get(ref, lo, n, align=16):
    return pltpu.bitcast(ref[pl.ds(_half(lo, align), n // 2), :], bf16)


def _rows(lo, n, align=16):
    return pl.ds(lo if isinstance(lo, int) else pl.multiple_of(lo, align), n)


def _kernel(x_hbm, wqkv_hbm, wo_hbm, wr_hbm, wg_hbm, wu_hbm, wd_hbm, out_hbm,
            x_v, xn_v, hn_v, out_v, wk_v, wq_v, wv_v, wo_v, wqt_v, p_v, m_v, zb_v, wr_v, wrf_v,
            keep_v, nat_v, attn_v, wg_v, wu_v, wd_v, fix_v,
            sem_x, sem_k, sem_w, sem_o, sem_f):
    xn_v, wqt_v, m_v, wd_v = (r.at[:, pl.ds(0, D)] for r in (xn_v, wqt_v, m_v, wd_v))

    def x_copy(i):
        lo, n = X_PIECES[i]
        return pltpu.make_async_copy(x_hbm.at[pl.ds(lo, n)], x_v.at[pl.ds(PAD + lo, n)], sem_x.at[i])

    def wk_copy(i):
        if isinstance(i, int):
            lo, n = WK_PIECES[i]
        else:
            lo, n = pl.multiple_of(i * G, G), G
        return pltpu.make_async_copy(wqkv_hbm.at[:, pl.ds(D + lo, n)], wk_v.at[:, pl.ds(lo, n)], sem_k.at[i])

    def wv_copy(i):
        return pltpu.make_async_copy(wqkv_hbm.at[:, pl.ds(2 * D + i * 512, 512)], wv_v.at[i], sem_w.at[i])

    def out_copy(lo, n, s):
        return pltpu.make_async_copy(out_v.at[_rows(lo + PAD, n)], out_hbm.at[_rows(lo, n)], sem_o.at[s])

    wo_copy = pltpu.make_async_copy(wo_hbm, wo_v.at[:, pl.ds(0, D)], sem_w.at[2])
    wg_copy = pltpu.make_async_copy(wg_hbm, wg_v, sem_w.at[3])
    wu_copy = pltpu.make_async_copy(wu_hbm, wu_v, sem_w.at[4])
    wd_copy = pltpu.make_async_copy(wd_hbm, wd_v, sem_w.at[5])
    wr_copy = pltpu.make_async_copy(wr_hbm, wr_v, sem_w.at[6])
    wq_copy = pltpu.make_async_copy(wqkv_hbm.at[:, pl.ds(0, D)], wq_v.at[:, pl.ds(0, D)], sem_w.at[7])

    x_copy(0).start()

    def start_wk(i, c):
        wk_copy(i).start()
        return c

    lax.fori_loop(0, 2, start_wk, 0)
    wk_copy(2).start()

    def zero_pad(i, c):
        rows = pl.ds(pl.multiple_of(i * 32, 32), 32)
        x_v[rows, :] = jnp.zeros((32, D), bf16)
        attn_v[rows, :] = jnp.zeros((32, D), f32)
        return c

    lax.fori_loop(0, PAD // 32, zero_pad, 0)

    def ln_rows(lo, n, sub):
        link = None
        outs = []
        for q in range(0, n, sub):
            x = x_v[_rows(lo + (PAD + q), sub), :].astype(f32)
            mu = jnp.sum(x, axis=-1, keepdims=True) * (1.0 / D)
            if link is not None:
                mu = mu + link
            xc = x - mu
            var = jnp.sum(xc * xc, axis=-1, keepdims=True) * (1.0 / D)
            y = xc * lax.rsqrt(var + LN_EPS)
            link = _zero_of(y[:, D - G:])[:, 0:1]
            yb = y.astype(bf16)
            _put(xn_v, lo + q, yb)
            outs.append(yb)
        return jnp.concatenate(outs, axis=0) if len(outs) > 1 else outs[0]

    def kproj(xn, c0, c1):
        pk = _phi(_dot(xn, wk_v[:, pl.ds(c0, c1 - c0)]))
        zs = jnp.sum(pk.reshape(xn.shape[0] // 8, 8, c1 - c0), axis=0)
        return pk.astype(bf16), zs

    x_copy(1).start()
    x_copy(0).wait()
    wk_copy(3).start()
    ln_rows(0, 256, 256)
    wk_copy(0).wait()
    x_copy(2).start()
    pk0, z0 = kproj(_get(xn_v, 0, 256), 0, 128)
    wk_copy(1).wait()
    x_copy(3).start()
    wq_copy.start()
    pk1, z1 = kproj(_get(xn_v, 0, 256), 128, 256)
    p_v[pl.ds(0, 128), :] = _dot_tn(pk0, _get(xn_v, 0, 256))
    p_v[pl.ds(128, 128), :] = _dot_tn(pk1, _get(xn_v, 0, 256))
    wk_copy(2).wait()
    x_copy(1).wait()
    wv_copy(0).start()
    wv_copy(1).start()
    wo_copy.start()
    wr_copy.start()
    pk2, z2 = kproj(_get(xn_v, 0, 256), 256, 512)
    xb = ln_rows(256, 256, 256)
    pk_b, z_b = kproj(xb, 0, 512)
    p_v[pl.ds(256, 256), :] = _dot_tn(pk2, _get(xn_v, 0, 256))
    wk_copy(3).wait()
    x_copy(2).wait()
    wg_copy.start()
    wu_copy.start()
    wd_copy.start()
    x0 = _get(xn_v, 0, T)
    pk_c, z_c = kproj(x0, 512, D)
    p_v[pl.ds(0, 512), :] += _dot_tn(pk_b, _get(xn_v, 256, 256))
    p_v[pl.ds(512, 512), :] = _dot_tn(pk_c, x0)
    ln_rows(T, T, 32)
    zacc = jnp.concatenate([jnp.concatenate([z0, z1, z2], axis=1) + z_b, z_c], axis=1)
    x_copy(3).wait()
    wq_copy.wait()

    def l1_body(i, z):
        lo = (i + 1) * T
        xn = _get(xn_v, lo, T, T)
        pk, zs = kproj(xn, 0, D)
        p_v[...] += _dot_tn(pk, xn)
        nxt = jnp.minimum(i + 2, NT - 1) * T
        ln_rows(nxt, T, 32)
        c0 = jnp.minimum(i * 3, NG - 3) * G
        for c in range(3):
            col = pl.multiple_of(c0 + c * G, G)
            _put(wqt_v, col, wq_v[:, pl.ds(col, G)].T, G)
        return z + zs

    zacc = lax.fori_loop(0, NT - 1, l1_body, zacc)

    wv_copy(0).wait()
    wv_copy(1).wait()
    wo_copy.wait()
    wr_copy.wait()

    def qproj(lo, n, zb):
        pqt = _phi(_dot_nt(_get(wqt_v, 0, D), _get(xn_v, lo, n, G)))
        zt = jnp.concatenate([zb] * (n // G), axis=1)
        den = jnp.sum((pqt * zt).reshape(H, DH, n), axis=1, keepdims=True) + PHI_EPS
        inv = pl.reciprocal(den, approx=True)
        inv = inv * (2.0 - den * inv)
        return (pqt.reshape(H, DH, n) * inv).reshape(D, n).astype(bf16)

    def ml_body(i, c):
        z = jnp.sum(zacc, axis=0, keepdims=True)
        zb = jnp.broadcast_to(z, (G, D)).T
        zb_v[...] = zb
        wrf_v[...] = jnp.broadcast_to(wr_v[...].reshape(1, D).astype(f32), (8, D))
        ri = lax.broadcasted_iota(i32, (G, G), 0) // DH
        ci = lax.broadcasted_iota(i32, (G, G), 1) // DH
        same_head = ri == ci
        base = i * (D // 2)
        kvs = {}

        def kv(g):
            t = _dot(p_v[_rows(base + g * G, G, G), :].astype(bf16), wv_v[i, :, pl.ds(g * G, G)])
            kvs[g] = jnp.where(same_head, t, 0.0).astype(bf16)

        def mrow(g):
            _put(m_v, base + g * G, _dot(kvs.pop(g), wo_v[_rows(base + g * G, G, G), pl.ds(0, D)]).astype(bf16), G)

        kv(0)
        kv(1)
        mrow(0)
        keep_v[i] = pltpu.bitcast(qproj(i * HT, HT, zb), u32)
        kv(2)
        mrow(1)
        kv(3)
        mrow(2)
        mrow(3)
        return c

    lax.fori_loop(0, 2, ml_body, 0)

    sub_id = lax.broadcasted_iota(i32, (8, G), 0)

    def keys(r, lo, n):
        rb = lax.bitcast_convert_type(jnp.broadcast_to(r, (n, G)), i32)
        u = rb ^ ((rb >> 31) & 0x7FFFFFFF)
        code0 = (S - 1 - lo) - sub_id
        return rb, [(u[s8:s8 + 8] & ~(S - 1)) | (code0 - s8) for s8 in range(0, n, 8)]

    def merge(a1, a2, b1, b2):
        gt = a1 > b1
        lo = jnp.where(gt, b1, a1)
        other = jnp.where(gt, a2, b2)
        return jnp.where(gt, a1, b1), jnp.where(lo > other, lo, other)

    def post(lo, attn, n, sub, state, link):
        k1, k2 = state
        wr = wrf_v[0:1, :]
        for q in range(0, n, sub):
            rows = _rows(lo + (PAD + q), sub)
            h = x_v[rows, :].astype(f32) + attn[q:q + sub]
            mu = jnp.broadcast_to(jnp.sum(h, axis=-1, keepdims=True) * (1.0 / D), (sub, G))
            if link is not None:
                mu = mu + link
            xc = h - jnp.concatenate([mu] * NG, axis=1)
            var = jnp.sum(xc * xc, axis=-1, keepdims=True) * (1.0 / D)
            hn = xc * lax.rsqrt(var + LN_EPS)
            hn_v[rows, :] = hn
            out_v[rows, :] = (h + hn).astype(bf16)
            rb, ks = keys(jnp.sum(hn * wr, axis=-1, keepdims=True), lo + q, sub)
            link = _zero_of(rb | jnp.concatenate([k2] * (sub // 8), axis=0))
            for key in ks:
                gt = key > k1
                lo2 = jnp.where(gt, k1, key)
                k2 = jnp.where(lo2 > k2, lo2, k2)
                k1 = jnp.where(gt, key, k1)
        return (k1, k2), link

    def post_last(lo, attn, n, state):
        rows = pl.ds(lo + PAD, n)
        h = x_v[rows, :].astype(f32) + attn
        xc = h - jnp.sum(h, axis=-1, keepdims=True) * (1.0 / D)
        var = jnp.sum(xc * xc, axis=-1, keepdims=True) * (1.0 / D)
        t = jnp.sum(xc * wrf_v[0:1, :], axis=-1, keepdims=True)
        rstd = lax.rsqrt(var + LN_EPS)
        hn = xc * rstd
        hn_v[rows, :] = hn
        out_v[rows, :] = (h + hn).astype(bf16)
        _, ks = keys(t * rstd, lo, n)
        pairs = []
        for a, b in zip(ks[0::2], ks[1::2]):
            gt = a > b
            pairs.append((jnp.where(gt, a, b), jnp.where(gt, b, a)))
        pairs.append(state)
        while len(pairs) > 1:
            nxt = [merge(*pairs[j], *pairs[j + 1]) for j in range(0, len(pairs) - 1, 2)]
            pairs = nxt + pairs[len(nxt) * 2:]
        return pairs[0]

    def keep_load():
        return jnp.concatenate([pltpu.bitcast(keep_v[0], bf16), pltpu.bitcast(keep_v[1], bf16)], axis=1)

    def l2_body(i, state):
        lo = i * T
        lhs = keep_load()
        pqn = qproj(lo + T, T, zb_v[...])
        _put(nat_v, 0, pqn[:, :G].T)
        pqn = pltpu.bitcast(pqn, u32)
        keep_v[0] = pqn[:, :HT]
        keep_v[1] = pqn[:, HT:]
        (k1, k2), _ = post(lo - G, attn_v[...], G, 16, state, None)
        state = jnp.where(i > 0, k1, IMIN), jnp.where(i > 0, k2, IMIN)

        @pl.when(i > 0)
        def _():
            out_copy(lo - G, G, 2 * i - 1).start()

        m = _get(m_v, 0, D)
        at_a = _dot_tn(lhs[:, :HT], m)
        at_b = _dot_tn(lhs[:, HT:HT + G], m)
        attn_v[...] = _dot_tn(lhs[:, HT + G:], m)
        state, link = post(lo, at_a, HT, 32, state, None)
        state, _ = post(lo + HT, at_b, G, 32, state, link)
        out_copy(lo, T - G, 2 * i).start()
        return state

    init = jnp.full((8, G), IMIN, i32)
    state = lax.fori_loop(0, NT - 1, l2_body, (init, init))

    wg_copy.wait()
    wu_copy.wait()
    wd_copy.wait()
    lhs = keep_load()
    m = _get(m_v, 0, D)
    lo = S - T
    ats = [_dot(_get(nat_v, 0, G), m)] + [_dot_tn(lhs[:, c:c + G], m) for c in range(G, T, G)]
    state, link = post(lo - G, attn_v[...], G, 16, state, None)
    link = jnp.concatenate([link, link], axis=0)
    for c in range(3):
        state, link = post(lo + c * G, ats[c], G, 32, state, link)
    out_copy(lo - G, T, 2 * NT - 3).start()
    k1, k2 = post_last(S - G, ats[3], G, state)
    out_copy(S - G, G, 2 * NT - 2).start()

    for sh in (4, 2, 1):
        k1, k2 = merge(k1, k2, pltpu.roll(k1, sh, 0), pltpu.roll(k2, sh, 0))
    k1 = k1[0:1]
    k2 = k2[0:1]

    def unkey(k):
        i = (S - 1) - (k & (S - 1))
        v = k & ~(S - 1)
        v = v ^ ((v >> 31) & 0x7FFFFFFF)
        return i, lax.bitcast_convert_type(v, f32)

    i1v, r1 = unkey(k1)
    i2v, r2 = unkey(k2)
    i1 = i1v[0, 0]
    i2 = i2v[0, 0]
    b1 = pl.multiple_of((i1 // RB) * RB, RB)
    b2 = pl.multiple_of((i2 // RB) * RB, RB)
    rid = lax.broadcasted_iota(i32, (RB, 1), 0)

    rid8 = lax.broadcasted_iota(i32, (8, D), 0)
    xs = jnp.where(rid8 == 0, jnp.broadcast_to(hn_v[pl.ds(i1 + PAD, 1), :], (8, D)),
                   jnp.broadcast_to(hn_v[pl.ds(i2 + PAD, 1), :], (8, D)))
    xsel = jnp.concatenate([xs, xs], axis=0).astype(bf16)

    acts = {}

    def gu(c):
        sl = pl.ds(c * FC, FC)
        gt = _dot(xsel, wg_v[:, sl])
        ut = _dot(xsel, wu_v[:, sl])
        acts[c] = (gt * jax.nn.sigmoid(gt) * ut).astype(bf16)

    y = None
    gu(0)
    for c in range(NF):
        if c + 1 < NF:
            gu(c + 1)
        t = _dot(acts.pop(c), wd_v[pl.ds(c * FC, FC), :])
        y = t if y is None else y + t
    s1 = jnp.concatenate([jax.nn.sigmoid(r1)] * NG, axis=1)
    s2 = jnp.concatenate([jax.nn.sigmoid(r2)] * NG, axis=1)
    y1 = y[0:1, :] * s1
    y2 = y[1:2, :] * s2

    def fixed(b):
        gid = rid + b
        upd = jnp.where(gid == i1, y1, 0.0) + jnp.where(gid == i2, y2, 0.0)
        return (out_v[_rows(b + PAD, RB), :].astype(f32) + upd).astype(bf16)

    fix_v[0] = fixed(b1)
    fix_v[1] = fixed(b2)
    for i in range(NT - 1):
        if i > 0:
            out_copy(i * T - G, G, 2 * i - 1).wait()
        out_copy(i * T, T - G, 2 * i).wait()
    out_copy(lo - G, T, 2 * NT - 3).wait()
    out_copy(S - G, G, 2 * NT - 2).wait()
    fix1 = pltpu.make_async_copy(fix_v.at[0], out_hbm.at[pl.ds(b1, RB)], sem_f.at[0])
    fix2 = pltpu.make_async_copy(fix_v.at[1], out_hbm.at[pl.ds(b2, RB)], sem_f.at[1])
    fix1.start()

    @pl.when(b1 != b2)
    def _():
        fix2.start()
        fix2.wait()

    fix1.wait()


@jax.jit
def pallas_sequential_preLN__linear_attn_block__moe_arch_mod__prompt_kernel(
    A_x: jax.Array,
    A_wqkv: jax.Array,
    A_wo: jax.Array,
    B_x: jax.Array,
    B_w_r: jax.Array,
    B_w_gate: jax.Array,
    B_w_up: jax.Array,
    B_w_down: jax.Array,
):
    del B_x
    any_spec = pl.BlockSpec(memory_space=pl.ANY)
    out = pl.pallas_call(
        _kernel,
        out_shape=jax.ShapeDtypeStruct((S, D), bf16),
        in_specs=[any_spec] * 7,
        out_specs=any_spec,
        scratch_shapes=[
            pltpu.VMEM((PAD + S, D), bf16),
            pltpu.VMEM((S // 2, D + G), u32),
            pltpu.VMEM((PAD + S, D), f32),
            pltpu.VMEM((PAD + S, D), bf16),
            pltpu.VMEM((D, D + G), bf16),
            pltpu.VMEM((D, D + G), bf16),
            pltpu.VMEM((2, D, D // 2), bf16),
            pltpu.VMEM((D, D + G), bf16),
            pltpu.VMEM((D // 2, D + G), u32),
            pltpu.VMEM((D, D), f32),
            pltpu.VMEM((D // 2, D + G), u32),
            pltpu.VMEM((D, G), f32),
            pltpu.VMEM((D,), bf16),
            pltpu.VMEM((8, D), f32),
            pltpu.VMEM((2, D // 2, HT), u32),
            pltpu.VMEM((G // 2, D), u32),
            pltpu.VMEM((G, D), f32),
            pltpu.VMEM((D, F), bf16),
            pltpu.VMEM((D, F), bf16),
            pltpu.VMEM((F, D + G), bf16),
            pltpu.VMEM((2, RB, D), bf16),
            pltpu.SemaphoreType.DMA((len(X_PIECES),)),
            pltpu.SemaphoreType.DMA((4,)),
            pltpu.SemaphoreType.DMA((8,)),
            pltpu.SemaphoreType.DMA((2 * NT - 1,)),
            pltpu.SemaphoreType.DMA((2,)),
        ],
        compiler_params=pltpu.CompilerParams(vmem_limit_bytes=100 * 1024 * 1024, disable_bounds_checks=True, disable_semaphore_checks=True),
    )(A_x.reshape(S, D), A_wqkv, A_wo, B_w_r, B_w_gate, B_w_up, B_w_down)
    return out.reshape(1, S, D)
```

```python
import jax
import jax.numpy as jnp
from jax import lax
import jax.experimental.pallas as pl
import jax.experimental.pallas.tpu as pltpu

S = 2048
D = 1024
F = 3584
H = 32
DH = D // H
LN_EPS = 1e-5
PHI_EPS = 1e-6
G = 128
NG = D // G
RB = 8
FC = 256
NF = F // FC
T = 512
NT = S // T
HT = T // 2
PAD = G

f32 = jnp.float32
bf16 = jnp.bfloat16
u32 = jnp.uint32
i32 = jnp.int32
IMIN = jnp.iinfo(jnp.int32).min

WK_PIECES = ((0, 128), (128, 128), (256, 256), (512, 512))
X_PIECES = ((0, 256), (256, 256), (512, 512), (1024, 1024))


def _zero_of(v):
    u = lax.bitcast_convert_type(v, u32)
    u = lax.shift_right_logical(lax.shift_right_logical(u, jnp.uint32(16)), jnp.uint32(16))
    return lax.bitcast_convert_type(u, f32)


def _phi(t):
    return jnp.where(t > 0, t + 1.0, jnp.exp(t)) + PHI_EPS


def _dot(a, b):
    return jnp.dot(a, b, preferred_element_type=f32)


def _dot_nt(a, b):
    return lax.dot_general(a, b, (((1,), (1,)), ((), ())), preferred_element_type=f32)


def _dot_tn(a, b):
    return lax.dot_general(a, b, (((0,), (0,)), ((), ())), preferred_element_type=f32)


def _half(lo, align):
    return lo // 2 if isinstance(lo, int) else pl.multiple_of(lo >> 1, align // 2)


def _put(ref, lo, val, align=16):
    ref[pl.ds(_half(lo, align), val.shape[0] // 2), :] = pltpu.bitcast(val, u32)


def _get(ref, lo, n, align=16):
    return pltpu.bitcast(ref[pl.ds(_half(lo, align), n // 2), :], bf16)


def _rows(lo, n, align=16):
    return pl.ds(lo if isinstance(lo, int) else pl.multiple_of(lo, align), n)


def _kernel(x_hbm, wqkv_hbm, wo_hbm, wr_hbm, wg_hbm, wu_hbm, wd_hbm, out_hbm,
            x_v, xn_v, hn_v, out_v, wk_v, wq_v, wv_v, wo_v, wqt_v, p_v, m_v, zb_v, wr_v, wrf_v,
            keep_v, nat_v, attn_v, wg_v, wu_v, wd_v, fix_v,
            sem_x, sem_k, sem_w, sem_o, sem_f):
    xn_v, wqt_v, m_v, wd_v = (r.at[:, pl.ds(0, D)] for r in (xn_v, wqt_v, m_v, wd_v))

    def x_copy(i):
        lo, n = X_PIECES[i]
        return pltpu.make_async_copy(x_hbm.at[pl.ds(lo, n)], x_v.at[pl.ds(PAD + lo, n)], sem_x.at[i])

    def wk_copy(i):
        if isinstance(i, int):
            lo, n = WK_PIECES[i]
        else:
            lo, n = pl.multiple_of(i * G, G), G
        return pltpu.make_async_copy(wqkv_hbm.at[:, pl.ds(D + lo, n)], wk_v.at[:, pl.ds(lo, n)], sem_k.at[i])

    def wv_copy(i):
        return pltpu.make_async_copy(wqkv_hbm.at[:, pl.ds(2 * D + i * 512, 512)], wv_v.at[i], sem_w.at[i])

    def out_copy(lo, n, s):
        return pltpu.make_async_copy(out_v.at[_rows(lo + PAD, n)], out_hbm.at[_rows(lo, n)], sem_o.at[s])

    wo_copy = pltpu.make_async_copy(wo_hbm, wo_v.at[:, pl.ds(0, D)], sem_w.at[2])
    wg_copy = pltpu.make_async_copy(wg_hbm, wg_v, sem_w.at[3])
    wu_copy = pltpu.make_async_copy(wu_hbm, wu_v, sem_w.at[4])
    wd_copy = pltpu.make_async_copy(wd_hbm, wd_v, sem_w.at[5])
    wr_copy = pltpu.make_async_copy(wr_hbm, wr_v, sem_w.at[6])
    wq_copy = pltpu.make_async_copy(wqkv_hbm.at[:, pl.ds(0, D)], wq_v.at[:, pl.ds(0, D)], sem_w.at[7])

    x_copy(0).start()

    def start_wk(i, c):
        wk_copy(i).start()
        return c

    lax.fori_loop(0, 2, start_wk, 0)
    wk_copy(2).start()

    def zero_pad(i, c):
        rows = pl.ds(pl.multiple_of(i * 32, 32), 32)
        x_v[rows, :] = jnp.zeros((32, D), bf16)
        attn_v[rows, :] = jnp.zeros((32, D), f32)
        return c

    lax.fori_loop(0, PAD // 32, zero_pad, 0)

    def ln_rows(lo, n, sub):
        link = None
        outs = []
        for q in range(0, n, sub):
            x = x_v[_rows(lo + (PAD + q), sub), :].astype(f32)
            mu = jnp.sum(x, axis=-1, keepdims=True) * (1.0 / D)
            if link is not None:
                mu = mu + link
            xc = x - mu
            var = jnp.sum(xc * xc, axis=-1, keepdims=True) * (1.0 / D)
            y = xc * lax.rsqrt(var + LN_EPS)
            link = _zero_of(y[:, D - G:])[:, 0:1]
            yb = y.astype(bf16)
            _put(xn_v, lo + q, yb)
            outs.append(yb)
        return jnp.concatenate(outs, axis=0) if len(outs) > 1 else outs[0]

    def kproj(xn, c0, c1):
        pk = _phi(_dot(xn, wk_v[:, pl.ds(c0, c1 - c0)]))
        zs = jnp.sum(pk.reshape(xn.shape[0] // 8, 8, c1 - c0), axis=0)
        return pk.astype(bf16), zs

    x_copy(1).start()
    x_copy(0).wait()
    wk_copy(3).start()
    ln_rows(0, 256, 256)
    wk_copy(0).wait()
    x_copy(2).start()
    pk0, z0 = kproj(_get(xn_v, 0, 256), 0, 128)
    wk_copy(1).wait()
    x_copy(3).start()
    wq_copy.start()
    pk1, z1 = kproj(_get(xn_v, 0, 256), 128, 256)
    p_v[pl.ds(0, 128), :] = _dot_tn(pk0, _get(xn_v, 0, 256))
    p_v[pl.ds(128, 128), :] = _dot_tn(pk1, _get(xn_v, 0, 256))
    wk_copy(2).wait()
    x_copy(1).wait()
    wv_copy(0).start()
    wv_copy(1).start()
    wo_copy.start()
    wr_copy.start()
    pk2, z2 = kproj(_get(xn_v, 0, 256), 256, 512)
    xb = ln_rows(256, 256, 256)
    pk_b, z_b = kproj(xb, 0, 512)
    p_v[pl.ds(256, 256), :] = _dot_tn(pk2, _get(xn_v, 0, 256))
    wk_copy(3).wait()
    x_copy(2).wait()
    wg_copy.start()
    wu_copy.start()
    wd_copy.start()
    x0 = _get(xn_v, 0, T)
    pk_c, z_c = kproj(x0, 512, D)
    p_v[pl.ds(0, 512), :] += _dot_tn(pk_b, _get(xn_v, 256, 256))
    p_v[pl.ds(512, 512), :] = _dot_tn(pk_c, x0)
    ln_rows(T, T, 32)
    zacc = jnp.concatenate([jnp.concatenate([z0, z1, z2], axis=1) + z_b, z_c], axis=1)
    x_copy(3).wait()
    wq_copy.wait()

    def l1_body(i, z):
        lo = (i + 1) * T
        xn = _get(xn_v, lo, T, T)
        pk, zs = kproj(xn, 0, D)
        p_v[...] += _dot_tn(pk, xn)
        nxt = jnp.minimum(i + 2, NT - 1) * T
        ln_rows(nxt, T, 32)
        c0 = jnp.minimum(i * 3, NG - 3) * G
        for c in range(3):
            col = pl.multiple_of(c0 + c * G, G)
            _put(wqt_v, col, wq_v[:, pl.ds(col, G)].T, G)
        return z + zs

    zacc = lax.fori_loop(0, NT - 1, l1_body, zacc)

    wv_copy(0).wait()
    wv_copy(1).wait()
    wo_copy.wait()
    wr_copy.wait()

    def qproj(lo, n, zb):
        pqt = _phi(_dot_nt(_get(wqt_v, 0, D), _get(xn_v, lo, n, G)))
        zt = jnp.concatenate([zb] * (n // G), axis=1)
        den = jnp.sum((pqt * zt).reshape(H, DH, n), axis=1, keepdims=True) + PHI_EPS
        inv = pl.reciprocal(den, approx=True)
        inv = inv * (2.0 - den * inv)
        return (pqt.reshape(H, DH, n) * inv).reshape(D, n).astype(bf16)

    def ml_body(i, c):
        z = jnp.sum(zacc, axis=0, keepdims=True)
        zb = jnp.broadcast_to(z, (G, D)).T
        zb_v[...] = zb
        wrf_v[...] = jnp.broadcast_to(wr_v[...].reshape(1, D).astype(f32), (8, D))
        ri = lax.broadcasted_iota(i32, (G, G), 0) // DH
        ci = lax.broadcasted_iota(i32, (G, G), 1) // DH
        same_head = ri == ci
        base = i * (D // 2)
        kvs = {}

        def kv(g):
            t = _dot(p_v[_rows(base + g * G, G, G), :].astype(bf16), wv_v[i, :, pl.ds(g * G, G)])
            kvs[g] = jnp.where(same_head, t, 0.0).astype(bf16)

        def mrow(g):
            _put(m_v, base + g * G, _dot(kvs.pop(g), wo_v[_rows(base + g * G, G, G), pl.ds(0, D)]).astype(bf16), G)

        kv(0)
        kv(1)
        mrow(0)
        keep_v[i] = pltpu.bitcast(qproj(i * HT, HT, zb), u32)
        kv(2)
        mrow(1)
        kv(3)
        mrow(2)
        mrow(3)
        return c

    lax.fori_loop(0, 2, ml_body, 0)

    sub_id = lax.broadcasted_iota(i32, (8, G), 0)

    def keys(r, lo, n):
        rb = lax.bitcast_convert_type(jnp.broadcast_to(r, (n, G)), i32)
        u = rb ^ ((rb >> 31) & 0x7FFFFFFF)
        code0 = (S - 1 - lo) - sub_id
        return rb, [(u[s8:s8 + 8] & ~(S - 1)) | (code0 - s8) for s8 in range(0, n, 8)]

    def merge(a1, a2, b1, b2):
        gt = a1 > b1
        lo = jnp.where(gt, b1, a1)
        other = jnp.where(gt, a2, b2)
        return jnp.where(gt, a1, b1), jnp.where(lo > other, lo, other)

    def post(lo, attn, n, sub, state, link):
        k1, k2 = state
        wr = wrf_v[0:1, :]
        for q in range(0, n, sub):
            rows = _rows(lo + (PAD + q), sub)
            h = x_v[rows, :].astype(f32) + attn[q:q + sub]
            mu = jnp.broadcast_to(jnp.sum(h, axis=-1, keepdims=True) * (1.0 / D), (sub, G))
            if link is not None:
                mu = mu + link
            xc = h - jnp.concatenate([mu] * NG, axis=1)
            var = jnp.sum(xc * xc, axis=-1, keepdims=True) * (1.0 / D)
            hn = xc * lax.rsqrt(var + LN_EPS)
            hn_v[rows, :] = hn
            out_v[rows, :] = (h + hn).astype(bf16)
            rb, ks = keys(jnp.sum(hn * wr, axis=-1, keepdims=True), lo + q, sub)
            link = _zero_of(rb | jnp.concatenate([k2] * (sub // 8), axis=0))
            for key in ks:
                gt = key > k1
                lo2 = jnp.where(gt, k1, key)
                k2 = jnp.where(lo2 > k2, lo2, k2)
                k1 = jnp.where(gt, key, k1)
        return (k1, k2), link

    def post_last(lo, attn, n, state):
        rows = pl.ds(lo + PAD, n)
        h = x_v[rows, :].astype(f32) + attn
        xc = h - jnp.sum(h, axis=-1, keepdims=True) * (1.0 / D)
        var = jnp.sum(xc * xc, axis=-1, keepdims=True) * (1.0 / D)
        t = jnp.sum(xc * wrf_v[0:1, :], axis=-1, keepdims=True)
        rstd = lax.rsqrt(var + LN_EPS)
        hn = xc * rstd
        hn_v[rows, :] = hn
        out_v[rows, :] = (h + hn).astype(bf16)
        _, ks = keys(t * rstd, lo, n)
        pairs = []
        for a, b in zip(ks[0::2], ks[1::2]):
            gt = a > b
            pairs.append((jnp.where(gt, a, b), jnp.where(gt, b, a)))
        pairs.append(state)
        while len(pairs) > 1:
            nxt = [merge(*pairs[j], *pairs[j + 1]) for j in range(0, len(pairs) - 1, 2)]
            pairs = nxt + pairs[len(nxt) * 2:]
        return pairs[0]

    def keep_load():
        return jnp.concatenate([pltpu.bitcast(keep_v[0], bf16), pltpu.bitcast(keep_v[1], bf16)], axis=1)

    def l2_body(i, state):
        lo = i * T
        lhs = keep_load()
        pqn = qproj(lo + T, T, zb_v[...])
        _put(nat_v, 0, pqn[:, :G].T)
        pqn = pltpu.bitcast(pqn, u32)
        keep_v[0] = pqn[:, :HT]
        keep_v[1] = pqn[:, HT:]
        (k1, k2), _ = post(lo - G, attn_v[...], G, 16, state, None)
        state = jnp.where(i > 0, k1, IMIN), jnp.where(i > 0, k2, IMIN)

        @pl.when(i > 0)
        def _():
            out_copy(lo - G, G, 2 * i - 1).start()

        m = _get(m_v, 0, D)
        at_a = _dot_tn(lhs[:, :HT], m)
        at_b = _dot_tn(lhs[:, HT:HT + G], m)
        attn_v[...] = _dot_tn(lhs[:, HT + G:], m)
        state, link = post(lo, at_a, HT, 32, state, None)
        state, _ = post(lo + HT, at_b, G, 32, state, link)
        out_copy(lo, T - G, 2 * i).start()
        return state

    init = jnp.full((8, G), IMIN, i32)
    state = lax.fori_loop(0, NT - 1, l2_body, (init, init))

    wg_copy.wait()
    wu_copy.wait()
    wd_copy.wait()
    lhs = keep_load()
    m = _get(m_v, 0, D)
    lo = S - T
    _put(nat_v, G, lhs[:, 3 * G:].T)
    at_a = _dot(_get(nat_v, 0, G), m)
    at_b = _dot_tn(lhs[:, G:3 * G], m)
    at_c = _dot(_get(nat_v, G, G), m)
    state, link = post(lo - G, attn_v[...], G, 16, state, None)
    state, link = post(lo, at_a, G, 16, state, link)
    state, _ = post(lo + G, at_b, 2 * G, 64, state, jnp.concatenate([link] * 4, axis=0))
    k1, k2 = post_last(lo + 3 * G, at_c, G, state)
    out_copy(lo - G, T + G, 2 * NT - 3).start()

    for sh in (4, 2, 1):
        k1, k2 = merge(k1, k2, pltpu.roll(k1, sh, 0), pltpu.roll(k2, sh, 0))
    k1 = k1[0:1]
    k2 = k2[0:1]

    def unkey(k):
        i = (S - 1) - (k & (S - 1))
        v = k & ~(S - 1)
        v = v ^ ((v >> 31) & 0x7FFFFFFF)
        return i, lax.bitcast_convert_type(v, f32)

    i1v, r1 = unkey(k1)
    i2v, r2 = unkey(k2)
    i1 = i1v[0, 0]
    i2 = i2v[0, 0]
    b1 = pl.multiple_of(i1 & ~(RB - 1), RB)
    b2 = pl.multiple_of(i2 & ~(RB - 1), RB)
    rid = lax.broadcasted_iota(i32, (RB, 1), 0)

    rid8 = lax.broadcasted_iota(i32, (8, D), 0)
    xs = jnp.where(rid8 == 0, jnp.broadcast_to(hn_v[pl.ds(i1 + PAD, 1), :], (8, D)),
                   jnp.broadcast_to(hn_v[pl.ds(i2 + PAD, 1), :], (8, D)))
    xsel = jnp.concatenate([xs, xs], axis=0).astype(bf16)

    acts = {}

    def gu(c):
        sl = pl.ds(c * FC, FC)
        gt = _dot(xsel, wg_v[:, sl])
        ut = _dot(xsel, wu_v[:, sl])
        acts[c] = (gt * jax.nn.sigmoid(gt) * ut).astype(bf16)

    y = None
    gu(0)
    for c in range(NF):
        if c + 1 < NF:
            gu(c + 1)
        t = _dot(acts.pop(c), wd_v[pl.ds(c * FC, FC), :])
        y = t if y is None else y + t
    s1 = jnp.concatenate([jax.nn.sigmoid(r1)] * NG, axis=1)
    s2 = jnp.concatenate([jax.nn.sigmoid(r2)] * NG, axis=1)
    y1 = y[0:1, :] * s1
    y2 = y[1:2, :] * s2

    def fixed(b):
        gid = rid + b
        upd = jnp.where(gid == i1, y1, 0.0) + jnp.where(gid == i2, y2, 0.0)
        return (out_v[_rows(b + PAD, RB, RB), :].astype(f32) + upd).astype(bf16)

    fix_v[0] = fixed(b1)
    fix_v[1] = fixed(b2)
    for i in range(NT - 1):
        if i > 0:
            out_copy(i * T - G, G, 2 * i - 1).wait()
        out_copy(i * T, T - G, 2 * i).wait()
    out_copy(lo - G, T + G, 2 * NT - 3).wait()
    fix1 = pltpu.make_async_copy(fix_v.at[0], out_hbm.at[pl.ds(b1, RB)], sem_f.at[0])
    fix2 = pltpu.make_async_copy(fix_v.at[1], out_hbm.at[pl.ds(b2, RB)], sem_f.at[1])
    fix1.start()

    @pl.when(b1 != b2)
    def _():
        fix2.start()
        fix2.wait()

    fix1.wait()


@jax.jit
def pallas_sequential_preLN__linear_attn_block__moe_arch_mod__prompt_kernel(
    A_x: jax.Array,
    A_wqkv: jax.Array,
    A_wo: jax.Array,
    B_x: jax.Array,
    B_w_r: jax.Array,
    B_w_gate: jax.Array,
    B_w_up: jax.Array,
    B_w_down: jax.Array,
):
    del B_x
    any_spec = pl.BlockSpec(memory_space=pl.ANY)
    out = pl.pallas_call(
        _kernel,
        out_shape=jax.ShapeDtypeStruct((S, D), bf16),
        in_specs=[any_spec] * 7,
        out_specs=any_spec,
        scratch_shapes=[
            pltpu.VMEM((PAD + S, D), bf16),
            pltpu.VMEM((S // 2, D + G), u32),
            pltpu.VMEM((PAD + S, D), f32),
            pltpu.VMEM((PAD + S, D), bf16),
            pltpu.VMEM((D, D + G), bf16),
            pltpu.VMEM((D, D + G), bf16),
            pltpu.VMEM((2, D, D // 2), bf16),
            pltpu.VMEM((D, D + G), bf16),
            pltpu.VMEM((D // 2, D + G), u32),
            pltpu.VMEM((D, D), f32),
            pltpu.VMEM((D // 2, D + G), u32),
            pltpu.VMEM((D, G), f32),
            pltpu.VMEM((D,), bf16),
            pltpu.VMEM((8, D), f32),
            pltpu.VMEM((2, D // 2, HT), u32),
            pltpu.VMEM((G, D), u32),
            pltpu.VMEM((G, D), f32),
            pltpu.VMEM((D, F), bf16),
            pltpu.VMEM((D, F), bf16),
            pltpu.VMEM((F, D + G), bf16),
            pltpu.VMEM((2, RB, D), bf16),
            pltpu.SemaphoreType.DMA((len(X_PIECES),)),
            pltpu.SemaphoreType.DMA((4,)),
            pltpu.SemaphoreType.DMA((8,)),
            pltpu.SemaphoreType.DMA((2 * NT - 2,)),
            pltpu.SemaphoreType.DMA((2,)),
        ],
        compiler_params=pltpu.CompilerParams(vmem_limit_bytes=100 * 1024 * 1024, disable_bounds_checks=True, disable_semaphore_checks=True),
    )(A_x.reshape(S, D), A_wqkv, A_wo, B_w_r, B_w_gate, B_w_up, B_w_down)
    return out.reshape(1, S, D)
```

```python
import jax
import jax.numpy as jnp
from jax import lax
import jax.experimental.pallas as pl
import jax.experimental.pallas.tpu as pltpu

S = 2048
D = 1024
F = 3584
H = 32
DH = D // H
LN_EPS = 1e-5
PHI_EPS = 1e-6
G = 128
NG = D // G
RB = 8
FC = 256
NF = F // FC
T = 512
NT = S // T
HT = T // 2
PAD = G

f32 = jnp.float32
bf16 = jnp.bfloat16
u32 = jnp.uint32
i32 = jnp.int32
IMIN = jnp.iinfo(jnp.int32).min

WK_PIECES = ((0, 128), (128, 128), (256, 256), (512, 512))
X_PIECES = ((0, 256), (256, 256), (512, 512), (1024, 1024))


def _zero_of(v):
    u = lax.bitcast_convert_type(v, u32)
    u = lax.shift_right_logical(lax.shift_right_logical(u, jnp.uint32(16)), jnp.uint32(16))
    return lax.bitcast_convert_type(u, f32)


def _phi(t):
    return jnp.where(t > 0, t + 1.0, jnp.exp(t)) + PHI_EPS


def _dot(a, b):
    return jnp.dot(a, b, preferred_element_type=f32)


def _dot_nt(a, b):
    return lax.dot_general(a, b, (((1,), (1,)), ((), ())), preferred_element_type=f32)


def _dot_tn(a, b):
    return lax.dot_general(a, b, (((0,), (0,)), ((), ())), preferred_element_type=f32)


def _half(lo, align):
    return lo // 2 if isinstance(lo, int) else pl.multiple_of(lo >> 1, align // 2)


def _put(ref, lo, val, align=16):
    ref[pl.ds(_half(lo, align), val.shape[0] // 2), :] = pltpu.bitcast(val, u32)


def _get(ref, lo, n, align=16):
    return pltpu.bitcast(ref[pl.ds(_half(lo, align), n // 2), :], bf16)


def _rows(lo, n, align=16):
    return pl.ds(lo if isinstance(lo, int) else pl.multiple_of(lo, align), n)


def _kernel(x_hbm, wqkv_hbm, wo_hbm, wr_hbm, wg_hbm, wu_hbm, wd_hbm, out_hbm,
            x_v, xn_v, hn_v, out_v, wk_v, wq_v, wv_v, wo_v, wqt_v, p_v, m_v, zb_v, wr_v, wrf_v,
            keep_v, nat_v, attn_v, wg_v, wu_v, wd_v, fix_v,
            sem_x, sem_k, sem_w, sem_o, sem_f):
    xn_v, wqt_v, m_v, wd_v = (r.at[:, pl.ds(0, D)] for r in (xn_v, wqt_v, m_v, wd_v))

    def x_copy(i):
        lo, n = X_PIECES[i]
        return pltpu.make_async_copy(x_hbm.at[pl.ds(lo, n)], x_v.at[pl.ds(PAD + lo, n)], sem_x.at[i])

    def wk_copy(i):
        if isinstance(i, int):
            lo, n = WK_PIECES[i]
        else:
            lo, n = pl.multiple_of(i * G, G), G
        return pltpu.make_async_copy(wqkv_hbm.at[:, pl.ds(D + lo, n)], wk_v.at[:, pl.ds(lo, n)], sem_k.at[i])

    def wv_copy(i):
        return pltpu.make_async_copy(wqkv_hbm.at[:, pl.ds(2 * D + i * 512, 512)], wv_v.at[i], sem_w.at[i])

    def out_copy(lo, n, s):
        return pltpu.make_async_copy(out_v.at[_rows(lo + PAD, n)], out_hbm.at[_rows(lo, n)], sem_o.at[s])

    wo_copy = pltpu.make_async_copy(wo_hbm, wo_v.at[:, pl.ds(0, D)], sem_w.at[2])
    wg_copy = pltpu.make_async_copy(wg_hbm, wg_v, sem_w.at[3])
    wu_copy = pltpu.make_async_copy(wu_hbm, wu_v, sem_w.at[4])
    wd_copy = pltpu.make_async_copy(wd_hbm, wd_v, sem_w.at[5])
    wr_copy = pltpu.make_async_copy(wr_hbm, wr_v, sem_w.at[6])
    wq_copy = pltpu.make_async_copy(wqkv_hbm.at[:, pl.ds(0, D)], wq_v.at[:, pl.ds(0, D)], sem_w.at[7])

    x_copy(0).start()

    def start_wk(i, c):
        wk_copy(i).start()
        return c

    lax.fori_loop(0, 2, start_wk, 0)
    wk_copy(2).start()

    def zero_pad(i, c):
        rows = pl.ds(pl.multiple_of(i * 32, 32), 32)
        x_v[rows, :] = jnp.zeros((32, D), bf16)
        attn_v[rows, :] = jnp.zeros((32, D), f32)
        return c

    lax.fori_loop(0, PAD // 32, zero_pad, 0)

    def ln_rows(lo, n, sub):
        link = None
        outs = []
        for q in range(0, n, sub):
            x = x_v[_rows(lo + (PAD + q), sub), :].astype(f32)
            mu = jnp.sum(x, axis=-1, keepdims=True) * (1.0 / D)
            if link is not None:
                mu = mu + link
            xc = x - mu
            var = jnp.sum(xc * xc, axis=-1, keepdims=True) * (1.0 / D)
            y = xc * lax.rsqrt(var + LN_EPS)
            link = _zero_of(y[:, D - G:])[:, 0:1]
            yb = y.astype(bf16)
            _put(xn_v, lo + q, yb)
            outs.append(yb)
        return jnp.concatenate(outs, axis=0) if len(outs) > 1 else outs[0]

    def kproj(xn, c0, c1):
        pk = _phi(_dot(xn, wk_v[:, pl.ds(c0, c1 - c0)]))
        zs = jnp.sum(pk.reshape(xn.shape[0] // 8, 8, c1 - c0), axis=0)
        return pk.astype(bf16), zs

    x_copy(1).start()
    x_copy(0).wait()
    wk_copy(3).start()
    ln_rows(0, 256, 256)
    wk_copy(0).wait()
    x_copy(2).start()
    pk0, z0 = kproj(_get(xn_v, 0, 256), 0, 128)
    wk_copy(1).wait()
    x_copy(3).start()
    wq_copy.start()
    pk1, z1 = kproj(_get(xn_v, 0, 256), 128, 256)
    p_v[pl.ds(0, 128), :] = _dot_tn(pk0, _get(xn_v, 0, 256))
    p_v[pl.ds(128, 128), :] = _dot_tn(pk1, _get(xn_v, 0, 256))
    wk_copy(2).wait()
    x_copy(1).wait()
    wv_copy(0).start()
    wv_copy(1).start()
    wo_copy.start()
    wr_copy.start()
    pk2, z2 = kproj(_get(xn_v, 0, 256), 256, 512)
    xb = ln_rows(256, 256, 256)
    pk_b, z_b = kproj(xb, 0, 512)
    p_v[pl.ds(256, 256), :] = _dot_tn(pk2, _get(xn_v, 0, 256))
    wk_copy(3).wait()
    x_copy(2).wait()
    wg_copy.start()
    wu_copy.start()
    wd_copy.start()
    x0 = _get(xn_v, 0, T)
    pk_c, z_c = kproj(x0, 512, D)
    p_v[pl.ds(0, 512), :] += _dot_tn(pk_b, _get(xn_v, 256, 256))
    p_v[pl.ds(512, 512), :] = _dot_tn(pk_c, x0)
    ln_rows(T, T, 32)
    zacc = jnp.concatenate([jnp.concatenate([z0, z1, z2], axis=1) + z_b, z_c], axis=1)
    x_copy(3).wait()
    wq_copy.wait()

    def l1_body(i, z):
        lo = (i + 1) * T
        xn = _get(xn_v, lo, T, T)
        pk, zs = kproj(xn, 0, D)
        p_v[...] += _dot_tn(pk, xn)
        nxt = jnp.minimum(i + 2, NT - 1) * T
        ln_rows(nxt, T, 32)
        col = pl.multiple_of(jnp.minimum(i * 3, NG - 3) * G, G)
        _put(wqt_v, col, wq_v[:, pl.ds(col, 3 * G)].T, G)
        return z + zs

    zacc = lax.fori_loop(0, NT - 1, l1_body, zacc)

    wv_copy(0).wait()
    wv_copy(1).wait()
    wo_copy.wait()
    wr_copy.wait()

    def qproj(lo, n, zb):
        pqt = _phi(_dot_nt(_get(wqt_v, 0, D), _get(xn_v, lo, n, G)))
        zt = jnp.concatenate([zb] * (n // G), axis=1)
        den = jnp.sum((pqt * zt).reshape(H, DH, n), axis=1, keepdims=True) + PHI_EPS
        inv = pl.reciprocal(den, approx=True)
        inv = inv * (2.0 - den * inv)
        return (pqt.reshape(H, DH, n) * inv).reshape(D, n).astype(bf16)

    def ml_body(i, c):
        z = jnp.sum(zacc, axis=0, keepdims=True)
        zb = jnp.broadcast_to(z, (G, D)).T
        zb_v[...] = zb
        wrf_v[...] = jnp.broadcast_to(wr_v[...].reshape(1, D).astype(f32), (8, D))
        ri = lax.broadcasted_iota(i32, (G, G), 0) // DH
        ci = lax.broadcasted_iota(i32, (G, G), 1) // DH
        same_head = ri == ci
        base = i * (D // 2)
        kvs = {}

        def kv(g):
            t = _dot(p_v[_rows(base + g * G, G, G), :].astype(bf16), wv_v[i, :, pl.ds(g * G, G)])
            kvs[g] = jnp.where(same_head, t, 0.0).astype(bf16)

        def mrow(g):
            _put(m_v, base + g * G, _dot(kvs.pop(g), wo_v[_rows(base + g * G, G, G), pl.ds(0, D)]).astype(bf16), G)

        kv(0)
        kv(1)
        mrow(0)
        keep_v[i] = pltpu.bitcast(qproj(i * HT, HT, zb), u32)
        kv(2)
        mrow(1)
        kv(3)
        mrow(2)
        mrow(3)
        return c

    lax.fori_loop(0, 2, ml_body, 0)

    sub_id = lax.broadcasted_iota(i32, (8, G), 0)

    def keys(r, lo, n):
        rb = lax.bitcast_convert_type(jnp.broadcast_to(r, (n, G)), i32)
        u = rb ^ ((rb >> 31) & 0x7FFFFFFF)
        code0 = (S - 1 - lo) - sub_id
        return rb, [(u[s8:s8 + 8] & ~(S - 1)) | (code0 - s8) for s8 in range(0, n, 8)]

    def merge(a1, a2, b1, b2):
        gt = a1 > b1
        lo = jnp.where(gt, b1, a1)
        other = jnp.where(gt, a2, b2)
        return jnp.where(gt, a1, b1), jnp.where(lo > other, lo, other)

    def post(lo, attn, n, sub, state, link):
        k1, k2 = state
        wr = wrf_v[0:1, :]
        for q in range(0, n, sub):
            rows = _rows(lo + (PAD + q), sub)
            h = x_v[rows, :].astype(f32) + attn[q:q + sub]
            mu = jnp.broadcast_to(jnp.sum(h, axis=-1, keepdims=True) * (1.0 / D), (sub, G))
            if link is not None:
                mu = mu + link
            xc = h - jnp.concatenate([mu] * NG, axis=1)
            var = jnp.sum(xc * xc, axis=-1, keepdims=True) * (1.0 / D)
            hn = xc * lax.rsqrt(var + LN_EPS)
            hn_v[rows, :] = hn
            out_v[rows, :] = (h + hn).astype(bf16)
            rb, ks = keys(jnp.sum(hn * wr, axis=-1, keepdims=True), lo + q, sub)
            link = _zero_of(rb | jnp.concatenate([k2] * (sub // 8), axis=0))
            for key in ks:
                gt = key > k1
                lo2 = jnp.where(gt, k1, key)
                k2 = jnp.where(lo2 > k2, lo2, k2)
                k1 = jnp.where(gt, key, k1)
        return (k1, k2), link

    def post_last(lo, attn, n, state):
        rows = pl.ds(lo + PAD, n)
        h = x_v[rows, :].astype(f32) + attn
        xc = h - jnp.sum(h, axis=-1, keepdims=True) * (1.0 / D)
        var = jnp.sum(xc * xc, axis=-1, keepdims=True) * (1.0 / D)
        t = jnp.sum(xc * wrf_v[0:1, :], axis=-1, keepdims=True)
        rstd = lax.rsqrt(var + LN_EPS)
        hn = xc * rstd
        hn_v[rows, :] = hn
        out_v[rows, :] = (h + hn).astype(bf16)
        _, ks = keys(t * rstd, lo, n)
        pairs = []
        for a, b in zip(ks[0::2], ks[1::2]):
            gt = a > b
            pairs.append((jnp.where(gt, a, b), jnp.where(gt, b, a)))
        pairs.append(state)
        while len(pairs) > 1:
            nxt = [merge(*pairs[j], *pairs[j + 1]) for j in range(0, len(pairs) - 1, 2)]
            pairs = nxt + pairs[len(nxt) * 2:]
        return pairs[0]

    def keep_load():
        return jnp.concatenate([pltpu.bitcast(keep_v[0], bf16), pltpu.bitcast(keep_v[1], bf16)], axis=1)

    def l2_body(i, state):
        lo = i * T
        lhs = keep_load()
        pqn = qproj(lo + T, T, zb_v[...])
        _put(nat_v, 0, pqn[:, :G].T)
        pqn = pltpu.bitcast(pqn, u32)
        keep_v[0] = pqn[:, :HT]
        keep_v[1] = pqn[:, HT:]
        (k1, k2), _ = post(lo - G, attn_v[...], G, 16, state, None)
        state = jnp.where(i > 0, k1, IMIN), jnp.where(i > 0, k2, IMIN)

        @pl.when(i > 0)
        def _():
            out_copy(lo - G, G, 2 * i - 1).start()

        m = _get(m_v, 0, D)
        at_a = _dot_tn(lhs[:, :HT], m)
        at_b = _dot_tn(lhs[:, HT:HT + G], m)
        attn_v[...] = _dot_tn(lhs[:, HT + G:], m)
        state, link = post(lo, at_a, HT, 32, state, None)
        state, _ = post(lo + HT, at_b, G, 32, state, link)
        out_copy(lo, T - G, 2 * i).start()
        return state

    init = jnp.full((8, G), IMIN, i32)
    state = lax.fori_loop(0, NT - 1, l2_body, (init, init))

    wg_copy.wait()
    wu_copy.wait()
    wd_copy.wait()
    lhs = keep_load()
    m = _get(m_v, 0, D)
    lo = S - T
    _put(nat_v, G, lhs[:, 3 * G:].T)
    at_a = _dot(_get(nat_v, 0, G), m)
    at_b = _dot_tn(lhs[:, G:3 * G], m)
    at_c = _dot(_get(nat_v, G, G), m)
    state, link = post(lo - G, attn_v[...], G, 16, state, None)
    state, link = post(lo, at_a, G, 16, state, link)
    state, _ = post(lo + G, at_b, 2 * G, 64, state, jnp.concatenate([link] * 4, axis=0))
    k1, k2 = post_last(lo + 3 * G, at_c, G, state)
    out_copy(lo - G, T + G, 2 * NT - 3).start()

    for sh in (4, 2, 1):
        k1, k2 = merge(k1, k2, pltpu.roll(k1, sh, 0), pltpu.roll(k2, sh, 0))
    k1 = k1[0:1]
    k2 = k2[0:1]

    def unkey(k):
        i = (S - 1) - (k & (S - 1))
        v = k & ~(S - 1)
        v = v ^ ((v >> 31) & 0x7FFFFFFF)
        return i, lax.bitcast_convert_type(v, f32)

    i1v, r1 = unkey(k1)
    i2v, r2 = unkey(k2)
    i1 = i1v[0, 0]
    i2 = i2v[0, 0]
    b1 = pl.multiple_of(i1 & ~(RB - 1), RB)
    b2 = pl.multiple_of(i2 & ~(RB - 1), RB)
    rid = lax.broadcasted_iota(i32, (RB, 1), 0)

    rid8 = lax.broadcasted_iota(i32, (8, D), 0)
    xs = jnp.where(rid8 == 0, jnp.broadcast_to(hn_v[pl.ds(i1 + PAD, 1), :], (8, D)),
                   jnp.broadcast_to(hn_v[pl.ds(i2 + PAD, 1), :], (8, D)))
    xsel = jnp.concatenate([xs, xs], axis=0).astype(bf16)

    acts = {}

    def gu(c):
        sl = pl.ds(c * FC, FC)
        gt = _dot(xsel, wg_v[:, sl])
        ut = _dot(xsel, wu_v[:, sl])
        acts[c] = (gt * jax.nn.sigmoid(gt) * ut).astype(bf16)

    y = None
    gu(0)
    for c in range(NF):
        if c + 1 < NF:
            gu(c + 1)
        t = _dot(acts.pop(c), wd_v[pl.ds(c * FC, FC), :])
        y = t if y is None else y + t
    s1 = jnp.concatenate([jax.nn.sigmoid(r1)] * NG, axis=1)
    s2 = jnp.concatenate([jax.nn.sigmoid(r2)] * NG, axis=1)
    y1 = y[0:1, :] * s1
    y2 = y[1:2, :] * s2

    def fixed(b):
        gid = rid + b
        upd = jnp.where(gid == i1, y1, 0.0) + jnp.where(gid == i2, y2, 0.0)
        return (out_v[_rows(b + PAD, RB, RB), :].astype(f32) + upd).astype(bf16)

    fix_v[0] = fixed(b1)
    fix_v[1] = fixed(b2)
    for i in range(NT - 1):
        if i > 0:
            out_copy(i * T - G, G, 2 * i - 1).wait()
        out_copy(i * T, T - G, 2 * i).wait()
    out_copy(lo - G, T + G, 2 * NT - 3).wait()
    fix1 = pltpu.make_async_copy(fix_v.at[0], out_hbm.at[pl.ds(b1, RB)], sem_f.at[0])
    fix2 = pltpu.make_async_copy(fix_v.at[1], out_hbm.at[pl.ds(b2, RB)], sem_f.at[1])
    fix1.start()

    @pl.when(b1 != b2)
    def _():
        fix2.start()
        fix2.wait()

    fix1.wait()


@jax.jit
def pallas_sequential_preLN__linear_attn_block__moe_arch_mod__prompt_kernel(
    A_x: jax.Array,
    A_wqkv: jax.Array,
    A_wo: jax.Array,
    B_x: jax.Array,
    B_w_r: jax.Array,
    B_w_gate: jax.Array,
    B_w_up: jax.Array,
    B_w_down: jax.Array,
):
    del B_x
    any_spec = pl.BlockSpec(memory_space=pl.ANY)
    out = pl.pallas_call(
        _kernel,
        out_shape=jax.ShapeDtypeStruct((S, D), bf16),
        in_specs=[any_spec] * 7,
        out_specs=any_spec,
        scratch_shapes=[
            pltpu.VMEM((PAD + S, D), bf16),
            pltpu.VMEM((S // 2, D + G), u32),
            pltpu.VMEM((PAD + S, D), f32),
            pltpu.VMEM((PAD + S, D), bf16),
            pltpu.VMEM((D, D + G), bf16),
            pltpu.VMEM((D, D + G), bf16),
            pltpu.VMEM((2, D, D // 2), bf16),
            pltpu.VMEM((D, D + G), bf16),
            pltpu.VMEM((D // 2, D + G), u32),
            pltpu.VMEM((D, D), f32),
            pltpu.VMEM((D // 2, D + G), u32),
            pltpu.VMEM((D, G), f32),
            pltpu.VMEM((D,), bf16),
            pltpu.VMEM((8, D), f32),
            pltpu.VMEM((2, D // 2, HT), u32),
            pltpu.VMEM((G, D), u32),
            pltpu.VMEM((G, D), f32),
            pltpu.VMEM((D, F), bf16),
            pltpu.VMEM((D, F), bf16),
            pltpu.VMEM((F, D + G), bf16),
            pltpu.VMEM((2, RB, D), bf16),
            pltpu.SemaphoreType.DMA((len(X_PIECES),)),
            pltpu.SemaphoreType.DMA((4,)),
            pltpu.SemaphoreType.DMA((8,)),
            pltpu.SemaphoreType.DMA((2 * NT - 2,)),
            pltpu.SemaphoreType.DMA((2,)),
        ],
        compiler_params=pltpu.CompilerParams(vmem_limit_bytes=100 * 1024 * 1024, disable_bounds_checks=True, disable_semaphore_checks=True),
    )(A_x.reshape(S, D), A_wqkv, A_wo, B_w_r, B_w_gate, B_w_up, B_w_down)
    return out.reshape(1, S, D)
```
